```python
import os as _os
_os.environ.setdefault('JAX_PLATFORMS', 'cpu')
import jax
import jax.numpy as jnp

def _softmax(x, axis=-1):
    return jax.nn.softmax(x, axis=axis)

def _gelu(x):
    return jax.nn.gelu(x, approximate=True)

def _silu(x):
    return jax.nn.silu(x)

def _sigmoid(x):
    return jax.nn.sigmoid(x)

def _layernorm(x, axis=-1, eps=1e-05):
    m = jnp.mean(x, axis=axis, keepdims=True)
    v = jnp.var(x, axis=axis, keepdims=True)
    return (x - m) / jnp.sqrt(v + eps)

def _scatter_add(tgt, idx, src, axis=0):
    return tgt.at[idx].add(src)

def _segment_sum(src, seg, n):
    return jax.ops.segment_sum(src, seg, n)

class _Rng:

    def __init__(self, key):
        self._k = key

    def _next(self):
        self._k, sub = jax.random.split(self._k)
        return sub

    def normal(self, shape):
        return jax.random.normal(self._next(), shape, dtype=jnp.bfloat16)

    def randint(self, lo, hi, shape):
        return jax.random.randint(self._next(), shape, lo, hi, dtype=jnp.int32)

    def uniform(self, shape, lo=0.0, hi=1.0):
        return jax.random.uniform(self._next(), shape, jnp.bfloat16, lo, hi)

    def permutation(self, n):
        return jax.random.permutation(self._next(), n)
kernel_name = 'concat_heads__spectral_gfnet__memory_aug_recurrent_mem_tr__prompt'

def setup_inputs():
    _rng = _Rng(jax.random.key(int.from_bytes(__import__("os").urandom(4), "little")))
    _w = lambda a: (lambda t: t.astype(jnp.bfloat16) if jnp.issubdtype(t.dtype, jnp.floating) else t)(jnp.asarray(a))

    def _A_setup():
        B, S, D = (1, 2048, 512)
        Df = D // 2 + 1
        return {'x': _w((lambda *s: _rng.normal(s) * 0.05)(B, S, D)), 'w_r': _w((lambda *s: _rng.normal(s) * 0.05)(S, Df) * 0.02), 'w_i': _w((lambda *s: _rng.normal(s) * 0.05)(S, Df) * 0.02)}
    _A_in = _A_setup()

    def _B_setup():
        B, S, Dm = (1, 2048, 512)
        H, Dh = (32, 128)
        M, seg = (8, 32)
        seg = min(seg, S)
        S = S // seg * seg
        return {'x': _w((lambda *s: _rng.normal(s) * 0.05)(B, S, Dm)), 'mem0': _w((lambda *s: _rng.normal(s) * 0.4)(B, M, Dm)), 'Wq': _w((lambda *s: _rng.normal(s) * 3.2)(Dm, H, Dh) * Dm ** (-0.5)), 'Wk': _w((lambda *s: _rng.normal(s) * 3.2)(Dm, H, Dh) * Dm ** (-0.5)), 'Wv': _w((lambda *s: _rng.normal(s) * 0.4)(Dm, H, Dh) * Dm ** (-0.5)), 'Wo': _w((lambda *s: _rng.normal(s) * 0.4)(H, Dh, Dm) * (H * Dh) ** (-0.5)), 'seg_len': seg}
    _B_in = _B_setup()
    return {'A_x': _A_in['x'], 'A_w_r': _A_in['w_r'], 'A_w_i': _A_in['w_i'], 'B_x': _B_in['x'], 'B_mem0': _B_in['mem0'], 'B_Wq': _B_in['Wq'], 'B_Wk': _B_in['Wk'], 'B_Wv': _B_in['Wv'], 'B_Wo': _B_in['Wo'], 'B_seg_len': _B_in['seg_len']}

def reference(A_x, A_w_r, A_w_i, B_x, B_mem0, B_Wq, B_Wk, B_Wv, B_Wo, B_seg_len):

    def _A_ref(x, w_r, w_i):
        B, S, D = x.shape
        X = (lambda x, axes=(-2, -1): jnp.fft.rfft2(x.astype(jnp.float32), axes=axes))(x, axes=(-2, -1))
        W = w_r + 1j * w_i
        X = X * W
        y = (lambda x, s, axes=(-2, -1): jnp.fft.irfft2(x, s=s, axes=axes).astype(jnp.bfloat16))(X, (S, D), axes=(-2, -1))
        return y

    def _B_ref(x, mem0, Wq, Wk, Wv, Wo, seg_len):
        B, S, Dm = x.shape
        H, Dh = (Wq.shape[1], Wq.shape[2])
        M = mem0.shape[1]
        scale = Dh ** (-0.5)
        n_seg = S // seg_len
        L = M + seg_len
        idx = jnp.arange(L)
        mask = (idx[:, None] < M) | (idx[:, None] >= idx[None, :])
        mem = mem0
        outs = []
        for s in range(n_seg):
            xs = x[:, s * seg_len:(s + 1) * seg_len, :].copy()
            h = jnp.concatenate([mem, xs], axis=1)
            q = jnp.einsum('btd,dhe->bhte', h, Wq)
            k = jnp.einsum('btd,dhe->bhte', h, Wk)
            v = jnp.einsum('btd,dhe->bhte', h, Wv)
            scores = jnp.einsum('bhqe,bhke->bhqk', q, k) * scale
            scores = jnp.where(mask[None, None], scores, -1000000000.0)
            p = _softmax(scores, axis=-1)
            o = jnp.einsum('bhqk,bhke->bhqe', p, v)
            o = jnp.einsum('bhte,hed->btd', o, Wo)
            mem = o[:, :M, :].copy()
            outs.append(o[:, M:, :])
        return jnp.concatenate(outs, axis=1)
    a = _A_ref(A_x, A_w_r, A_w_i)
    b = _B_ref(B_x, B_mem0, B_Wq, B_Wk, B_Wv, B_Wo, B_seg_len)
    return jnp.concatenate([a, b], axis=-1)
```

```python
import contextlib
import functools
import os

import numpy as np
import jax
import jax.numpy as jnp
from jax import lax
import jax.experimental.pallas as pl
import jax.experimental.pallas.tpu as pltpu

F32 = jnp.float32
BF16 = jnp.bfloat16
U32 = jnp.uint32

S, D = 2048, 512
H, DH = 32, 128
M, SEG = 8, 32
L = M + SEG
NP = H // 2
NIT = S // (2 * SEG)
SCALE = DH ** -0.5
LOG2E = 1.4426950408889634
NEG = -1000000000.0


def _nt(a, b):
    return lax.dot_general(a, b, (((1,), (1,)), ((), ())), preferred_element_type=F32)


def _nn(a, b):
    return jnp.dot(a, b, preferred_element_type=F32)


def _tobf(u):
    return pltpu.bitcast(u, BF16)


def _tou(b):
    return pltpu.bitcast(b, U32)


def _lo(u):
    return pltpu.bitcast(u << 16, F32)


def _hi(u):
    return pltpu.bitcast(u & jnp.uint32(0xFFFF0000), F32)


def _cs(num, den):
    ang = 2.0 * np.pi * np.mod(num, den) / den
    c, s = np.cos(ang), np.sin(ang)
    c[np.abs(c) < 1e-12] = 0.0
    s[np.abs(s) < 1e-12] = 0.0
    return c, s


def _fft_consts():
    d1, d2 = np.arange(128), np.arange(256)
    j80, j64, j128 = np.arange(80), np.arange(64), np.arange(128)
    c, s = _cs(np.outer(4 * j80, d1), D)
    c[65:] = 0.0
    s[65:] = 0.0
    l0 = np.concatenate([c, -s], 0)
    c, s = _cs(np.outer(4 * j64 + 2, d1), D)
    l2 = np.concatenate([c, -s], 0)
    c, s = _cs(np.outer(2 * j128 + 1, d2), D)
    l1 = np.concatenate([c, -s], 0)
    cc, ss = _cs(np.outer(j128, j128), 128)
    g = np.block([[cc, -ss], [ss, cc]])
    sc = 1.0 / (S * D)
    c, s = _cs(np.outer(4 * j64, d1), D)
    i0 = np.concatenate([2 * c, -2 * s], 0)
    i0[0] = 1.0
    i0[64] = 1.0 - 2.0 * (d1 % 2)
    l2p = np.concatenate([l2, np.zeros((32, 128))], 0)
    cf = np.concatenate([l1, g, np.concatenate([l0, l2p], 1)], 0)
    gi = []
    for n2 in range(16):
        c, s = _cs(np.outer(16 * j128 + n2, j128), S)
        gi.append(np.concatenate([c, -s], 1))
    ci = np.concatenate([2 * sc * l1, np.concatenate([i0 * sc, 2 * sc * l2], 1)] + gi, 0)
    tc, ts = _cs(np.outer(np.arange(16), j128), S)
    tw = np.concatenate([tc, ts], 0)
    return cf.astype(np.float32), ci.astype(np.float32), tw.astype(np.float32)


def _cmul_const(z, k, n, sign):
    re, im = z
    k = k % n
    if k == 0:
        return z
    if 4 * k == n:
        return (-im, re) if sign > 0 else (im, -re)
    c = float(np.cos(2 * np.pi * k / n))
    s = float(sign * np.sin(2 * np.pi * k / n))
    if (8 * k) % n == 0:
        a, b = re * c, im * c
        return (a - b, b + a) if s / c > 0 else (a + b, b - a)
    return (re * c - im * s, re * s + im * c)


def _dft4(a, b, c, d, sign):
    s0 = (a[0] + c[0], a[1] + c[1])
    s1 = (a[0] - c[0], a[1] - c[1])
    s2 = (b[0] + d[0], b[1] + d[1])
    s3 = (b[0] - d[0], b[1] - d[1])
    y0 = (s0[0] + s2[0], s0[1] + s2[1])
    y2 = (s0[0] - s2[0], s0[1] - s2[1])
    ya = (s1[0] + s3[1], s1[1] - s3[0])
    yb = (s1[0] - s3[1], s1[1] + s3[0])
    return [y0, ya, y2, yb] if sign < 0 else [y0, yb, y2, ya]


def _dft16(z, sign):
    t = [_dft4(z[b], z[4 + b], z[8 + b], z[12 + b], sign) for b in range(4)]
    out = [None] * 16
    for p in range(4):
        u = [_cmul_const(t[b][p], b * p, 16, sign) for b in range(4)]
        y = _dft4(u[0], u[1], u[2], u[3], sign)
        for q in range(4):
            out[p + 4 * q] = y[q]
    return out


_SCOPES = bool(os.environ.get("KSCOPES"))


def _scope(name):
    return jax.named_scope(name) if _SCOPES else contextlib.nullcontext()


SEM_XA = 0
SEM_XE = 3
SEM_W = 4
SEM_F = 14
SEM_B = 15
SEM_INV = 16
SEM_OA = 17
SEM_OB = 18
SEM_OB2 = 19
NSEM = 20
XA_GROUPS = (0, 1, 1, 2, 2, 2, 2, 2)
NA = 4
OA_POINTS = {4: 0, 7: 5}


def _wgroup(b):
    return 0 if b < 4 else 1 + (b - 4) // 5


def _kernel(xa_hbm, wr_hbm, wi_hbm, xb_hbm, mem0_hbm, wq_hbm, wk_hbm, wv_hbm, wo_hbm,
            cf_hbm, ci_hbm, tw_hbm, out_hbm,
            xa, wr, wi, cf, ci, tw, u_scr, yu,
            xb, xe, mem0, raw, w, wo, pre, carry8, q_scr, k_scr, v_scr, p_scr,
            om_scr, ox_scr, outb, fill_scr, sems):
    cp = pltpu.make_async_copy
    out_u = out_hbm.bitcast(U32)
    xa_u = xa_hbm.bitcast(U32)
    xb_u = xb_hbm.bitcast(U32)

    ra = 256 - 8 * NA
    c_fwd = [cp(cf_hbm.bitcast(U32), cf, sems.at[SEM_XA]), cp(tw_hbm, tw, sems.at[SEM_XA])]
    c_xa = [cp(xa_u.at[:, c, :], xa.at[c], sems.at[SEM_XA + XA_GROUPS[c]]) for c in range(8)]
    c_xe = [cp(xb_u.at[:, 12:20, :], xe, sems.at[SEM_XE]),
            cp(wr_hbm.at[ra:257], wr.at[ra:257], sems.at[SEM_XE]),
            cp(wi_hbm.at[ra:257], wi.at[ra:257], sems.at[SEM_XE])]
    c_w = []
    for t, src in enumerate((wq_hbm, wk_hbm, wv_hbm)):
        su = src.bitcast(U32)
        for p in range(NP):
            b = t * NP + p
            c_w.append(cp(su.at[:, p, :], raw.at[b], sems.at[SEM_W + _wgroup(b)]))
    c_f = [cp(wo_hbm.bitcast(U32), wo, sems.at[SEM_F]),
           cp(mem0_hbm, mem0, sems.at[SEM_F]),
           cp(xb_u.at[0:NA + 1], xb.at[0:NA + 1], sems.at[SEM_F])]
    c_b = [cp(xb_u.at[NA + 1:NIT], xb.at[NA + 1:NIT], sems.at[SEM_B]),
           cp(wr_hbm.at[0:ra], wr.at[0:ra], sems.at[SEM_B]),
           cp(wi_hbm.at[0:ra], wi.at[0:ra], sems.at[SEM_B])]
    c_inv = [cp(ci_hbm.bitcast(U32), ci, sems.at[SEM_INV])]
    for c in c_fwd + c_xa + c_xe[:1] + c_w[:4] + c_xe[1:] + c_w[4:] + c_f + c_b + c_inv:
        c.start()

    def wait_blocks(g, b0, n):
        blk = raw.at[pl.ds(b0, n)]
        cp(blk, blk, sems.at[SEM_W + g]).wait()

    def relayout_q(b, qt):
        e = raw[b, pl.ds(qt * 128, 64, stride=2), :]
        o = raw[b, pl.ds(qt * 128 + 1, 64, stride=2), :]
        rows = pl.ds(qt * 64, 64)
        w[b, rows, 0:128] = (e & jnp.uint32(0xFFFF)) | (o << 16)
        w[b, rows, 128:256] = (e >> 16) | (o & jnp.uint32(0xFFFF0000))

    def relayout(b):
        for qt in range(4):
            relayout_q(b, qt)

    def precompute(b, h):
        lhs = _tobf(xe[...].reshape(NIT * 8, D))
        pre[b, :, h * 128:(h + 1) * 128] = _nn(lhs, _tobf(w[b, :, h * 128:(h + 1) * 128]))

    ox_scr[...] = jnp.zeros_like(ox_scr)
    u_scr[:, :, 256:264, :] = jnp.zeros((16, 2, 8, 128), F32)

    row = lax.broadcasted_iota(jnp.int32, (80, 80), 0)
    col = lax.broadcasted_iota(jnp.int32, (80, 80), 1)
    rhead = jnp.where(row < 16, row // 8, (row - 16) // SEG)
    same_head = rhead == col // L
    fill_scr[...] = jnp.where(same_head, NEG / SCALE, -jnp.inf).astype(F32)

    def f1_d(n2):
        u = xa[n2 // 2]
        xf = _lo(u) if n2 % 2 == 0 else _hi(u)
        x0, x1, x2, x3 = [xf[:, j * 128:(j + 1) * 128] for j in range(4)]
        p = x0 + x2
        q = x1 + x3
        a0 = (p + q).astype(BF16)
        a2 = (p - q).astype(BF16)
        bc = jnp.concatenate([x0 - x2, x1 - x3], axis=1).astype(BF16)
        t0 = _nt(_tobf(cf[256:336, 0:128]), a0)
        t2 = _nt(_tobf(cf[256:320, 128:256]), a2)
        t1 = _nt(_tobf(cf[0:128, :]), bc)
        tr = jnp.concatenate([t0[0:80], t2[0:64], t1[0:128]], axis=0)
        ti = jnp.concatenate([t0[80:160], t2[64:128], t1[128:256]], axis=0)
        return jnp.concatenate([tr, ti], axis=1).astype(BF16)

    def f1_s(n2, t):
        u = _nn(t, _tobf(cf[128:256, :]))
        ur, ui = u[:, 0:128], u[:, 128:256]
        if n2:
            c, s = tw[n2:n2 + 1, :], tw[16 + n2:17 + n2, :]
            ur, ui = ur * c + ui * s, ui * c - ur * s
        for h, uh in enumerate((ur, ui)):
            u_scr[n2, h, pl.ds(0, 64, stride=4), :] = uh[0:64]
            u_scr[n2, h, 256:257, :] = uh[64:65]
            u_scr[n2, h, pl.ds(2, 64, stride=4), :] = uh[80:144]
            u_scr[n2, h, pl.ds(1, 128, stride=2), :] = uh[144:272]

    def f2(r0, fr, fi):
        z = []
        for n2 in range(16):
            re = u_scr[n2, 0, pl.ds(r0, 8), :]
            im = u_scr[n2, 1, pl.ds(r0, 8), :]
            z.append((re, im))
        x = _dft16(z, -1)
        y = []
        for j in range(16):
            a, b = fr(j), fi(j)
            y.append((x[j][0] * a - x[j][1] * b, x[j][0] * b + x[j][1] * a))
        v = _dft16(y, +1)
        for n2 in range(16):
            re, im = v[n2]
            u_scr[n2, 0, pl.ds(r0, 8), :] = re
            u_scr[n2, 1, pl.ds(r0, 8), :] = im

    def wait_xa(g):
        for c in range(8):
            if XA_GROUPS[c] == g:
                c_xa[c].wait()

    with _scope("w0"):
        for c in c_fwd:
            c.wait()
        wait_xa(0)
    with _scope("f1"):
        t_prev = f1_d(0)
        for n2 in range(1, 16):
            if n2 % 2 == 0 and XA_GROUPS[n2 // 2] != XA_GROUPS[n2 // 2 - 1]:
                wait_xa(XA_GROUPS[n2 // 2])
            t = f1_d(n2)
            f1_s(n2 - 1, t_prev)
            t_prev = t
        for c in c_xe:
            c.wait()
        wait_blocks(0, 0, 4)
        f1_s(15, t_prev)
        for b in range(4):
            relayout(b)
        wl_r = wr[256:257, :].astype(F32)
        wl_i = wi[256:257, :].astype(F32)
        f2(256,
           lambda j: jnp.broadcast_to(wl_r[:, j * 128:(j + 1) * 128], (8, 128)),
           lambda j: jnp.broadcast_to(wl_i[:, j * 128:(j + 1) * 128], (8, 128)))

    def pre_body(g, _):
        b0 = 4 + 5 * g
        wait_blocks(g + 1, b0, 5)
        pieces = [(t, qt) for t in range(5) for qt in range(4)]
        for t in range(8):
            precompute(g * 4 + t // 2, t % 2)
            for (rb, qt) in pieces[(5 * t) // 2:(5 * (t + 1)) // 2]:
                relayout_q(b0 + rb, qt)
        return 0

    with _scope("pre"):
        lax.fori_loop(0, 8, pre_body, 0)
    with _scope("w1"):
        wait_blocks(9, 44, 4)
        for b in range(44, 48):
            relayout(b)
        for c in c_f:
            c.wait()

    rpos = jnp.where(row < 16, L, (row - 16) % SEG + M)
    mask = same_head & (rpos >= col % L)

    def qkv(i, lhs, lhs_v, p, even):
        b = 0 if even else 1
        rq = _nn(lhs, _tobf(w[p]))
        rk = _nn(lhs, _tobf(w[NP + p]))
        rv = _nn(lhs_v, _tobf(w[2 * NP + p]))
        r16 = pl.multiple_of(i * 16, 16)
        if even:
            xq = jnp.concatenate([rq[8:32], pre[p, pl.ds(r16, 8), :]], axis=0)
            xk = jnp.concatenate([rk[8:32], pre[NP + p, pl.ds(r16, 8), :]], axis=0)
            xv = rv[8:40]
            carry8[p] = rv[40:48]
        else:
            xq = jnp.concatenate([pre[p, pl.ds(r16 + 8, 8), :], rq[8:32]], axis=0)
            xk = jnp.concatenate([pre[NP + p, pl.ds(r16 + 8, 8), :], rk[8:32]], axis=0)
            xv = jnp.concatenate([carry8[p], rv[8:32]], axis=0)
        h0 = lambda a: a[:, 0:128]
        h1 = lambda a: a[:, 128:256]
        mq, mk, mv = rq[0:8], rk[0:8], rv[0:8]
        q_scr[b, p] = _tou(jnp.concatenate([h0(mq), h1(mq), h0(xq), h1(xq)], axis=0).astype(BF16))
        k_scr[b, p] = _tou(jnp.concatenate([h0(mk), h0(xk), h1(mk), h1(xk)], axis=0).astype(BF16))
        v_scr[b, p] = _tou(jnp.concatenate([h0(mv), h0(xv), h1(mv), h1(xv)], axis=0).astype(BF16))

    def qk_group(g, even):
        b = 0 if even else 1
        for p in range(4 * g, 4 * g + 4):
            s = _nt(_tobf(q_scr[b, p]), _tobf(k_scr[b, p]))
            s = jnp.where(mask, s, fill_scr[...])
            m = jnp.max(s, axis=-1, keepdims=True)
            e = jnp.exp2((s - m) * (SCALE * LOG2E))
            l = jnp.sum(e, axis=-1, keepdims=True)
            p_scr[b, p] = _tou((e * pl.reciprocal(l, approx=True)).astype(BF16))

    def put_om(p, o):
        om_scr[:, (2 * p) * 128:(2 * p + 1) * 128] = o[0:8]
        om_scr[:, (2 * p + 1) * 128:(2 * p + 2) * 128] = o[8:16]

    def put_ox(b, p, o):
        ox_scr[b, :, (2 * p) * 128:(2 * p + 1) * 128] = o[0:32]
        ox_scr[b, :, (2 * p + 1) * 128:(2 * p + 2) * 128] = o[32:64]

    def pvm_group(g, even):
        b = 0 if even else 1
        for p in range(4 * g, 4 * g + 4):
            put_om(p, _nn(_tobf(p_scr[b, p, 0:8, :]), _tobf(v_scr[b, p])))

    def pvx_group(g, even):
        b = 0 if even else 1
        for p in range(4 * g, 4 * g + 4):
            put_ox(b, p, _nn(_tobf(p_scr[b, p, 8:40, :]), _tobf(v_scr[b, p])))

    def pv_group(g, even):
        b = 0 if even else 1
        for p in range(4 * g, 4 * g + 4):
            o = _nn(_tobf(p_scr[b, p]), _tobf(v_scr[b, p]))
            put_om(p, o[0:16])
            put_ox(b, p, o[16:80])

    def oproj(c, even, acc):
        cs = slice(c * 512, (c + 1) * 512)
        if even:
            lhs = jnp.concatenate([om_scr[:, cs], ox_scr[0, 24:32, cs], ox_scr[1, :, cs]], axis=0)
        else:
            lhs = jnp.concatenate([om_scr[:, cs], ox_scr[0, 0:24, cs]], axis=0)
        r = _nn(lhs.astype(BF16), _tobf(wo[c * 256:(c + 1) * 256, :]))
        return r if acc is None else r + acc

    def step(i, lhs_v, even):
        lhs = lhs_v[0:32]
        pv = pvm_group if even else pv_group
        for p in range(4):
            qkv(i, lhs, lhs_v, p, even)
        for g in range(3):
            qkv(i, lhs, lhs_v, 4 * g + 4, even)
            qk_group(g, even)
            for p in range(4 * g + 5, 4 * g + 8):
                qkv(i, lhs, lhs_v, p, even)
            pv(g, even)
        acc = oproj(0, even, None)
        qk_group(3, even)
        for c in range(1, 4):
            acc = oproj(c, even, acc)
        pv(3, even)
        for c in range(4, 8):
            acc = oproj(c, even, acc)
        if even:
            for g in range(4):
                pvx_group(g, even)
        return acc

    def out_copy(i):
        return cp(outb.at[pl.ds(4 * i, 4)], out_u.at[pl.ds(4 * i - 3, 4), :, D:2 * D], sems.at[SEM_OB])

    def even_lhs(i, mem):
        xf = _tobf(xb[i, 0:24, :]).astype(F32)
        return _tou(jnp.concatenate([mem, xf[0:40]], axis=0).astype(BF16))

    def body(i, carry):
        lhs_u, stash = carry

        @pl.when(i == NA)
        def _():
            for c in c_b:
                c.wait()

        acc = step(i, _tobf(lhs_u), True)
        o48 = _tou(jnp.concatenate([stash, acc[8:48]], axis=0).astype(BF16))
        outb[pl.ds(4 * i, 3)] = o48.reshape(3, 8, D)
        xf = _tobf(xb[i, 16:32, :]).astype(F32)
        acc = step(i, jnp.concatenate([acc[0:8], xf[8:32]], axis=0).astype(BF16), False)
        outb[4 * i + 3] = _tou(acc[8:24].astype(BF16))
        r8 = pl.multiple_of((NIT - 1 - i) * 8, 8)
        f2(r8,
           lambda j: wr[pl.ds(r8, 8), j * 128:(j + 1) * 128].astype(F32),
           lambda j: wi[pl.ds(r8, 8), j * 128:(j + 1) * 128].astype(F32))
        lhs_next = even_lhs(jnp.minimum(i + 1, NIT - 1), acc[0:8])

        @pl.when(i > 0)
        def _():
            out_copy(i).start()

        return lhs_next, acc[24:32]

    with _scope("main"):
        _, stash = lax.fori_loop(0, NIT, body, (even_lhs(0, mem0[...].astype(F32)), jnp.zeros((8, D), F32)))

    first = lax.broadcasted_iota(jnp.int32, (8, 128), 0) == 0

    def f3_s(n2):
        r0, i0 = [u_scr[n2, h, pl.ds(0, 64, stride=4), :] for h in range(2)]
        r2, i2 = [u_scr[n2, h, pl.ds(2, 64, stride=4), :] for h in range(2)]
        r1, i1 = [u_scr[n2, h, pl.ds(1, 128, stride=2), :] for h in range(2)]
        rl, il = [u_scr[n2, h, 256:264, :] for h in range(2)]
        rhs1 = jnp.concatenate([r0, jnp.where(first, rl, i0[0:8]), i0[8:64], r2, i2, r1, i1], axis=0)
        rhs2 = jnp.concatenate([i0, jnp.where(first, il, -r0[0:8]), -r0[8:64], i2, -r2, i1, -r1], axis=0)
        rhs = jnp.concatenate([rhs1, rhs2], axis=1).astype(BF16)
        return _nt(_tobf(ci[192 + 64 * n2:256 + 64 * n2, :]), rhs).astype(BF16)

    c_oa = [cp(yu.at[c], out_u.at[:, c, 0:D], sems.at[SEM_OA]) for c in range(8)]

    def f3_d(z):
        b0 = _nn(z[:, 0:128], _tobf(ci[128:192, 0:128]))
        b2 = _nn(z[:, 128:256], _tobf(ci[128:192, 128:256]))
        o = _nn(z[:, 256:512], _tobf(ci[0:128, :]))
        p = b0 + b2
        q = b0 - b2
        return jnp.concatenate([p + o[:, 0:128], q + o[:, 128:256], p - o[:, 0:128], q - o[:, 128:256]], axis=1)

    def f3_out(c, z):
        yu[c] = pltpu.pack_elementwise([f3_d(z[0]), f3_d(z[1])], packed_dtype=BF16)

    with _scope("f3"):
        c_first = cp(outb.at[3:4], out_u.at[0:1, :, D:2 * D], sems.at[SEM_OB2])
        c_first.start()
        for c in c_inv:
            c.wait()
        zp = (f3_s(0), f3_s(1))
        for c in range(1, 8):
            z = (f3_s(2 * c), f3_s(2 * c + 1))
            f3_out(c - 1, zp)
            if c - 1 in OA_POINTS:
                for cc in range(OA_POINTS[c - 1], c):
                    c_oa[cc].start()
            zp = z
        f3_out(7, zp)
        for cc in range(OA_POINTS[7], 8):
            c_oa[cc].start()
    with _scope("epi"):
        lhs = jnp.concatenate([ox_scr[0, 24:32, :], ox_scr[1]], axis=0).astype(BF16)
        acc = _nn(lhs, _tobf(wo[...]))
        o48 = _tou(jnp.concatenate([stash, acc], axis=0).astype(BF16))
        outb[4 * NIT:4 * NIT + 3] = o48.reshape(3, 8, D)
        c_last = cp(outb.at[4 * NIT:4 * NIT + 3], out_u.at[4 * NIT - 3:4 * NIT, :, D:2 * D], sems.at[SEM_OB2])
        c_last.start()
        for c in c_oa:
            c.wait()
        for i in range(1, NIT):
            out_copy(i).wait()
        c_first.wait()
        c_last.wait()


@functools.partial(jax.jit, static_argnames=("B_seg_len",))
def pallas_concat_heads__spectral_gfnet__memory_aug_recurrent_mem_tr__prompt_kernel(
    A_x, A_w_r, A_w_i, B_x, B_mem0, B_Wq, B_Wk, B_Wv, B_Wo, B_seg_len,
):
    assert int(B_seg_len) == SEG
    assert A_x.shape == (1, S, D) and B_x.shape == (1, S, D) and B_mem0.shape == (1, M, D)
    cf, ci, tw = _fft_consts()
    hbm = pl.BlockSpec(memory_space=pltpu.HBM)
    out = pl.pallas_call(
        _kernel,
        out_shape=jax.ShapeDtypeStruct((S // 16, 16, 2 * D), BF16),
        in_specs=[hbm] * 12,
        out_specs=hbm,
        scratch_shapes=[
            pltpu.VMEM((8, 128, D), U32),
            pltpu.VMEM((257, S), BF16),
            pltpu.VMEM((257, S), BF16),
            pltpu.VMEM((336, 256), U32),
            pltpu.VMEM((1216, 256), U32),
            pltpu.VMEM((32, 128), F32),
            pltpu.VMEM((16, 2, 264, 128), F32),
            pltpu.VMEM((8, 128, D), U32),
            pltpu.VMEM((NIT, 32, D), U32),
            pltpu.VMEM((NIT, 8, D), U32),
            pltpu.VMEM((M, D), BF16),
            pltpu.VMEM((3 * NP, D, 128), U32),
            pltpu.VMEM((3 * NP, D // 2, 256), U32),
            pltpu.VMEM((H * DH // 2, D), U32),
            pltpu.VMEM((2 * NP, NIT * 16, 256), F32),
            pltpu.VMEM((NP, 8, 256), F32),
            pltpu.VMEM((2, NP, 40, 128), U32),
            pltpu.VMEM((2, NP, 40, 128), U32),
            pltpu.VMEM((2, NP, 40, 128), U32),
            pltpu.VMEM((2, NP, 40, 80), U32),
            pltpu.VMEM((M, H * DH), F32),
            pltpu.VMEM((2, SEG, H * DH), F32),
            pltpu.VMEM((4 * NIT + 3, 8, D), U32),
            pltpu.VMEM((80, 80), F32),
            pltpu.SemaphoreType.DMA((NSEM,)),
        ],
        compiler_params=pltpu.CompilerParams(vmem_limit_bytes=100 * 1024 * 1024),
    )(
        A_x.reshape(S // 16, 16, D), A_w_r.T, A_w_i.T,
        B_x.reshape(NIT, 2 * SEG, D), B_mem0.reshape(M, D),
        B_Wq, B_Wk, B_Wv, B_Wo.reshape(H * DH, D),
        jnp.asarray(cf, BF16), jnp.asarray(ci, BF16), jnp.asarray(tw),
    )
    return out.reshape(1, S, 2 * D)
```

```python
import functools

import numpy as np
import jax
import jax.numpy as jnp
from jax import lax
import jax.experimental.pallas as pl
import jax.experimental.pallas.tpu as pltpu

F32 = jnp.float32
BF16 = jnp.bfloat16
U32 = jnp.uint32

S, D = 2048, 512
H, DH = 32, 128
M, SEG = 8, 32
L = M + SEG
NP = H // 2
NIT = S // (2 * SEG)
SCALE = DH ** -0.5
LOG2E = 1.4426950408889634
NEG = -1000000000.0
R2 = float(np.sqrt(0.5))


def _nt(a, b):
    return lax.dot_general(a, b, (((1,), (1,)), ((), ())), preferred_element_type=F32)


def _nn(a, b):
    return jnp.dot(a, b, preferred_element_type=F32)


def _tobf(u):
    return pltpu.bitcast(u, BF16)


def _tou(b):
    return pltpu.bitcast(b, U32)


def _swap(a):
    return pltpu.roll(a, 64, a.ndim - 1)


def _cs(num, den):
    ang = 2.0 * np.pi * np.mod(num, den) / den
    c, s = np.cos(ang), np.sin(ang)
    c[np.abs(c) < 1e-12] = 0.0
    s[np.abs(s) < 1e-12] = 0.0
    return c, s


def _pack_rows(a):
    b = np.asarray(a, np.float32).astype(jnp.bfloat16).view(np.uint16).astype(np.uint32)
    return b[0::2] | (b[1::2] << 16)


def _fft_consts():
    d1, e64, j32 = np.arange(128), np.arange(64), np.arange(32)
    f0 = np.concatenate([8 * j32, 8 * j32 + 4])
    f2 = np.concatenate([8 * j32 + 2, 8 * j32 + 6])
    fa = np.concatenate([8 * j32 + 1, 8 * j32 + 7])
    fb = np.concatenate([8 * j32 + 5, 8 * j32 + 3])
    c, s = _cs(np.outer(f0, d1), D)
    l0 = np.concatenate([c, -s], 0)
    l0[64] = 1.0 - 2.0 * (d1 % 2)
    c, s = _cs(np.outer(f2, d1), D)
    l2 = np.concatenate([c, -s], 0)

    def odd(f, imsign):
        c, s = _cs(np.outer(f, e64), D)
        sg = np.where(f % 4 == 1, imsign, -imsign)[:, None]
        return np.block([[c, sg * s], [-s, sg * c]])

    la, lb = odd(fa, -1.0), odd(fb, 1.0)
    g, hm = [], []
    for par in range(2):
        c, s = _cs(np.outer(2 * e64 + par, e64), 128)
        sg = 1.0 - 2.0 * par
        g.append(np.block([[c, -s], [s, c]]))
        hm.append(np.block([[c, -sg * s], [s, sg * c]]))
    sc = 2.0 / (S * D)
    i0 = sc * l0
    i0[0] *= 0.5
    i0[64] *= 0.5
    il = lambda a: a.reshape(2, 4, 16, 128).transpose(1, 0, 2, 3).reshape(128, 128)
    mats = [il(l0), il(l2), il(la), il(lb), g[0], g[1], il(hm[0]), il(hm[1]), i0, sc * l2, sc * la, sc * lb]
    tc, ts = _cs(np.outer(np.arange(16), d1), S)
    return _pack_rows(np.concatenate(mats, 0)), np.concatenate([tc, ts], 0).astype(np.float32)


def _cmul_const(z, k, n, sign):
    re, im = z
    k = k % n
    if k == 0:
        return z
    if 4 * k == n:
        return (-im, re) if sign > 0 else (im, -re)
    c = float(np.cos(2 * np.pi * k / n))
    s = float(sign * np.sin(2 * np.pi * k / n))
    if (8 * k) % n == 0:
        a, b = re * c, im * c
        return (a - b, b + a) if s / c > 0 else (a + b, b - a)
    return (re * c - im * s, re * s + im * c)


def _dft4(a, b, c, d, sign):
    s0 = (a[0] + c[0], a[1] + c[1])
    s1 = (a[0] - c[0], a[1] - c[1])
    s2 = (b[0] + d[0], b[1] + d[1])
    s3 = (b[0] - d[0], b[1] - d[1])
    y0 = (s0[0] + s2[0], s0[1] + s2[1])
    y2 = (s0[0] - s2[0], s0[1] - s2[1])
    ya = (s1[0] + s3[1], s1[1] - s3[0])
    yb = (s1[0] - s3[1], s1[1] + s3[0])
    return [y0, ya, y2, yb] if sign < 0 else [y0, yb, y2, ya]


UNROLL = 4
NLOOP = NIT // UNROLL
NU0 = 4
NA, NB = 3, 8
BA, BB = 4, 3
N5 = 3
NTAIL = 3
PPB = 14
NPRE = 4 + NA * BA + NB * BB + N5
FSPLIT = (0, 4, 8, 13, 17, 21, 25, 30, 34, 38, 43, 48, 48)
LAG = 2
UP = 9
HP = 132
U_LAST = 32 * UP
U_PIN, U_ROWS = 296, 312
WO0 = 12 * 16 * HP
WO_ROWS = H * DH // NB
XS0 = WO0 + 4 * 2048

SEM_U0 = 0
SEM_XE = SEM_U0 + NU0
SEM_A = SEM_XE + 1
SEM_XA = SEM_A + NA
SEM_C = SEM_XA + 2
SEM_W = SEM_C + 1
SEM_F = SEM_W + NB
SEM_B = SEM_F + 1
SEM_O = SEM_B + 1
NSEM = SEM_O + 1


def _kernel(xa_hbm, wr_hbm, wi_hbm, xb_hbm, mem0_hbm, wq_hbm, wk_hbm, wv_hbm, wo_hbm,
            cm_hbm, tw_hbm, out_hbm,
            xa, ys, wr, wi, cm, tw, u_scr, yb, xb, xe, xeu,
            raw, w, wo_raw, pre, lhs_scr, tail8, om_scr, ox_scr, outb,
            wlast, t256, mem0, carry8, fill_scr, opq, sems):
    cp = pltpu.make_async_copy

    wsrc = (wq_hbm, wk_hbm, wv_hbm)

    def w_copies(p0, p1, sem):
        out = []
        while p0 < p1:
            u, c = divmod(p0, 16)
            n = min(p1 - p0, 16 - c)
            for half in range(2):
                d0 = 256 * half + 16 * c
                out.append(cp(wsrc[u // 4].at[d0:d0 + 16 * n, 8 * (u % 4):8 * (u % 4) + 8, :],
                              raw.at[16 * p0:16 * (p0 + n), 8 * half:8 * half + 8, :], sem))
            p0 += n
        return out

    pu = 16 // NU0
    c_xe = cp(xb_hbm.at[:, 24:40, :], xe, sems.at[SEM_XE])
    c_in = [c_xe]
    for k in range(NU0):
        c_in += w_copies(k * pu, (k + 1) * pu, sems.at[SEM_U0 + k])
    for g in range(NA):
        c_in += w_copies(16 * (g + 1), 16 * (g + 2), sems.at[SEM_A + g])
        if g:
            c_in.append(cp(xa_hbm.at[64 * (g - 1):64 * g], xa.at[64 * (g - 1):64 * g], sems.at[SEM_XA + g - 1]))
    c_c = [cp(cm_hbm, cm, sems.at[SEM_C]), cp(tw_hbm, tw, sems.at[SEM_C])]
    c_c += w_copies(16 * (NA + 1), 16 * (NA + 2), sems.at[SEM_C])
    c_in += c_c
    for g in range(NB):
        sem = sems.at[SEM_W + g]
        c_in += w_copies(16 * (NA + 2) + PPB * g, 16 * (NA + 2) + PPB * (g + 1), sem)
        rows = slice(g * WO_ROWS, (g + 1) * WO_ROWS)
        c_in.append(cp(wo_hbm.at[rows], wo_raw.at[rows], sem))
        rows = slice(32 * g, 32 * g + 32)
        c_in += [cp(wr_hbm.at[rows], wr.at[rows], sem), cp(wi_hbm.at[rows], wi.at[rows], sem)]
    c_f = [cp(mem0_hbm, mem0, sems.at[SEM_F]),
           cp(wr_hbm.at[256:257], wlast.at[0], sems.at[SEM_F]),
           cp(wi_hbm.at[256:257], wlast.at[1], sems.at[SEM_F])]
    c_b = [cp(xb_hbm, xb, sems.at[SEM_B])]
    for c in c_in + c_f + c_b:
        c.start()

    opq[0] = U_PIN
    ox_scr[1] = jnp.zeros((SEG, H * DH), F32)
    u_scr[:, :, U_LAST:U_LAST + 8, :] = jnp.zeros((16, 2, 8, 128), F32)
    u_scr[0, 0, U_PIN + 8:U_PIN + 16, :] = jnp.zeros((8, 128), F32)
    ys[0, 16 * HP + 8:16 * HP + 16, :] = jnp.zeros((8, 128), F32)
    xa[128] = jnp.zeros((16, D), BF16)

    row = lax.broadcasted_iota(jnp.int32, (80, 80), 0)
    col = lax.broadcasted_iota(jnp.int32, (80, 80), 1)
    rhead = jnp.where(row < 16, row // 8, (row - 16) // SEG)
    same_head = rhead == col // L
    fill_scr[...] = jnp.where(same_head, NEG / SCALE, -jnp.inf).astype(F32)

    def wait_raw(p0, n, sem):
        blk = raw.at[pl.ds(p0 * 16, n * 16)]
        cp(blk, blk, sem).wait()

    def relayout(pc, zero=None):
        eo = _tou(raw[pl.ds(pc * 16, 16)])
        if zero is not None:
            eo = eo | zero
        eo = eo.reshape(8, 2, 8, 128)
        e, o = eo[:, 0], eo[:, 1]
        h0 = (e & jnp.uint32(0xFFFF)) | (o << 16)
        h1 = (e >> 16) | (o & jnp.uint32(0xFFFF0000))
        base = (pc // 16) * (16 * HP) + (pc % 16) * 8
        for par, hh in enumerate((h0, h1)):
            for t in range(8):
                w[pl.ds(base + par * 8 * HP + t, 8, stride=HP), :] = hh[t]

    def wplane(b, par):
        r0 = ((b // 4) * 16 + par * 8 + b % 4) * HP
        return _tobf(jnp.concatenate([w[pl.ds(r0, 128), :], w[pl.ds(r0 + 4 * HP, 128), :]], axis=0))

    def retile_wo(r16):
        v = _tou(wo_raw[pl.ds(pl.multiple_of(r16 * 16, 16), 16), :])
        for j in range(4):
            w[pl.ds(WO0 + j * 2048 + r16 * 8, 8), :] = v[:, j * 128:(j + 1) * 128]

    def wo_rows(r0, n):
        return _tobf(jnp.concatenate(
            [w[WO0 + j * 2048 + r0 // 2:WO0 + j * 2048 + (r0 + n) // 2, :] for j in range(4)], axis=1))

    def stage_x(n1):
        v = _tou(xa[n1].astype(F32))
        for j in range(4):
            for half in range(2):
                w[pl.ds(XS0 + (j * 16 + half * 8) * HP + n1, 8, stride=HP), :] = (
                    v[8 * half:8 * half + 8, j * 128:(j + 1) * 128])

    def precompute(b, h, m0=0, nm=NIT, zero=None):
        u = xeu[m0 * 8:(m0 + nm) * 8, :]
        if zero is not None:
            top = jnp.concatenate([u[0:8, 0:128] | zero, u[0:8, 128:D]], axis=1)
            u = jnp.concatenate([top, u[8:]], axis=0)
        r = _nn(_tobf(u), wplane(b, h))
        pre[b, m0 * 16:(m0 + nm) * 16, h * 128:(h + 1) * 128] = r
        return r

    def half_dot(b0, t, zero=None):
        return precompute(b0 + t // 4, (t // 2) % 2, (t % 2) * 16, 16, zero)

    def mat(k):
        return _tobf(cm[64 * k:64 * k + 64, :])

    def lo_half(rows):
        return lax.broadcasted_iota(jnp.int32, (rows, 128), 1) < 64

    first = lax.broadcasted_iota(jnp.int32, (8, 128), 0) == 0
    classes = tuple(tuple((r, 32, UP) for r in cl) for cl in ((0, 4), (2, 6), (1, 7), (5, 3)))

    def part(u, h, rows=16):
        return jnp.concatenate([u[(2 * g + h) * rows:(2 * g + h + 1) * rows] for g in range(4)], axis=0)

    def f1_s(n2, x12, kk):
        h, k = kk % 2, kk // 2
        u = _nn(x12[h][k], mat(4 + h))
        r = 0
        for cl in classes[2 * k:2 * k + 2]:
            for (st, n, sd) in cl:
                u_scr[n2, h, pl.ds(st, n, stride=sd), :] = u[r:r + n]
                r += n

    def f1_d(n2, prev):
        def ldx(j):
            r0 = XS0 + (j * 16 + n2) * HP
            u = jnp.concatenate([w[pl.ds(r0 + par, 64, stride=2), :] for par in range(2)], axis=0)
            return pltpu.bitcast(u, F32)

        x0, x1, x2, x3 = [ldx(j) for j in range(4)]
        lo = lo_half(128)
        p, q, b, c = x0 + x2, x1 + x3, x0 - x2, x1 - x3
        r = _swap(jnp.where(lo, c, (b - c) * R2))
        y = jnp.where(lo, b, (b + c) * R2)
        t = []
        for k, a in enumerate((p + q, p - q, y + r, y - r)):
            t.append(_nt(mat(k), a.astype(BF16)))
            if prev is not None:
                f1_s(n2 - LAG, prev, k)
        t256[n2:n2 + 1, :] = t[0][16:17]
        t[0] = jnp.concatenate([t[0][0:16], jnp.where(first, 0.0, t[0][16:24]), t[0][24:128]], axis=0)
        tr = jnp.concatenate([part(u, 0) for u in t], axis=0)
        ti = jnp.concatenate([part(u, 1) for u in t], axis=0)
        lo = lo_half(256)
        rb = _swap(jnp.where(lo, ti, tr))
        x12 = (jnp.where(lo, tr, rb), jnp.where(lo, rb, ti))
        return [[x[128 * k:128 * k + 128].astype(BF16) for k in range(2)] for x in x12]

    def f1_all():
        p0 = 16 * (NA + 1)
        zvec = _tou(ys[0, 16 * HP + 8:16 * HP + 16, :])
        xq = [None] * LAG
        for n2 in range(16 + LAG):
            if n2 % 2 == 0 and n2 < 16:
                r = half_dot(2 + NA * BA, n2 // 2)
                relayout(p0 + n2, _tou(r[0:8]) & zvec)
                relayout(p0 + n2 + 1, _tou(r[96:104]) & zvec)
            if n2 < 16:
                xq.append(f1_d(n2, xq.pop(0)))
            else:
                xp = xq.pop(0)
                for kk in range(4):
                    f1_s(n2 - LAG, xp, kk)
        t = t256[...]
        lo = lo_half(16)
        for h, v in enumerate((t, _swap(t))):
            u = _nn(jnp.where(lo, v, 0.0).astype(BF16), mat(4 + h))
            for n2 in range(16):
                u_scr[n2, h, U_LAST:U_LAST + 1, :] = u[n2:n2 + 1]

    tok = [None]

    def f2_pieces(ru, filt):
        def ld(n):
            z = [u_scr[n, h, pl.ds(ru, 8), :] for h in range(2)]
            if tok[0] is not None:
                z = [pltpu.bitcast(_tou(v) | tok[0], F32) for v in z]
            return tuple(z)

        lo = lo_half(8)

        def st(n, z):
            u_scr[n, 0, pl.ds(ru, 8), :] = z[0]
            u_scr[n, 1, pl.ds(ru, 8), :] = z[1]

        def ld_in(n):
            e, o = ld(n)
            p, q = e + o, e - o
            r = _swap(jnp.where(lo, q, p))
            re, im = jnp.where(lo, p, r), jnp.where(lo, r, q)
            if n == 0:
                return re, im
            c, s = tw[n:n + 1, :], tw[16 + n:17 + n, :]
            return re * c + im * s, im * c - re * s

        def st_out(n, z):
            re, im = z
            if n:
                c, s = tw[n:n + 1, :], tw[16 + n:17 + n, :]
                re, im = re * c - im * s, im * c + re * s
            a = jnp.where(lo, re, im)
            r = _swap(jnp.where(lo, im, re))
            st(n, (a + r, a - r))

        def outer(b, sign):
            y = _dft4(*[(ld_in if sign < 0 else ld)(4 * a + b) for a in range(4)], sign)
            for a in range(4):
                (st if sign < 0 else st_out)(4 * a + b, y[a])

        def inner(p):
            x = _dft4(*[_cmul_const(ld(4 * p + b), b * p, 16, -1) for b in range(4)], -1)
            y = []
            for q in range(4):
                lanes = slice((p + 4 * q) * 128, (p + 4 * q + 1) * 128)
                a, b = filt(lanes)
                y.append((x[q][0] * a - x[q][1] * b, x[q][0] * b + x[q][1] * a))
            v = _dft4(*y, +1)
            for b in range(4):
                st(4 * p + b, _cmul_const(v[b], b * p, 16, +1))

        return ([functools.partial(outer, b, -1) for b in range(4)],
                [functools.partial(inner, p) for p in range(4)],
                [functools.partial(outer, b, +1) for b in range(4)])

    def f3_s(n2, zero=None):
        lo = lo_half(128)
        zs = []
        for par in range(2):
            cls = [jnp.concatenate([u_scr[n2, par, pl.ds(st, n, stride=sd), :] for (st, n, sd) in cl], axis=0)
                   for cl in classes]
            hmu = cm[64 * (6 + par):64 * (7 + par), :]
            last = _swap(u_scr[n2, par, U_LAST:U_LAST + 8, :]) * jnp.where(lo_half(8), 2.0 * par - 1.0, 1.0 - 2.0 * par)
            if zero is not None and par == 1:
                last = last + zero
            rhs_a = jnp.concatenate([cls[0], cls[1]], axis=0).astype(BF16)
            rhs_b = jnp.concatenate([jnp.where(first, last, cls[0][0:8]), cls[0][8:64], cls[1]],
                                    axis=0).astype(BF16)
            zo = _nt(_tobf(hmu), jnp.concatenate([cls[2], cls[3]], axis=0).astype(BF16))
            zs.append((_nt(_tobf(part(hmu, 0, 8)), rhs_a), _nt(_tobf(part(hmu, 1, 8)), rhs_b),
                       part(zo, 0), part(zo, 1)))
        out = []
        for k in range(2):
            re = jnp.concatenate([zs[0][2 * k], zs[1][2 * k]], axis=0)
            im = jnp.concatenate([zs[0][2 * k + 1], zs[1][2 * k + 1]], axis=0)
            r = _swap(jnp.where(lo, im, re))
            out += [jnp.where(lo, re, r).astype(BF16), jnp.where(lo, r, im).astype(BF16)]
        return out

    def f3_d(n2, z):
        b0, b2, g1, g5 = [_nn(z[k], mat(8 + k)) for k in range(4)]
        lo = lo_half(128)
        y = g1 + g5
        r = _swap(g1 - g5)
        b = jnp.where(lo, y, (y + r) * R2)
        c = jnp.where(lo, r, (y - r) * R2)
        p, q = b0 + b2, b0 - b2
        for j, v in enumerate((p + b, q + c, p - b, q - c)):
            for par in range(2):
                ys[j, pl.ds(n2 * HP + par, 64, stride=2), :] = v[64 * par:64 * par + 64]

    def gather_y(n1, half):
        v = [ys[j, pl.ds(half * 8 * HP + n1, 8, stride=HP), :] for j in range(4)]
        yb[n1, half * 8:half * 8 + 8, :] = jnp.concatenate(v, axis=1).astype(BF16)

    def f3_all():
        prow = pl.multiple_of(opq[0] + (16 * HP - U_PIN), 8)
        b0 = NPRE - N5
        nin = 4 * N5 - NTAIL - 2
        wl = [wlast[k].astype(F32) for k in range(2)]
        for stage in f2_pieces(U_LAST, lambda lanes: [jnp.broadcast_to(v[:, lanes], (8, 128)) for v in wl]):
            for pc in stage:
                pc()
        half_dot(b0, 0)
        half_dot(b0, 1)
        zq = [f3_s(0), f3_s(1)]
        zero = None
        for n2 in range(16):
            for t in range(n2 * nin // 16, (n2 + 1) * nin // 16):
                half_dot(b0, 2 + t)
            if n2 + 2 < 16:
                zq.append(f3_s(n2 + 2, zero))
            zero = ys[0, pl.ds(prow + 8, 8), :]
            f3_d(n2, zq.pop(0))
            if n2 >= 8:
                ys[0, pl.ds(prow, 8), :] = zero
                for n1 in range((n2 - 8) * 16, (n2 - 7) * 16):
                    gather_y(n1, 0)
        npin = 8 * NTAIL
        for k in range(NTAIL):
            r = half_dot(b0, 2 + nin + k)
            for j in range(8):
                ys[0, pl.ds(prow, 8), :] = r[32 * j:32 * j + 8]
                for n1 in range((8 * k + j) * 128 // npin, (8 * k + j + 1) * 128 // npin):
                    gather_y(n1, 1)

    def unit0(k, _):
        wait_raw(k * pu, pu, sems.at[SEM_U0 + k])
        for t in range(pu):
            relayout(k * pu + t)
        return 0

    c_xe.wait()
    xeu[...] = _tou(xe[...].reshape(NIT * 16, D))
    lax.fori_loop(0, NU0, unit0, 0)
    for t in range(4):
        precompute(t // 2, t % 2)

    def body_a(g, _):
        p0 = 16 * (g + 1)
        wait_raw(p0, 16, sems.at[SEM_A + g])

        @pl.when(g > 0)
        def _():
            gm = jnp.maximum(g - 1, 0)
            blk = xa.at[pl.ds(64 * gm, 64)]
            cp(blk, blk, sems.at[SEM_XA + gm]).wait()

        for t in range(4 * BA):
            half_dot(2 + BA * g, t)
            if t < 8:
                relayout(p0 + 2 * t)
                relayout(p0 + 2 * t + 1)
            for k in range(2 * t if t < 8 else 6 * t - 32, 2 * t + 2 if t < 8 else 6 * t - 26):
                stage_x(jnp.where(g > 0, 64 * (g - 1) + k, 128))
        return 0

    lax.fori_loop(0, NA, body_a, 0)
    for c in c_c:
        c.wait()
    f1_all()

    def body_b(g, _):
        p0 = 16 * (NA + 2) + PPB * g
        sem = sems.at[SEM_W + g]
        wait_raw(p0, PPB, sem)
        r32 = pl.multiple_of(g * 32, 32)
        for blk in (wo_raw.at[pl.ds(pl.multiple_of(g * WO_ROWS, WO_ROWS), WO_ROWS)],
                    wr.at[pl.ds(r32, 32)], wi.at[pl.ds(r32, 32)]):
            cp(blk, blk, sem).wait()
        pin_row = pl.multiple_of(opq[0], 8)
        groups = [f2_pieces(g * (4 * UP) + UP * k, lambda lanes, k=k: (wr[pl.ds(r32 + 8 * k, 8), lanes].astype(F32),
                                                             wi[pl.ds(r32 + 8 * k, 8), lanes].astype(F32)))
                  for k in range(4)]
        pieces = [pc for st in range(3) for k in range(4) for pc in groups[k][st]]
        nd = 4 * BB
        zeros = [None, None]
        zvec = _tou(ys[0, 16 * HP + 8:16 * HP + 16, :])
        for t in range(nd):
            v = half_dot(4 + NA * BA + BB * g, t, zeros.pop(0))
            for k in range(-(-PPB * t // nd), -(-PPB * (t + 1) // nd)):
                relayout(p0 + k)
            for k in range(32 * t // nd, 32 * (t + 1) // nd):
                retile_wo(g * (WO_ROWS // 16) + k)
            todo = pieces[FSPLIT[t]:FSPLIT[t + 1]]
            for k, pc in enumerate(todo):
                r0 = 8 * ((32 * k) // len(todo))
                tok[0] = _tou(v[r0:r0 + 8]) & zvec
                pc()
            tok[0] = None
            zeros.append(_tou(u_scr[0, 0, pl.ds(pin_row + 8, 8), :]) if todo else None)
        return 0

    lax.fori_loop(0, NB, body_b, 0)
    for c in c_f:
        c.wait()
    f3_all()
    c_oa = cp(yb, out_hbm.at[:, :, 0:D], sems.at[SEM_O])
    c_oa.start()
    for c in c_b:
        c.wait()

    rpos = jnp.where(row < 16, L, (row - 16) % SEG + M)
    mask = same_head & (rpos >= col % L)

    def qkv(st, i, lhs, lhs_v, p, even):
        r16 = pl.multiple_of(i * 16, 16)

        def proj(blk):
            wb = jnp.concatenate([wplane(blk, 0), wplane(blk, 1)], axis=1)
            if blk < NPRE:
                r = _nn(lhs, wb)
                if even:
                    return r[0:8], jnp.concatenate([r[8:32], pre[blk, pl.ds(r16, 8), :]], axis=0)
                return r[0:8], jnp.concatenate([pre[blk, pl.ds(r16 + 8, 8), :], r[8:32]], axis=0)
            r = _nn(lhs_v, wb)
            if even:
                carry8[blk - NPRE] = r[40:48]
                return r[0:8], r[8:40]
            return r[0:8], jnp.concatenate([carry8[blk - NPRE], r[8:32]], axis=0)

        mq, xq = proj(p)
        mk, xk = proj(NP + p)
        mv, xv = proj(2 * NP + p)
        h0 = lambda a: a[:, 0:128]
        h1 = lambda a: a[:, 128:256]
        st["q"][p] = jnp.concatenate([h0(mq), h1(mq), h0(xq), h1(xq)], axis=0).astype(BF16)
        st["k"][p] = jnp.concatenate([h0(mk), h0(xk), h1(mk), h1(xk)], axis=0).astype(BF16)
        st["v"][p] = jnp.concatenate([h0(mv), h0(xv), h1(mv), h1(xv)], axis=0).astype(BF16)

    def qk_group(st, g):
        for p in range(4 * g, 4 * g + 4):
            s = _nt(st["q"][p], st["k"][p])
            s = jnp.where(mask, s, fill_scr[...])
            m = jnp.max(s, axis=-1, keepdims=True)
            e = jnp.exp2((s - m) * (SCALE * LOG2E))
            l = jnp.sum(e, axis=-1, keepdims=True)
            st["p"][p] = e * pl.reciprocal(l, approx=True)

    def put_om(p, o):
        om_scr[:, (2 * p) * 128:(2 * p + 1) * 128] = o[0:8]
        om_scr[:, (2 * p + 1) * 128:(2 * p + 2) * 128] = o[8:16]

    def put_ox(b, p, o):
        ox_scr[b, :, (2 * p) * 128:(2 * p + 1) * 128] = o[0:32]
        ox_scr[b, :, (2 * p + 1) * 128:(2 * p + 2) * 128] = o[32:64]

    def pvm_group(st, g, b):
        for p in range(4 * g, 4 * g + 4):
            put_om(p, _nn(st["p"][p][0:16].astype(BF16), st["v"][p]))

    def pvx_group(st, g, b):
        for p in range(4 * g, 4 * g + 4):
            put_ox(b, p, _nn(st["p"][p][16:80].astype(BF16), st["v"][p]))

    def pv_group(st, g, b):
        for p in range(4 * g, 4 * g + 4):
            o = _nn(st["p"][p].astype(BF16), st["v"][p])
            put_om(p, o[0:16])
            put_ox(b, p, o[16:80])

    def oproj(c, even, acc):
        cs = slice(c * 512, (c + 1) * 512)
        if even:
            lhs = jnp.concatenate([om_scr[:, cs], ox_scr[1, 0:24, cs]], axis=0)
            tail8[:, cs] = ox_scr[1, 24:32, cs]
        else:
            lhs = jnp.concatenate([om_scr[:, cs], tail8[:, cs], ox_scr[0, :, cs]], axis=0)
        r = _nn(lhs.astype(BF16), wo_rows(c * 512, 512))
        return r if acc is None else r + acc

    def step(i, lhs_v, even, late):
        b = 0 if even else 1
        st = dict(q={}, k={}, v={}, p={})
        lhs = lhs_v[0:32]
        pv = pvm_group if late else pv_group
        for p in range(4):
            qkv(st, i, lhs, lhs_v, p, even)
        for g in range(3):
            qkv(st, i, lhs, lhs_v, 4 * g + 4, even)
            qk_group(st, g)
            for p in range(4 * g + 5, 4 * g + 8):
                qkv(st, i, lhs, lhs_v, p, even)
            pv(st, g, b)
        acc = oproj(0, even, None)
        qk_group(st, 3)
        for c in range(1, 4):
            acc = oproj(c, even, acc)
        pv(st, 3, b)
        for c in range(4, 8):
            acc = oproj(c, even, acc)
        if late:
            for g in range(4):
                pvx_group(st, g, b)
        return acc

    nb = 4 * (NIT - UNROLL)
    ob = lambda g0, g1: cp(outb.at[g0:g1], out_hbm.at[g0 - 2:g1 - 2, :, D:2 * D], sems.at[SEM_O])
    c_out = [c_oa, ob(2, nb), ob(nb, 4 * NIT), ob(4 * NIT, 4 * NIT + 2)]

    def even_lhs(i, mem):
        return jnp.concatenate([mem, xb[i, 0:40, :].astype(F32)], axis=0).astype(BF16)

    def pair(i, lhs, last):
        acc = step(i, lhs, True, True)
        outb[4 * i] = acc[8:24].astype(BF16)
        stash = acc[24:32]
        xf = xb[i, 40:64, :].astype(F32)
        acc = step(i, jnp.concatenate([acc[0:8], xf], axis=0).astype(BF16), False, not last)
        o48 = jnp.concatenate([stash, acc[8:48]], axis=0)
        outb[pl.ds(4 * i + 1, 3)] = o48.reshape(3, 16, D).astype(BF16)
        return even_lhs(jnp.minimum(i + 1, NIT - 1), acc[0:8])

    def body(it, _):
        @pl.when(it == NLOOP - 1)
        def _():
            c_out[1].start()

        lhs = _tobf(lhs_scr[...])
        for u in range(UNROLL):
            lhs = pair(it * UNROLL + u, lhs, u == UNROLL - 1)
        lhs_scr[...] = _tou(lhs)
        return 0

    lhs_scr[...] = _tou(even_lhs(0, mem0[...].astype(F32)))
    lax.fori_loop(0, NLOOP, body, 0)

    c_out[2].start()
    acc = _nn(ox_scr[1].astype(BF16), wo_rows(0, H * DH))
    outb[4 * NIT:4 * NIT + 2] = acc.reshape(2, 16, D).astype(BF16)
    c_out[3].start()
    for c in c_out:
        c.wait()


@jax.jit
def pallas_concat_heads__spectral_gfnet__memory_aug_recurrent_mem_tr__prompt_kernel(
    A_x, A_w_r, A_w_i, B_x, B_mem0, B_Wq, B_Wk, B_Wv, B_Wo, B_seg_len,
):
    del B_seg_len
    assert A_x.shape == (1, S, D) and B_x.shape == (1, S, D) and B_mem0.shape == (1, M, D)
    cm, tw = _fft_consts()
    hbm = pl.BlockSpec(memory_space=pltpu.HBM)
    out = pl.pallas_call(
        _kernel,
        out_shape=jax.ShapeDtypeStruct((S // 16, 16, 2 * D), BF16),
        in_specs=[hbm] * 11,
        out_specs=hbm,
        scratch_shapes=[
            pltpu.VMEM((129, 16, D), BF16),
            pltpu.VMEM((4, 16 * HP + 128, 128), F32),
            pltpu.VMEM((256, S), BF16),
            pltpu.VMEM((256, S), BF16),
            pltpu.VMEM((12 * 64, 128), U32),
            pltpu.VMEM((32, 128), F32),
            pltpu.VMEM((16, 2, U_ROWS, 128), F32),
            pltpu.VMEM((128, 16, D), BF16),
            pltpu.VMEM((NIT, 2 * SEG, D), BF16),
            pltpu.VMEM((NIT, 16, D), BF16),
            pltpu.VMEM((NIT * 8, D), U32),
            pltpu.VMEM((6 * D, 16, 128), BF16),
            pltpu.VMEM((XS0 + 64 * HP + 160, 128), U32),
            pltpu.VMEM((H * DH, D), BF16),
            pltpu.VMEM((NPRE, NIT * 16, 256), F32),
            pltpu.VMEM((24, D), U32),
            pltpu.VMEM((8, H * DH), F32),
            pltpu.VMEM((M, H * DH), F32),
            pltpu.VMEM((2, SEG, H * DH), F32),
            pltpu.VMEM((4 * NIT + 2, 16, D), BF16),
            pltpu.VMEM((2, 1, S), BF16),
            pltpu.VMEM((16, 128), F32),
            pltpu.VMEM((M, D), BF16),
            pltpu.VMEM((3 * NP - NPRE, 8, 256), F32),
            pltpu.VMEM((80, 80), F32),
            pltpu.SMEM((1,), jnp.int32),
            pltpu.SemaphoreType.DMA((NSEM,)),
        ],
        compiler_params=pltpu.CompilerParams(vmem_limit_bytes=110 * 1024 * 1024),
    )(
        A_x.reshape(S // 16, 16, D), A_w_r.T, A_w_i.T,
        B_x.reshape(NIT, 2 * SEG, D), B_mem0.reshape(M, D),
        B_Wq, B_Wk, B_Wv, B_Wo.reshape(H * DH, D),
        jnp.asarray(cm), jnp.asarray(tw),
    )
    return out.reshape(1, S, 2 * D)
```

```python
import functools

import numpy as np
import jax
import jax.numpy as jnp
from jax import lax
import jax.experimental.pallas as pl
import jax.experimental.pallas.tpu as pltpu

F32 = jnp.float32
BF16 = jnp.bfloat16
U32 = jnp.uint32

S, D = 2048, 512
H, DH = 32, 128
M, SEG = 8, 32
L = M + SEG
NP = H // 2
NIT = S // (2 * SEG)
SCALE = DH ** -0.5
LOG2E = 1.4426950408889634
NEG = -1000000000.0
R2 = float(np.sqrt(0.5))


def _nt(a, b):
    return lax.dot_general(a, b, (((1,), (1,)), ((), ())), preferred_element_type=F32)


def _nn(a, b):
    return jnp.dot(a, b, preferred_element_type=F32)


def _tobf(u):
    return pltpu.bitcast(u, BF16)


def _tou(b):
    return pltpu.bitcast(b, U32)


def _swap(a):
    return pltpu.roll(a, 64, a.ndim - 1)


def _cs(num, den):
    ang = 2.0 * np.pi * np.mod(num, den) / den
    c, s = np.cos(ang), np.sin(ang)
    c[np.abs(c) < 1e-12] = 0.0
    s[np.abs(s) < 1e-12] = 0.0
    return c, s


def _pack_rows(a):
    b = np.asarray(a, np.float32).astype(jnp.bfloat16).view(np.uint16).astype(np.uint32)
    return b[0::2] | (b[1::2] << 16)


def _fft_consts():
    d1, e64, j32 = np.arange(128), np.arange(64), np.arange(32)
    f0 = np.concatenate([8 * j32, 8 * j32 + 4])
    f2 = np.concatenate([8 * j32 + 2, 8 * j32 + 6])
    fa = np.concatenate([8 * j32 + 1, 8 * j32 + 7])
    fb = np.concatenate([8 * j32 + 5, 8 * j32 + 3])
    c, s = _cs(np.outer(f0, d1), D)
    l0 = np.concatenate([c, -s], 0)
    l0[64] = 1.0 - 2.0 * (d1 % 2)
    c, s = _cs(np.outer(f2, d1), D)
    l2 = np.concatenate([c, -s], 0)

    def odd(f, imsign):
        c, s = _cs(np.outer(f, e64), D)
        sg = np.where(f % 4 == 1, imsign, -imsign)[:, None]
        return np.block([[c, sg * s], [-s, sg * c]])

    la, lb = odd(fa, -1.0), odd(fb, 1.0)
    g, hm = [], []
    for par in range(2):
        c, s = _cs(np.outer(2 * e64 + par, e64), 128)
        sg = 1.0 - 2.0 * par
        g.append(np.block([[c, -s], [s, c]]))
        hm.append(np.block([[c, -sg * s], [s, sg * c]]))
    sc = 2.0 / (S * D)
    i0 = sc * l0
    i0[0] *= 0.5
    i0[64] *= 0.5
    il = lambda a: a.reshape(2, 4, 16, 128).transpose(1, 0, 2, 3).reshape(128, 128)
    mats = [il(l0), il(l2), il(la), il(lb), g[0], g[1], il(hm[0]), il(hm[1]), i0, sc * l2, sc * la, sc * lb]
    tc, ts = _cs(np.outer(np.arange(16), d1), S)
    return _pack_rows(np.concatenate(mats, 0)), np.concatenate([tc, ts], 0).astype(np.float32)


def _cmul_const(z, k, n, sign):
    re, im = z
    k = k % n
    if k == 0:
        return z
    if 4 * k == n:
        return (-im, re) if sign > 0 else (im, -re)
    c = float(np.cos(2 * np.pi * k / n))
    s = float(sign * np.sin(2 * np.pi * k / n))
    if (8 * k) % n == 0:
        a, b = re * c, im * c
        return (a - b, b + a) if s / c > 0 else (a + b, b - a)
    return (re * c - im * s, re * s + im * c)


def _dft4(a, b, c, d, sign):
    s0 = (a[0] + c[0], a[1] + c[1])
    s1 = (a[0] - c[0], a[1] - c[1])
    s2 = (b[0] + d[0], b[1] + d[1])
    s3 = (b[0] - d[0], b[1] - d[1])
    y0 = (s0[0] + s2[0], s0[1] + s2[1])
    y2 = (s0[0] - s2[0], s0[1] - s2[1])
    ya = (s1[0] + s3[1], s1[1] - s3[0])
    yb = (s1[0] - s3[1], s1[1] + s3[0])
    return [y0, ya, y2, yb] if sign < 0 else [y0, yb, y2, ya]


UNROLL = 4
NLOOP = NIT // UNROLL
NU0 = 4
NA, NB = 3, 8
BA, BB = 4, 3
N5 = 3
NTAIL = 3
PPB = 14
NPRE = 4 + NA * BA + NB * BB + N5
FSPLIT = (0, 4, 8, 13, 17, 21, 25, 30, 34, 38, 43, 48, 48)
LAG = 2
UP = 9
HP = 132
U_LAST = 32 * UP
U_PIN, U_ROWS = 296, 312
WO0 = 12 * 16 * HP
WO_ROWS = H * DH // NB
XS0 = WO0 + 4 * 2048

SEM_U0 = 0
SEM_XE = SEM_U0 + NU0
SEM_A = SEM_XE + 1
SEM_XA = SEM_A + NA
SEM_C = SEM_XA + 2
SEM_W = SEM_C + 1
SEM_F = SEM_W + NB
NSEM = SEM_F + 1


def _body(sems, osem, xa_hbm, wr_hbm, wi_hbm, xb_hbm, mem0_hbm, wq_hbm, wk_hbm, wv_hbm, wo_hbm,
          cm_hbm, tw_hbm, out_hbm,
          xa, ys, wr, wi, cm, tw, u_scr, yb, xb, xe, xeu,
          raw, w, wo_raw, pre, lhs_scr, tail8, om_scr, ox_scr, outb,
          wlast, t256, mem0, carry8, fill_scr, opq):
    cp = pltpu.make_async_copy

    wsrc = (wq_hbm, wk_hbm, wv_hbm)

    def w_copies(p0, p1, sem):
        out = []
        while p0 < p1:
            u, c = divmod(p0, 16)
            n = min(p1 - p0, 16 - c)
            for half in range(2):
                d0 = 256 * half + 16 * c
                out.append(cp(wsrc[u // 4].at[d0:d0 + 16 * n, 8 * (u % 4):8 * (u % 4) + 8, :],
                              raw.at[16 * p0:16 * (p0 + n), 8 * half:8 * half + 8, :], sem))
            p0 += n
        return out

    pu = 16 // NU0
    c_xe = cp(xb_hbm.at[:, 24:40, :], xe, sems.at[SEM_XE])
    c_in = [c_xe]
    for k in range(NU0):
        c_in += w_copies(k * pu, (k + 1) * pu, sems.at[SEM_U0 + k])
    for g in range(NA):
        c_in += w_copies(16 * (g + 1), 16 * (g + 2), sems.at[SEM_A + g])
        if g:
            c_in.append(cp(xa_hbm.at[64 * (g - 1):64 * g], xa.at[64 * (g - 1):64 * g], sems.at[SEM_XA + g - 1]))
    c_c = [cp(cm_hbm, cm, sems.at[SEM_C]), cp(tw_hbm, tw, sems.at[SEM_C])]
    c_c += w_copies(16 * (NA + 1), 16 * (NA + 2), sems.at[SEM_C])
    c_in += c_c
    for g in range(NB):
        sem = sems.at[SEM_W + g]
        c_in += w_copies(16 * (NA + 2) + PPB * g, 16 * (NA + 2) + PPB * (g + 1), sem)
        rows = slice(g * WO_ROWS, (g + 1) * WO_ROWS)
        c_in.append(cp(wo_hbm.at[rows], wo_raw.at[rows], sem))
        rows = slice(32 * g, 32 * g + 32)
        c_in += [cp(wr_hbm.at[rows], wr.at[rows], sem), cp(wi_hbm.at[rows], wi.at[rows], sem)]
    c_f = [cp(mem0_hbm, mem0, sems.at[SEM_F]),
           cp(wr_hbm.at[256:257], wlast.at[0], sems.at[SEM_F]),
           cp(wi_hbm.at[256:257], wlast.at[1], sems.at[SEM_F]),
           cp(xb_hbm, xb, sems.at[SEM_F])]
    for c in c_in + c_f:
        c.start()

    opq[0] = U_PIN
    ox_scr[1] = jnp.zeros((SEG, H * DH), F32)
    u_scr[:, :, U_LAST:U_LAST + 8, :] = jnp.zeros((16, 2, 8, 128), F32)
    u_scr[0, 0, U_PIN + 8:U_PIN + 16, :] = jnp.zeros((8, 128), F32)
    ys[0, 16 * HP + 8:16 * HP + 16, :] = jnp.zeros((8, 128), F32)
    xa[128] = jnp.zeros((16, D), BF16)

    row = lax.broadcasted_iota(jnp.int32, (80, 80), 0)
    col = lax.broadcasted_iota(jnp.int32, (80, 80), 1)
    rhead = jnp.where(row < 16, row // 8, (row - 16) // SEG)
    same_head = rhead == col // L
    fill_scr[...] = jnp.where(same_head, NEG / SCALE, -jnp.inf).astype(F32)

    def wait_raw(p0, n, sem):
        blk = raw.at[pl.ds(p0 * 16, n * 16)]
        cp(blk, blk, sem).wait()

    def relayout(pc, zero=None):
        eo = _tou(raw[pl.ds(pc * 16, 16)])
        if zero is not None:
            eo = eo | zero
        eo = eo.reshape(8, 2, 8, 128)
        e, o = eo[:, 0], eo[:, 1]
        h0 = (e & jnp.uint32(0xFFFF)) | (o << 16)
        h1 = (e >> 16) | (o & jnp.uint32(0xFFFF0000))
        base = (pc // 16) * (16 * HP) + (pc % 16) * 8
        for par, hh in enumerate((h0, h1)):
            for t in range(8):
                w[pl.ds(base + par * 8 * HP + t, 8, stride=HP), :] = hh[t]

    def wplane(b, par):
        r0 = ((b // 4) * 16 + par * 8 + b % 4) * HP
        return _tobf(jnp.concatenate([w[pl.ds(r0, 128), :], w[pl.ds(r0 + 4 * HP, 128), :]], axis=0))

    def retile_wo(r16):
        v = _tou(wo_raw[pl.ds(pl.multiple_of(r16 * 16, 16), 16), :])
        for j in range(4):
            w[pl.ds(WO0 + j * 2048 + r16 * 8, 8), :] = v[:, j * 128:(j + 1) * 128]

    def wo_rows(r0, n):
        return _tobf(jnp.concatenate(
            [w[WO0 + j * 2048 + r0 // 2:WO0 + j * 2048 + (r0 + n) // 2, :] for j in range(4)], axis=1))

    def stage_x(n1):
        v = _tou(xa[n1].astype(F32))
        for j in range(4):
            for half in range(2):
                w[pl.ds(XS0 + (j * 16 + half * 8) * HP + n1, 8, stride=HP), :] = (
                    v[8 * half:8 * half + 8, j * 128:(j + 1) * 128])

    def precompute(b, h, m0=0, nm=NIT, zero=None):
        u = xeu[m0 * 8:(m0 + nm) * 8, :]
        if zero is not None:
            top = jnp.concatenate([u[0:8, 0:128] | zero, u[0:8, 128:D]], axis=1)
            u = jnp.concatenate([top, u[8:]], axis=0)
        r = _nn(_tobf(u), wplane(b, h))
        pre[b, m0 * 16:(m0 + nm) * 16, h * 128:(h + 1) * 128] = r
        return r

    def half_dot(b0, t, zero=None):
        return precompute(b0 + t // 4, (t // 2) % 2, (t % 2) * 16, 16, zero)

    def mat(k):
        return _tobf(cm[64 * k:64 * k + 64, :])

    def lo_half(rows):
        return lax.broadcasted_iota(jnp.int32, (rows, 128), 1) < 64

    first = lax.broadcasted_iota(jnp.int32, (8, 128), 0) == 0
    classes = tuple(tuple((r, 32, UP) for r in cl) for cl in ((0, 4), (2, 6), (1, 7), (5, 3)))

    def part(u, h, rows=16):
        return jnp.concatenate([u[(2 * g + h) * rows:(2 * g + h + 1) * rows] for g in range(4)], axis=0)

    def f1_s(n2, x12, kk):
        h, k = kk % 2, kk // 2
        u = _nn(x12[h][k], mat(4 + h))
        r = 0
        for cl in classes[2 * k:2 * k + 2]:
            for (st, n, sd) in cl:
                u_scr[n2, h, pl.ds(st, n, stride=sd), :] = u[r:r + n]
                r += n

    def f1_d(n2, prev):
        def ldx(j):
            r0 = XS0 + (j * 16 + n2) * HP
            u = jnp.concatenate([w[pl.ds(r0 + par, 64, stride=2), :] for par in range(2)], axis=0)
            return pltpu.bitcast(u, F32)

        x0, x1, x2, x3 = [ldx(j) for j in range(4)]
        lo = lo_half(128)
        p, q, b, c = x0 + x2, x1 + x3, x0 - x2, x1 - x3
        r = _swap(jnp.where(lo, c, (b - c) * R2))
        y = jnp.where(lo, b, (b + c) * R2)
        t = []
        for k, a in enumerate((p + q, p - q, y + r, y - r)):
            t.append(_nt(mat(k), a.astype(BF16)))
            if prev is not None:
                f1_s(n2 - LAG, prev, k)
        t256[n2:n2 + 1, :] = t[0][16:17]
        t[0] = jnp.concatenate([t[0][0:16], jnp.where(first, 0.0, t[0][16:24]), t[0][24:128]], axis=0)
        tr = jnp.concatenate([part(u, 0) for u in t], axis=0)
        ti = jnp.concatenate([part(u, 1) for u in t], axis=0)
        lo = lo_half(256)
        rb = _swap(jnp.where(lo, ti, tr))
        x12 = (jnp.where(lo, tr, rb), jnp.where(lo, rb, ti))
        return [[x[128 * k:128 * k + 128].astype(BF16) for k in range(2)] for x in x12]

    def f1_all():
        p0 = 16 * (NA + 1)
        zvec = _tou(ys[0, 16 * HP + 8:16 * HP + 16, :])
        xq = [None] * LAG
        dots = (0, 2, 4, 7, 9, 11, 14, 17)
        for n2 in range(16 + LAG):
            if n2 in dots:
                k = dots.index(n2)
                r = half_dot(2 + NA * BA, k)
                relayout(p0 + 2 * k, _tou(r[0:8]) & zvec)
                relayout(p0 + 2 * k + 1, _tou(r[96:104]) & zvec)
            if n2 < 16:
                xq.append(f1_d(n2, xq.pop(0)))
            else:
                xp = xq.pop(0)
                for kk in range(4):
                    f1_s(n2 - LAG, xp, kk)
        t = t256[...]
        lo = lo_half(16)
        for h, v in enumerate((t, _swap(t))):
            u = _nn(jnp.where(lo, v, 0.0).astype(BF16), mat(4 + h))
            for n2 in range(16):
                u_scr[n2, h, U_LAST:U_LAST + 1, :] = u[n2:n2 + 1]

    tok = [None]

    def f2_pieces(ru, filt):
        def ld(n):
            z = [u_scr[n, h, pl.ds(ru, 8), :] for h in range(2)]
            if tok[0] is not None:
                z = [pltpu.bitcast(_tou(v) | tok[0], F32) for v in z]
            return tuple(z)

        lo = lo_half(8)

        def st(n, z):
            u_scr[n, 0, pl.ds(ru, 8), :] = z[0]
            u_scr[n, 1, pl.ds(ru, 8), :] = z[1]

        def ld_in(n):
            e, o = ld(n)
            p, q = e + o, e - o
            r = _swap(jnp.where(lo, q, p))
            re, im = jnp.where(lo, p, r), jnp.where(lo, r, q)
            if n == 0:
                return re, im
            c, s = tw[n:n + 1, :], tw[16 + n:17 + n, :]
            return re * c + im * s, im * c - re * s

        def st_out(n, z):
            re, im = z
            if n:
                c, s = tw[n:n + 1, :], tw[16 + n:17 + n, :]
                re, im = re * c - im * s, im * c + re * s
            a = jnp.where(lo, re, im)
            r = _swap(jnp.where(lo, im, re))
            st(n, (a + r, a - r))

        def outer(b, sign):
            y = _dft4(*[(ld_in if sign < 0 else ld)(4 * a + b) for a in range(4)], sign)
            for a in range(4):
                (st if sign < 0 else st_out)(4 * a + b, y[a])

        def inner(p):
            x = _dft4(*[_cmul_const(ld(4 * p + b), b * p, 16, -1) for b in range(4)], -1)
            y = []
            for q in range(4):
                lanes = slice((p + 4 * q) * 128, (p + 4 * q + 1) * 128)
                a, b = filt(lanes)
                y.append((x[q][0] * a - x[q][1] * b, x[q][0] * b + x[q][1] * a))
            v = _dft4(*y, +1)
            for b in range(4):
                st(4 * p + b, _cmul_const(v[b], b * p, 16, +1))

        return ([functools.partial(outer, b, -1) for b in range(4)],
                [functools.partial(inner, p) for p in range(4)],
                [functools.partial(outer, b, +1) for b in range(4)])

    def f3_s(n2, zero=None):
        lo = lo_half(128)
        zs = []
        for par in range(2):
            cls = [jnp.concatenate([u_scr[n2, par, pl.ds(st, n, stride=sd), :] for (st, n, sd) in cl], axis=0)
                   for cl in classes]
            hmu = cm[64 * (6 + par):64 * (7 + par), :]
            sign = jnp.where(lo_half(8), 2.0 * par - 1.0, 1.0 - 2.0 * par)
            last = _swap(u_scr[n2, par, U_LAST:U_LAST + 8, :]) * sign
            if zero is not None and par == 1:
                last = last + zero
            rhs_a = jnp.concatenate([cls[0], cls[1]], axis=0).astype(BF16)
            rhs_b = jnp.concatenate([jnp.where(first, last, cls[0][0:8]), cls[0][8:64], cls[1]],
                                    axis=0).astype(BF16)
            zo = _nt(_tobf(hmu), jnp.concatenate([cls[2], cls[3]], axis=0).astype(BF16))
            zs.append((_nt(_tobf(part(hmu, 0, 8)), rhs_a), _nt(_tobf(part(hmu, 1, 8)), rhs_b),
                       part(zo, 0), part(zo, 1)))
        out = []
        for k in range(2):
            re = jnp.concatenate([zs[0][2 * k], zs[1][2 * k]], axis=0)
            im = jnp.concatenate([zs[0][2 * k + 1], zs[1][2 * k + 1]], axis=0)
            r = _swap(jnp.where(lo, im, re))
            out += [jnp.where(lo, re, r).astype(BF16), jnp.where(lo, r, im).astype(BF16)]
        return out

    def f3_d(n2, z):
        b0, b2, g1, g5 = [_nn(z[k], mat(8 + k)) for k in range(4)]
        lo = lo_half(128)
        y = g1 + g5
        r = _swap(g1 - g5)
        b = jnp.where(lo, y, (y + r) * R2)
        c = jnp.where(lo, r, (y - r) * R2)
        p, q = b0 + b2, b0 - b2
        for j, v in enumerate((p + b, q + c, p - b, q - c)):
            for par in range(2):
                ys[j, pl.ds(n2 * HP + par, 64, stride=2), :] = v[64 * par:64 * par + 64]

    def gather_y(n1, half):
        v = [ys[j, pl.ds(half * 8 * HP + n1, 8, stride=HP), :] for j in range(4)]
        yb[n1, half * 8:half * 8 + 8, :] = jnp.concatenate(v, axis=1).astype(BF16)

    def f3_all():
        prow = pl.multiple_of(opq[0] + (16 * HP - U_PIN), 8)
        b0 = NPRE - N5
        nin = 4 * N5 - NTAIL - 2
        wl = [wlast[k].astype(F32) for k in range(2)]
        stages = f2_pieces(U_LAST, lambda lanes: [jnp.broadcast_to(v[:, lanes], (8, 128)) for v in wl])
        zvec = _tou(ys[0, 16 * HP + 8:16 * HP + 16, :])
        r = half_dot(b0, 0)
        for k, pc in enumerate(stages[0] + stages[1] + stages[2]):
            tok[0] = (_tou(r[(k - 4) * 24:(k - 4) * 24 + 8]) & zvec) if k >= 4 else None
            pc()
        tok[0] = None
        half_dot(b0, 1)
        zq = [f3_s(0), f3_s(1)]
        zero = None
        for n2 in range(16):
            for t in range(n2 * nin // 16, (n2 + 1) * nin // 16):
                half_dot(b0, 2 + t)
            if n2 + 2 < 16:
                zq.append(f3_s(n2 + 2, zero))
            zero = ys[0, pl.ds(prow + 8, 8), :]
            f3_d(n2, zq.pop(0))
            if n2 >= 8:
                ys[0, pl.ds(prow, 8), :] = zero
                for n1 in range((n2 - 8) * 16, (n2 - 7) * 16):
                    gather_y(n1, 0)
        npin = 8 * NTAIL - 5
        for k in range(NTAIL):
            r = half_dot(b0, 2 + nin + k)
            for j in range(min(8, npin - 8 * k)):
                ys[0, pl.ds(prow, 8), :] = r[32 * j:32 * j + 8]
                for n1 in range((8 * k + j) * 128 // npin, (8 * k + j + 1) * 128 // npin):
                    gather_y(n1, 1)

    def unit0(k, _):
        wait_raw(k * pu, pu, sems.at[SEM_U0 + k])
        for t in range(pu):
            relayout(k * pu + t)
        return 0

    c_xe.wait()
    xeu[...] = _tou(xe[...].reshape(NIT * 16, D))
    lax.fori_loop(0, NU0, unit0, 0)
    for t in range(4):
        precompute(t // 2, t % 2)

    def body_a(g, _):
        p0 = 16 * (g + 1)
        wait_raw(p0, 16, sems.at[SEM_A + g])

        @pl.when(g > 0)
        def _():
            gm = jnp.maximum(g - 1, 0)
            blk = xa.at[pl.ds(64 * gm, 64)]
            cp(blk, blk, sems.at[SEM_XA + gm]).wait()

        for t in range(4 * BA):
            half_dot(2 + BA * g, t)
            if t < 8:
                relayout(p0 + 2 * t)
                relayout(p0 + 2 * t + 1)
            for k in range(2 * t if t < 8 else 6 * t - 32, 2 * t + 2 if t < 8 else 6 * t - 26):
                stage_x(jnp.where(g > 0, 64 * (g - 1) + k, 128))
        return 0

    lax.fori_loop(0, NA, body_a, 0)
    for c in c_c:
        c.wait()
    f1_all()

    def body_b(g, _):
        p0 = 16 * (NA + 2) + PPB * g
        sem = sems.at[SEM_W + g]
        wait_raw(p0, PPB, sem)
        r32 = pl.multiple_of(g * 32, 32)
        for blk in (wo_raw.at[pl.ds(pl.multiple_of(g * WO_ROWS, WO_ROWS), WO_ROWS)],
                    wr.at[pl.ds(r32, 32)], wi.at[pl.ds(r32, 32)]):
            cp(blk, blk, sem).wait()
        pin_row = pl.multiple_of(opq[0], 8)
        filt = lambda k, lanes: [v[pl.ds(r32 + 8 * k, 8), lanes].astype(F32) for v in (wr, wi)]
        groups = [f2_pieces(g * (4 * UP) + UP * k, functools.partial(filt, k)) for k in range(4)]
        pieces = [pc for st in range(3) for k in range(4) for pc in groups[k][st]]
        nd = 4 * BB
        zeros = [None, None]
        zvec = _tou(ys[0, 16 * HP + 8:16 * HP + 16, :])
        for t in range(nd):
            v = half_dot(4 + NA * BA + BB * g, t, zeros.pop(0))
            for k in range(-(-PPB * t // nd), -(-PPB * (t + 1) // nd)):
                relayout(p0 + k)
            for k in range(32 * t // nd, 32 * (t + 1) // nd):
                retile_wo(g * (WO_ROWS // 16) + k)
            todo = pieces[FSPLIT[t]:FSPLIT[t + 1]]
            for k, pc in enumerate(todo):
                r0 = 8 * ((32 * k) // len(todo))
                tok[0] = _tou(v[r0:r0 + 8]) & zvec
                pc()
            tok[0] = None
            zeros.append(_tou(u_scr[0, 0, pl.ds(pin_row + 8, 8), :]) if todo else None)
        return 0

    lax.fori_loop(0, NB, body_b, 0)
    for c in c_f:
        c.wait()
    f3_all()

    rpos = jnp.where(row < 16, L, (row - 16) % SEG + M)
    mask = same_head & (rpos >= col % L)

    def qkv(st, i, lhs, lhs_v, p, even):
        r16 = pl.multiple_of(i * 16, 16)

        def proj(blk):
            wb = jnp.concatenate([wplane(blk, 0), wplane(blk, 1)], axis=1)
            if blk < NPRE:
                r = _nn(lhs, wb)
                if even:
                    return r[0:8], jnp.concatenate([r[8:32], pre[blk, pl.ds(r16, 8), :]], axis=0)
                return r[0:8], jnp.concatenate([pre[blk, pl.ds(r16 + 8, 8), :], r[8:32]], axis=0)
            r = _nn(lhs_v, wb)
            if even:
                carry8[blk - NPRE] = r[40:48]
                return r[0:8], r[8:40]
            return r[0:8], jnp.concatenate([carry8[blk - NPRE], r[8:32]], axis=0)

        mq, xq = proj(p)
        mk, xk = proj(NP + p)
        mv, xv = proj(2 * NP + p)
        h0 = lambda a: a[:, 0:128]
        h1 = lambda a: a[:, 128:256]
        st["q"][p] = jnp.concatenate([h0(mq), h1(mq), h0(xq), h1(xq)], axis=0).astype(BF16)
        st["k"][p] = jnp.concatenate([h0(mk), h0(xk), h1(mk), h1(xk)], axis=0).astype(BF16)
        st["v"][p] = jnp.concatenate([h0(mv), h0(xv), h1(mv), h1(xv)], axis=0).astype(BF16)

    def qk_group(st, g):
        for p in range(4 * g, 4 * g + 4):
            s = _nt(st["q"][p], st["k"][p])
            s = jnp.where(mask, s, fill_scr[...])
            m = jnp.max(s, axis=-1, keepdims=True)
            e = jnp.exp2((s - m) * (SCALE * LOG2E))
            l = jnp.sum(e, axis=-1, keepdims=True)
            st["p"][p] = e * pl.reciprocal(l, approx=True)

    def put_om(p, o):
        om_scr[:, (2 * p) * 128:(2 * p + 1) * 128] = o[0:8]
        om_scr[:, (2 * p + 1) * 128:(2 * p + 2) * 128] = o[8:16]

    def put_ox(b, p, o):
        ox_scr[b, :, (2 * p) * 128:(2 * p + 1) * 128] = o[0:32]
        ox_scr[b, :, (2 * p + 1) * 128:(2 * p + 2) * 128] = o[32:64]

    def pvm_group(st, g, b):
        for p in range(4 * g, 4 * g + 4):
            put_om(p, _nn(st["p"][p][0:16].astype(BF16), st["v"][p]))

    def pvx_group(st, g, b):
        for p in range(4 * g, 4 * g + 4):
            put_ox(b, p, _nn(st["p"][p][16:80].astype(BF16), st["v"][p]))

    def pv_group(st, g, b):
        for p in range(4 * g, 4 * g + 4):
            o = _nn(st["p"][p].astype(BF16), st["v"][p])
            put_om(p, o[0:16])
            put_ox(b, p, o[16:80])

    def oproj(c, even, acc):
        cs = slice(c * 512, (c + 1) * 512)
        if even:
            lhs = jnp.concatenate([om_scr[:, cs], ox_scr[1, 0:24, cs]], axis=0)
            tail8[:, cs] = ox_scr[1, 24:32, cs]
        else:
            lhs = jnp.concatenate([om_scr[:, cs], tail8[:, cs], ox_scr[0, :, cs]], axis=0)
        r = _nn(lhs.astype(BF16), wo_rows(c * 512, 512))
        return r if acc is None else r + acc

    def step(i, lhs_v, even, late):
        b = 0 if even else 1
        st = dict(q={}, k={}, v={}, p={})
        lhs = lhs_v[0:32]
        pv = pvm_group if late else pv_group
        for p in range(4):
            qkv(st, i, lhs, lhs_v, p, even)
        for g in range(3):
            qkv(st, i, lhs, lhs_v, 4 * g + 4, even)
            qk_group(st, g)
            for p in range(4 * g + 5, 4 * g + 8):
                qkv(st, i, lhs, lhs_v, p, even)
            pv(st, g, b)
        acc = oproj(0, even, None)
        qk_group(st, 3)
        for c in range(1, 4):
            acc = oproj(c, even, acc)
        pv(st, 3, b)
        for c in range(4, 8):
            acc = oproj(c, even, acc)
        if late:
            for g in range(4):
                pvx_group(st, g, b)
        return acc

    nb = 4 * (NIT - UNROLL)
    ob = lambda g0, g1: cp(outb.at[g0:g1], out_hbm.at[g0 - 2:g1 - 2, :, D:2 * D], osem)
    c_out = [cp(yb, out_hbm.at[:, :, 0:D], osem), ob(2, nb), ob(nb, 4 * NIT), ob(4 * NIT, 4 * NIT + 2)]

    def even_lhs(i, mem):
        return jnp.concatenate([mem, xb[i, 0:40, :].astype(F32)], axis=0).astype(BF16)

    def pair(i, lhs, last):
        acc = step(i, lhs, True, True)
        outb[4 * i] = acc[8:24].astype(BF16)
        stash = acc[24:32]
        xf = xb[i, 40:64, :].astype(F32)
        acc = step(i, jnp.concatenate([acc[0:8], xf], axis=0).astype(BF16), False, not last)
        o48 = jnp.concatenate([stash, acc[8:48]], axis=0)
        outb[pl.ds(4 * i + 1, 3)] = o48.reshape(3, 16, D).astype(BF16)
        return even_lhs(jnp.minimum(i + 1, NIT - 1), acc[0:8])

    def body(it, _):
        @pl.when(it == NLOOP - 1)
        def _():
            c_out[0].start()
            c_out[1].start()

        lhs = _tobf(lhs_scr[...])
        for u in range(UNROLL):
            lhs = pair(it * UNROLL + u, lhs, u == UNROLL - 1)
        lhs_scr[...] = _tou(lhs)
        return 0

    lhs_scr[...] = _tou(even_lhs(0, mem0[...].astype(F32)))
    lax.fori_loop(0, NLOOP, body, 0)

    c_out[2].start()
    acc = _nn(ox_scr[1].astype(BF16), wo_rows(0, H * DH))
    outb[4 * NIT:4 * NIT + 2] = acc.reshape(2, 16, D).astype(BF16)
    c_out[3].start()


def _kernel(*refs):
    refs, osem = refs[:-1], refs[-1]
    pl.run_scoped(lambda sems: _body(sems, osem, *refs), pltpu.SemaphoreType.DMA((NSEM,)))
    out_hbm = refs[11]
    pltpu.make_async_copy(out_hbm, out_hbm, osem).wait()


@jax.jit
def pallas_concat_heads__spectral_gfnet__memory_aug_recurrent_mem_tr__prompt_kernel(
    A_x, A_w_r, A_w_i, B_x, B_mem0, B_Wq, B_Wk, B_Wv, B_Wo, B_seg_len,
):
    del B_seg_len
    assert A_x.shape == (1, S, D) and B_x.shape == (1, S, D) and B_mem0.shape == (1, M, D)
    cm, tw = _fft_consts()
    hbm = pl.BlockSpec(memory_space=pltpu.HBM)
    out = pl.pallas_call(
        _kernel,
        out_shape=jax.ShapeDtypeStruct((S // 16, 16, 2 * D), BF16),
        in_specs=[hbm] * 11,
        out_specs=hbm,
        scratch_shapes=[
            pltpu.VMEM((129, 16, D), BF16),
            pltpu.VMEM((4, 16 * HP + 128, 128), F32),
            pltpu.VMEM((256, S), BF16),
            pltpu.VMEM((256, S), BF16),
            pltpu.VMEM((12 * 64, 128), U32),
            pltpu.VMEM((32, 128), F32),
            pltpu.VMEM((16, 2, U_ROWS, 128), F32),
            pltpu.VMEM((128, 16, D), BF16),
            pltpu.VMEM((NIT, 2 * SEG, D), BF16),
            pltpu.VMEM((NIT, 16, D), BF16),
            pltpu.VMEM((NIT * 8, D), U32),
            pltpu.VMEM((6 * D, 16, 128), BF16),
            pltpu.VMEM((XS0 + 64 * HP + 160, 128), U32),
            pltpu.VMEM((H * DH, D), BF16),
            pltpu.VMEM((NPRE, NIT * 16, 256), F32),
            pltpu.VMEM((24, D), U32),
            pltpu.VMEM((8, H * DH), F32),
            pltpu.VMEM((M, H * DH), F32),
            pltpu.VMEM((2, SEG, H * DH), F32),
            pltpu.VMEM((4 * NIT + 2, 16, D), BF16),
            pltpu.VMEM((2, 1, S), BF16),
            pltpu.VMEM((16, 128), F32),
            pltpu.VMEM((M, D), BF16),
            pltpu.VMEM((3 * NP - NPRE, 8, 256), F32),
            pltpu.VMEM((80, 80), F32),
            pltpu.SMEM((1,), jnp.int32),
            pltpu.SemaphoreType.DMA(()),
        ],
        compiler_params=pltpu.CompilerParams(vmem_limit_bytes=110 * 1024 * 1024),
    )(
        A_x.reshape(S // 16, 16, D), A_w_r.T, A_w_i.T,
        B_x.reshape(NIT, 2 * SEG, D), B_mem0.reshape(M, D),
        B_Wq, B_Wk, B_Wv, B_Wo.reshape(H * DH, D),
        jnp.asarray(cm), jnp.asarray(tw),
    )
    return out.reshape(1, S, 2 * D)
```

```python
import functools

import numpy as np
import jax
import jax.numpy as jnp
from jax import lax
import jax.experimental.pallas as pl
import jax.experimental.pallas.tpu as pltpu

F32 = jnp.float32
BF16 = jnp.bfloat16
U32 = jnp.uint32

S, D = 2048, 512
H, DH = 32, 128
M, SEG = 8, 32
L = M + SEG
NP = H // 2
NIT = S // (2 * SEG)
SCALE = DH ** -0.5
LOG2E = 1.4426950408889634
NEG = -1000000000.0
R2 = float(np.sqrt(0.5))


def _nt(a, b):
    return lax.dot_general(a, b, (((1,), (1,)), ((), ())), preferred_element_type=F32)


def _nn(a, b):
    return jnp.dot(a, b, preferred_element_type=F32)


def _tobf(u):
    return pltpu.bitcast(u, BF16)


def _tou(b):
    return pltpu.bitcast(b, U32)


def _swap(a):
    return pltpu.roll(a, 64, a.ndim - 1)


def _cs(num, den):
    ang = 2.0 * np.pi * np.mod(num, den) / den
    c, s = np.cos(ang), np.sin(ang)
    c[np.abs(c) < 1e-12] = 0.0
    s[np.abs(s) < 1e-12] = 0.0
    return c, s


def _pack_rows(a):
    b = np.asarray(a, np.float32).astype(jnp.bfloat16).view(np.uint16).astype(np.uint32)
    return b[0::2] | (b[1::2] << 16)


def _fft_consts():
    d1, e64, j32 = np.arange(128), np.arange(64), np.arange(32)
    f0 = np.concatenate([8 * j32, 8 * j32 + 4])
    f2 = np.concatenate([8 * j32 + 2, 8 * j32 + 6])
    fa = np.concatenate([8 * j32 + 1, 8 * j32 + 7])
    fb = np.concatenate([8 * j32 + 5, 8 * j32 + 3])
    c, s = _cs(np.outer(f0, d1), D)
    l0 = np.concatenate([c, -s], 0)
    l0[64] = 1.0 - 2.0 * (d1 % 2)
    c, s = _cs(np.outer(f2, d1), D)
    l2 = np.concatenate([c, -s], 0)

    def odd(f, imsign):
        c, s = _cs(np.outer(f, e64), D)
        sg = np.where(f % 4 == 1, imsign, -imsign)[:, None]
        return np.block([[c, sg * s], [-s, sg * c]])

    la, lb = odd(fa, -1.0), odd(fb, 1.0)
    g, hm = [], []
    for par in range(2):
        c, s = _cs(np.outer(2 * e64 + par, e64), 128)
        sg = 1.0 - 2.0 * par
        g.append(np.block([[c, -s], [s, c]]))
        hm.append(np.block([[c, -sg * s], [s, sg * c]]))
    sc = 2.0 / (S * D)
    i0 = sc * l0
    i0[0] *= 0.5
    i0[64] *= 0.5
    il = lambda a: a.reshape(2, 4, 16, 128).transpose(1, 0, 2, 3).reshape(128, 128)
    mats = [il(l0), il(l2), il(la), il(lb), g[0], g[1], il(hm[0]), il(hm[1]), i0, sc * l2, sc * la, sc * lb]
    tc, ts = _cs(np.outer(np.arange(16), d1), S)
    return _pack_rows(np.concatenate(mats, 0)), np.concatenate([tc, ts], 0).astype(np.float32)


def _cmul_const(z, k, n, sign):
    re, im = z
    k = k % n
    if k == 0:
        return z
    if 4 * k == n:
        return (-im, re) if sign > 0 else (im, -re)
    c = float(np.cos(2 * np.pi * k / n))
    s = float(sign * np.sin(2 * np.pi * k / n))
    if (8 * k) % n == 0:
        a, b = re * c, im * c
        return (a - b, b + a) if s / c > 0 else (a + b, b - a)
    return (re * c - im * s, re * s + im * c)


def _dft4(a, b, c, d, sign):
    s0 = (a[0] + c[0], a[1] + c[1])
    s1 = (a[0] - c[0], a[1] - c[1])
    s2 = (b[0] + d[0], b[1] + d[1])
    s3 = (b[0] - d[0], b[1] - d[1])
    y0 = (s0[0] + s2[0], s0[1] + s2[1])
    y2 = (s0[0] - s2[0], s0[1] - s2[1])
    ya = (s1[0] + s3[1], s1[1] - s3[0])
    yb = (s1[0] - s3[1], s1[1] + s3[0])
    return [y0, ya, y2, yb] if sign < 0 else [y0, yb, y2, ya]


UNROLL = 4
NLOOP = NIT // UNROLL
NU0 = 2
NA, NB = 3, 8
BA, BB = 4, 3
N5 = 3
NTAIL = 3
PB0 = 16 * (NA + 2) + 8
PPB = 13
B0 = 3
NPRE = B0 + 2 + NA * BA + NB * BB + N5
FSPLIT = (0, 4, 8, 13, 17, 21, 25, 30, 34, 38, 43, 48, 48)
LAG = 2
UP = 9
HP = 132
U_LAST = 32 * UP
U_PIN, U_ROWS = 296, 312
WO0 = 12 * 16 * HP
WO_ROWS = H * DH // NB
XS0 = WO0 + 4 * 2048

SEM_U0 = 0
SEM_XE = SEM_U0 + NU0
SEM_U0B = SEM_XE + 1
SEM_A = SEM_U0B + 1
SEM_XA = SEM_A + NA
SEM_C = SEM_XA + 2
SEM_W = SEM_C + 1
SEM_F = SEM_W + NB
NSEM = SEM_F + 1


def _body(sems, osem, xa_hbm, wr_hbm, wi_hbm, xb_hbm, mem0_hbm, wq_hbm, wk_hbm, wv_hbm, wo_hbm,
          cm_hbm, tw_hbm, out_hbm,
          xa, ys, wr, wi, cm, tw, u_scr, yb, xb, xe, xeu,
          raw, w, wo_raw, pre, mem_scr, tail8, om_scr, ox_scr, outb,
          wlast, t256, mem0, carry8, fill_scr, opq):
    cp = pltpu.make_async_copy

    wsrc = (wq_hbm, wk_hbm, wv_hbm)

    def w_copies(p0, p1, sem):
        out = []
        while p0 < p1:
            u, c = divmod(p0, 16)
            n = min(p1 - p0, 16 - c)
            for half in range(2):
                d0 = 256 * half + 16 * c
                out.append(cp(wsrc[u // 4].at[d0:d0 + 16 * n, 8 * (u % 4):8 * (u % 4) + 8, :],
                              raw.at[16 * p0:16 * (p0 + n), 8 * half:8 * half + 8, :], sem))
            p0 += n
        return out

    pu = 8 // NU0
    xe_cp = lambda j, sem: cp(xb_hbm.at[:, 24:40, 128 * j:128 * j + 128], xe.at[:, :, 128 * j:128 * j + 128], sem)
    c_xe = [xe_cp(0, sems.at[SEM_XE]), xe_cp(2, sems.at[SEM_XE])]
    c_in = list(c_xe)
    for k in range(NU0):
        c_in += w_copies(k * pu, (k + 1) * pu, sems.at[SEM_U0 + k])
    c_u0b = [xe_cp(1, sems.at[SEM_U0B]), xe_cp(3, sems.at[SEM_U0B])] + w_copies(8, 16, sems.at[SEM_U0B])
    c_in += c_u0b
    for g in range(NA):
        c_in += w_copies(16 * (g + 1), 16 * (g + 2), sems.at[SEM_A + g])
        if g:
            c_in.append(cp(xa_hbm.at[64 * (g - 1):64 * g], xa.at[64 * (g - 1):64 * g], sems.at[SEM_XA + g - 1]))
    c_c = [cp(cm_hbm, cm, sems.at[SEM_C]), cp(tw_hbm, tw, sems.at[SEM_C])]
    c_c += w_copies(16 * (NA + 1), PB0, sems.at[SEM_C])
    c_in += c_c
    for g in range(NB):
        sem = sems.at[SEM_W + g]
        c_in += w_copies(PB0 + PPB * g, PB0 + PPB * (g + 1), sem)
        rows = slice(g * WO_ROWS, (g + 1) * WO_ROWS)
        c_in.append(cp(wo_hbm.at[rows], wo_raw.at[rows], sem))
        rows = slice(32 * g, 32 * g + 32)
        c_in += [cp(wr_hbm.at[rows], wr.at[rows], sem), cp(wi_hbm.at[rows], wi.at[rows], sem)]
    c_f = [cp(mem0_hbm, mem0, sems.at[SEM_F]),
           cp(wr_hbm.at[256:257], wlast.at[0], sems.at[SEM_F]),
           cp(wi_hbm.at[256:257], wlast.at[1], sems.at[SEM_F]),
           cp(xb_hbm, xb, sems.at[SEM_F])]
    for c in c_in + c_f:
        c.start()

    opq[0] = U_PIN
    ox_scr[1] = jnp.zeros((SEG, H * DH), F32)
    u_scr[:, :, U_LAST:U_LAST + 8, :] = jnp.zeros((16, 2, 8, 128), F32)
    u_scr[0, 0, U_PIN + 8:U_PIN + 16, :] = jnp.zeros((8, 128), F32)
    ys[0, 16 * HP + 8:16 * HP + 16, :] = jnp.zeros((8, 128), F32)
    xa[128] = jnp.zeros((16, D), BF16)

    row = lax.broadcasted_iota(jnp.int32, (80, 80), 0)
    col = lax.broadcasted_iota(jnp.int32, (80, 80), 1)
    rhead = jnp.where(row < 16, row // 8, (row - 16) // SEG)
    same_head = rhead == col // L
    fill_scr[...] = jnp.where(same_head, NEG / SCALE, -jnp.inf).astype(F32)

    def wait_raw(p0, n, sem):
        blk = raw.at[pl.ds(p0 * 16, n * 16)]
        cp(blk, blk, sem).wait()

    def relayout(pc, zero=None):
        eo = _tou(raw[pl.ds(pc * 16, 16)])
        if zero is not None:
            eo = eo | zero
        eo = eo.reshape(8, 2, 8, 128)
        e, o = eo[:, 0], eo[:, 1]
        h0 = (e & jnp.uint32(0xFFFF)) | (o << 16)
        h1 = (e >> 16) | (o & jnp.uint32(0xFFFF0000))
        base = (pc // 16) * (16 * HP) + (pc % 16) * 8
        for par, hh in enumerate((h0, h1)):
            for t in range(8):
                w[pl.ds(base + par * 8 * HP + t, 8, stride=HP), :] = hh[t]

    def wplane(b, par):
        r0 = ((b // 4) * 16 + par * 8 + b % 4) * HP
        return _tobf(jnp.concatenate([w[pl.ds(r0, 128), :], w[pl.ds(r0 + 4 * HP, 128), :]], axis=0))

    def retile_wo(r16):
        v = _tou(wo_raw[pl.ds(pl.multiple_of(r16 * 16, 16), 16), :])
        for j in range(4):
            w[pl.ds(WO0 + j * 2048 + r16 * 8, 8), :] = v[:, j * 128:(j + 1) * 128]

    def wo_rows(r0, n):
        return _tobf(jnp.concatenate(
            [w[WO0 + j * 2048 + r0 // 2:WO0 + j * 2048 + (r0 + n) // 2, :] for j in range(4)], axis=1))

    def stage_x(n1):
        v = _tou(xa[n1].astype(F32))
        for j in range(4):
            for half in range(2):
                w[pl.ds(XS0 + (j * 16 + half * 8) * HP + n1, 8, stride=HP), :] = (
                    v[8 * half:8 * half + 8, j * 128:(j + 1) * 128])

    def precompute(b, h, m0=0, nm=NIT, zero=None):
        u = xeu[m0 * 8:(m0 + nm) * 8, :]
        if zero is not None:
            top = jnp.concatenate([u[0:8, 0:128] | zero, u[0:8, 128:D]], axis=1)
            u = jnp.concatenate([top, u[8:]], axis=0)
        r = _nn(_tobf(u), wplane(b, h))
        pre[b, m0 * 16:(m0 + nm) * 16, h * 128:(h + 1) * 128] = r
        return r

    def half_dot(b0, t, zero=None):
        return precompute(b0 + t // 4, (t // 2) % 2, (t % 2) * 16, 16, zero)

    def mat(k):
        return _tobf(cm[64 * k:64 * k + 64, :])

    def lo_half(rows):
        return lax.broadcasted_iota(jnp.int32, (rows, 128), 1) < 64

    first = lax.broadcasted_iota(jnp.int32, (8, 128), 0) == 0
    classes = tuple(tuple((r, 32, UP) for r in cl) for cl in ((0, 4), (2, 6), (1, 7), (5, 3)))

    def part(u, h, rows=16):
        return jnp.concatenate([u[(2 * g + h) * rows:(2 * g + h + 1) * rows] for g in range(4)], axis=0)

    def f1_s(n2, x12, kk):
        h, k = kk % 2, kk // 2
        u = _nn(x12[h][k], mat(4 + h))
        r = 0
        for cl in classes[2 * k:2 * k + 2]:
            for (st, n, sd) in cl:
                u_scr[n2, h, pl.ds(st, n, stride=sd), :] = u[r:r + n]
                r += n

    def f1_d(n2, prev):
        def ldx(j):
            r0 = XS0 + (j * 16 + n2) * HP
            u = jnp.concatenate([w[pl.ds(r0 + par, 64, stride=2), :] for par in range(2)], axis=0)
            return pltpu.bitcast(u, F32)

        x0, x1, x2, x3 = [ldx(j) for j in range(4)]
        lo = lo_half(128)
        p, q, b, c = x0 + x2, x1 + x3, x0 - x2, x1 - x3
        r = _swap(jnp.where(lo, c, (b - c) * R2))
        y = jnp.where(lo, b, (b + c) * R2)
        t = []
        for k, a in enumerate((p + q, p - q, y + r, y - r)):
            t.append(_nt(mat(k), a.astype(BF16)))
            if prev is not None:
                f1_s(n2 - LAG, prev, k)
        t256[n2:n2 + 1, :] = t[0][16:17]
        t[0] = jnp.concatenate([t[0][0:16], jnp.where(first, 0.0, t[0][16:24]), t[0][24:128]], axis=0)
        tr = jnp.concatenate([part(u, 0) for u in t], axis=0)
        ti = jnp.concatenate([part(u, 1) for u in t], axis=0)
        lo = lo_half(256)
        rb = _swap(jnp.where(lo, ti, tr))
        x12 = (jnp.where(lo, tr, rb), jnp.where(lo, rb, ti))
        return [[x[128 * k:128 * k + 128].astype(BF16) for k in range(2)] for x in x12]

    def f1_all():
        p0 = 16 * (NA + 1)
        zvec = _tou(ys[0, 16 * HP + 8:16 * HP + 16, :])
        xq = [None] * LAG
        dots = (0, 2, 4, 7, 9, 11, 14, 17)
        for n2 in range(16 + LAG):
            if n2 in dots:
                k = dots.index(n2)
                r = half_dot(B0 + NA * BA, k)
                for j in range(4 if k < 4 else 2):
                    relayout(p0 + (4 * k if k < 4 else 2 * k + 8) + j, _tou(r[64 * j:64 * j + 8]) & zvec)
            if n2 < 16:
                xq.append(f1_d(n2, xq.pop(0)))
            else:
                xp = xq.pop(0)
                for kk in range(4):
                    f1_s(n2 - LAG, xp, kk)
        t = t256[...]
        lo = lo_half(16)
        for h, v in enumerate((t, _swap(t))):
            u = _nn(jnp.where(lo, v, 0.0).astype(BF16), mat(4 + h))
            for n2 in range(16):
                u_scr[n2, h, U_LAST:U_LAST + 1, :] = u[n2:n2 + 1]

    tok = [None]

    def f2_pieces(ru, filt):
        def ld(n):
            z = [u_scr[n, h, pl.ds(ru, 8), :] for h in range(2)]
            if tok[0] is not None:
                z = [pltpu.bitcast(_tou(v) | tok[0], F32) for v in z]
            return tuple(z)

        lo = lo_half(8)

        def st(n, z):
            u_scr[n, 0, pl.ds(ru, 8), :] = z[0]
            u_scr[n, 1, pl.ds(ru, 8), :] = z[1]

        def ld_in(n):
            e, o = ld(n)
            p, q = e + o, e - o
            r = _swap(jnp.where(lo, q, p))
            re, im = jnp.where(lo, p, r), jnp.where(lo, r, q)
            if n == 0:
                return re, im
            c, s = tw[n:n + 1, :], tw[16 + n:17 + n, :]
            return re * c + im * s, im * c - re * s

        def st_out(n, z):
            re, im = z
            if n:
                c, s = tw[n:n + 1, :], tw[16 + n:17 + n, :]
                re, im = re * c - im * s, im * c + re * s
            a = jnp.where(lo, re, im)
            r = _swap(jnp.where(lo, im, re))
            st(n, (a + r, a - r))

        def outer(b, sign):
            y = _dft4(*[(ld_in if sign < 0 else ld)(4 * a + b) for a in range(4)], sign)
            for a in range(4):
                (st if sign < 0 else st_out)(4 * a + b, y[a])

        def inner(p):
            x = _dft4(*[_cmul_const(ld(4 * p + b), b * p, 16, -1) for b in range(4)], -1)
            y = []
            for q in range(4):
                lanes = slice((p + 4 * q) * 128, (p + 4 * q + 1) * 128)
                a, b = filt(lanes)
                y.append((x[q][0] * a - x[q][1] * b, x[q][0] * b + x[q][1] * a))
            v = _dft4(*y, +1)
            for b in range(4):
                st(4 * p + b, _cmul_const(v[b], b * p, 16, +1))

        return ([functools.partial(outer, b, -1) for b in range(4)],
                [functools.partial(inner, p) for p in range(4)],
                [functools.partial(outer, b, +1) for b in range(4)])

    def f3_s(n2, zero=None):
        lo = lo_half(128)
        zs = []
        for par in range(2):
            cls = [jnp.concatenate([u_scr[n2, par, pl.ds(st, n, stride=sd), :] for (st, n, sd) in cl], axis=0)
                   for cl in classes]
            hmu = cm[64 * (6 + par):64 * (7 + par), :]
            sign = jnp.where(lo_half(8), 2.0 * par - 1.0, 1.0 - 2.0 * par)
            last = _swap(u_scr[n2, par, U_LAST:U_LAST + 8, :]) * sign
            if zero is not None and par == 1:
                last = last + zero
            rhs_a = jnp.concatenate([cls[0], cls[1]], axis=0).astype(BF16)
            rhs_b = jnp.concatenate([jnp.where(first, last, cls[0][0:8]), cls[0][8:64], cls[1]],
                                    axis=0).astype(BF16)
            zo = _nt(_tobf(hmu), jnp.concatenate([cls[2], cls[3]], axis=0).astype(BF16))
            zs.append((_nt(_tobf(part(hmu, 0, 8)), rhs_a), _nt(_tobf(part(hmu, 1, 8)), rhs_b),
                       part(zo, 0), part(zo, 1)))
        out = []
        for k in range(2):
            re = jnp.concatenate([zs[0][2 * k], zs[1][2 * k]], axis=0)
            im = jnp.concatenate([zs[0][2 * k + 1], zs[1][2 * k + 1]], axis=0)
            r = _swap(jnp.where(lo, im, re))
            out += [jnp.where(lo, re, r).astype(BF16), jnp.where(lo, r, im).astype(BF16)]
        return out

    def f3_d(n2, z):
        b0, b2, g1, g5 = [_nn(z[k], mat(8 + k)) for k in range(4)]
        lo = lo_half(128)
        y = g1 + g5
        r = _swap(g1 - g5)
        b = jnp.where(lo, y, (y + r) * R2)
        c = jnp.where(lo, r, (y - r) * R2)
        p, q = b0 + b2, b0 - b2
        for j, v in enumerate((p + b, q + c, p - b, q - c)):
            for par in range(2):
                ys[j, pl.ds(n2 * HP + par, 64, stride=2), :] = v[64 * par:64 * par + 64]

    def gather_y(n1, half):
        v = [ys[j, pl.ds(half * 8 * HP + n1, 8, stride=HP), :] for j in range(4)]
        yb[n1, half * 8:half * 8 + 8, :] = jnp.concatenate(v, axis=1).astype(BF16)

    def f3_all():
        prow = pl.multiple_of(opq[0] + (16 * HP - U_PIN), 8)
        b0 = NPRE - N5
        nin = 4 * N5 - NTAIL - 2
        wl = [wlast[k].astype(F32) for k in range(2)]
        stages = f2_pieces(U_LAST, lambda lanes: [jnp.broadcast_to(v[:, lanes], (8, 128)) for v in wl])
        zvec = _tou(ys[0, 16 * HP + 8:16 * HP + 16, :])
        r = half_dot(b0, 0)
        for k, pc in enumerate(stages[0] + stages[1] + stages[2]):
            tok[0] = (_tou(r[(k - 4) * 24:(k - 4) * 24 + 8]) & zvec) if k >= 4 else None
            pc()
        tok[0] = None
        half_dot(b0, 1)
        zq = [f3_s(0), f3_s(1)]
        zero = None
        for n2 in range(16):
            for t in range(n2 * nin // 16, (n2 + 1) * nin // 16):
                half_dot(b0, 2 + t)
            if n2 + 2 < 16:
                zq.append(f3_s(n2 + 2, zero))
            zero = ys[0, pl.ds(prow + 8, 8), :]
            f3_d(n2, zq.pop(0))
            if n2 >= 8:
                ys[0, pl.ds(prow, 8), :] = zero
                for n1 in range((n2 - 8) * 16, (n2 - 7) * 16):
                    gather_y(n1, 0)
        npin = 8 * NTAIL - 5
        for k in range(NTAIL):
            r = half_dot(b0, 2 + nin + k)
            for j in range(min(8, npin - 8 * k)):
                ys[0, pl.ds(prow, 8), :] = r[32 * j:32 * j + 8]
                for n1 in range((8 * k + j) * 128 // npin, (8 * k + j + 1) * 128 // npin):
                    gather_y(n1, 1)

    def unit0(k, _):
        wait_raw(k * pu, pu, sems.at[SEM_U0 + k])
        for t in range(pu):
            relayout(k * pu + t)
        return 0

    def retile_xe(j):
        xeu[:, 128 * j:128 * j + 128] = _tou(xe[:, :, 128 * j:128 * j + 128].reshape(NIT * 16, 128))

    def partial(b, kh):
        lhs = jnp.concatenate([xeu[:, 128 * j:128 * j + 128] for j in (kh, kh + 2)], axis=1)
        rhs = jnp.concatenate(
            [jnp.concatenate([w[pl.ds((par * 8 + b + 4 * half) * HP + 64 * kh, 64), :] for half in range(2)], axis=0)
             for par in range(2)], axis=1)
        r = _nn(_tobf(lhs), _tobf(rhs))
        pre[b] = r + pre[b] if kh else r

    for c in c_xe:
        c.wait()
    retile_xe(0)
    retile_xe(2)
    lax.fori_loop(0, NU0, unit0, 0)
    partial(0, 0)
    partial(1, 0)
    for c in c_u0b:
        c.wait()
    partial(2, 0)
    retile_xe(1)
    retile_xe(3)
    for pc in range(8, 16):
        relayout(pc)
    for b in range(B0):
        partial(b, 1)

    def body_a(g, _):
        p0 = 16 * (g + 1)
        wait_raw(p0, 16, sems.at[SEM_A + g])

        @pl.when(g > 0)
        def _():
            gm = jnp.maximum(g - 1, 0)
            blk = xa.at[pl.ds(64 * gm, 64)]
            cp(blk, blk, sems.at[SEM_XA + gm]).wait()

        for t in range(8):
            precompute(B0 + BA * g, t // 4, (t % 4) * 8, 8)
            relayout(p0 + 2 * t)
            relayout(p0 + 2 * t + 1)
        for t in range(4, 4 * BA):
            half_dot(B0 + BA * g, t)
            for k in range(64 * (t - 4) // 12, 64 * (t - 3) // 12):
                stage_x(jnp.where(g > 0, 64 * (g - 1) + k, 128))
        return 0

    lax.fori_loop(0, NA, body_a, 0)
    for c in c_c:
        c.wait()
    f1_all()

    def body_b(g, _):
        p0 = PB0 + PPB * g
        sem = sems.at[SEM_W + g]
        wait_raw(p0, PPB, sem)
        r32 = pl.multiple_of(g * 32, 32)
        for blk in (wo_raw.at[pl.ds(pl.multiple_of(g * WO_ROWS, WO_ROWS), WO_ROWS)],
                    wr.at[pl.ds(r32, 32)], wi.at[pl.ds(r32, 32)]):
            cp(blk, blk, sem).wait()
        pin_row = pl.multiple_of(opq[0], 8)
        filt = lambda k, lanes: [v[pl.ds(r32 + 8 * k, 8), lanes].astype(F32) for v in (wr, wi)]
        groups = [f2_pieces(g * (4 * UP) + UP * k, functools.partial(filt, k)) for k in range(4)]
        pieces = [pc for st in range(3) for k in range(4) for pc in groups[k][st]]
        nd = 4 * BB
        zeros = [None, None]
        zvec = _tou(ys[0, 16 * HP + 8:16 * HP + 16, :])
        for t in range(nd):
            v = half_dot(B0 + 2 + NA * BA + BB * g, t, zeros.pop(0))
            for k in range(-(-PPB * t // nd), -(-PPB * (t + 1) // nd)):
                relayout(p0 + k)
            for k in range(32 * t // nd, 32 * (t + 1) // nd):
                retile_wo(g * (WO_ROWS // 16) + k)
            todo = pieces[FSPLIT[t]:FSPLIT[t + 1]]
            for k, pc in enumerate(todo):
                r0 = 8 * ((32 * k) // len(todo))
                tok[0] = _tou(v[r0:r0 + 8]) & zvec
                pc()
            tok[0] = None
            zeros.append(_tou(u_scr[0, 0, pl.ds(pin_row + 8, 8), :]) if todo else None)
        return 0

    lax.fori_loop(0, NB, body_b, 0)
    for c in c_f:
        c.wait()
    f3_all()

    rpos = jnp.where(row < 16, L, (row - 16) % SEG + M)
    mask = same_head & (rpos >= col % L)

    def qkv(st, i, lhs, lhs_v, p, even):
        r16 = pl.multiple_of(i * 16, 16)

        def proj(blk):
            wb = jnp.concatenate([wplane(blk, 0), wplane(blk, 1)], axis=1)
            if blk < NPRE:
                r = _nn(lhs, wb)
                if even:
                    return r[0:8], jnp.concatenate([r[8:32], pre[blk, pl.ds(r16, 8), :]], axis=0)
                return r[0:8], jnp.concatenate([pre[blk, pl.ds(r16 + 8, 8), :], r[8:32]], axis=0)
            r = _nn(lhs_v, wb)
            if even:
                carry8[blk - NPRE] = r[40:48]
                return r[0:8], r[8:40]
            return r[0:8], jnp.concatenate([carry8[blk - NPRE], r[8:32]], axis=0)

        mq, xq = proj(p)
        mk, xk = proj(NP + p)
        mv, xv = proj(2 * NP + p)
        h0 = lambda a: a[:, 0:128]
        h1 = lambda a: a[:, 128:256]
        st["q"][p] = jnp.concatenate([h0(mq), h1(mq), h0(xq), h1(xq)], axis=0).astype(BF16)
        st["k"][p] = jnp.concatenate([h0(mk), h0(xk), h1(mk), h1(xk)], axis=0).astype(BF16)
        st["v"][p] = jnp.concatenate([h0(mv), h0(xv), h1(mv), h1(xv)], axis=0).astype(BF16)

    def qk_group(st, g):
        for p in range(4 * g, 4 * g + 4):
            s = _nt(st["q"][p], st["k"][p])
            s = jnp.where(mask, s, fill_scr[...])
            m = jnp.max(s, axis=-1, keepdims=True)
            e = jnp.exp2((s - m) * (SCALE * LOG2E))
            l = jnp.sum(e, axis=-1, keepdims=True)
            st["p"][p] = e * pl.reciprocal(l, approx=True)

    def put_om(p, o):
        om_scr[:, (2 * p) * 128:(2 * p + 1) * 128] = o[0:8]
        om_scr[:, (2 * p + 1) * 128:(2 * p + 2) * 128] = o[8:16]

    def put_ox(b, p, o):
        ox_scr[b, :, (2 * p) * 128:(2 * p + 1) * 128] = o[0:32]
        ox_scr[b, :, (2 * p + 1) * 128:(2 * p + 2) * 128] = o[32:64]

    def pvm_group(st, g, b):
        for p in range(4 * g, 4 * g + 4):
            put_om(p, _nn(st["p"][p][0:16].astype(BF16), st["v"][p]))

    def pvx_group(st, g, b):
        for p in range(4 * g, 4 * g + 4):
            put_ox(b, p, _nn(st["p"][p][16:80].astype(BF16), st["v"][p]))

    def pv_group(st, g, b):
        for p in range(4 * g, 4 * g + 4):
            o = _nn(st["p"][p].astype(BF16), st["v"][p])
            put_om(p, o[0:16])
            put_ox(b, p, o[16:80])

    def oproj(c, even, acc):
        cs = slice(c * 512, (c + 1) * 512)
        if even:
            lhs = jnp.concatenate([om_scr[:, cs], ox_scr[1, 0:24, cs]], axis=0)
            tail8[:, cs] = ox_scr[1, 24:32, cs]
        else:
            lhs = jnp.concatenate([om_scr[:, cs], tail8[:, cs], ox_scr[0, :, cs]], axis=0)
        r = _nn(lhs.astype(BF16), wo_rows(c * 512, 512))
        return r if acc is None else r + acc

    def step(i, lhs_v, even, late):
        b = 0 if even else 1
        st = dict(q={}, k={}, v={}, p={})
        lhs = lhs_v[0:32]
        for p in range(4):
            qkv(st, i, lhs, lhs_v, p, even)
        for g in range(3):
            qkv(st, i, lhs, lhs_v, 4 * g + 4, even)
            qk_group(st, g)
            for p in range(4 * g + 5, 4 * g + 8):
                qkv(st, i, lhs, lhs_v, p, even)
                if not late and g and p == 4 * g + 5:
                    pvx_group(st, g - 1, b)
            pvm_group(st, g, b)
        acc = oproj(0, even, None)
        qk_group(st, 3)
        for c in range(1, 4):
            acc = oproj(c, even, acc)
            if not late and c == 1:
                pvx_group(st, 2, b)
        (pvm_group if late else pv_group)(st, 3, b)
        for c in range(4, 8):
            acc = oproj(c, even, acc)
        if late:
            for g in range(4):
                pvx_group(st, g, b)
        return acc

    nb = 4 * (NIT - UNROLL)
    ob = lambda g0, g1: cp(outb.at[g0:g1], out_hbm.at[g0 - 2:g1 - 2, :, D:2 * D], osem)
    c_out = [cp(yb, out_hbm.at[:, :, 0:D], osem), ob(2, nb), ob(nb, 4 * NIT), ob(4 * NIT, 4 * NIT + 2)]

    def even_lhs(i, mem):
        return jnp.concatenate([mem, xb[i, 0:40, :].astype(F32)], axis=0).astype(BF16)

    def pair(i, mem, last):
        acc = step(i, even_lhs(i, mem), True, True)
        outb[4 * i] = acc[8:24].astype(BF16)
        stash = acc[24:32]
        xf = xb[i, 40:64, :].astype(F32)
        acc = step(i, jnp.concatenate([acc[0:8], xf], axis=0).astype(BF16), False, not last)
        o48 = jnp.concatenate([stash, acc[8:48]], axis=0)
        outb[pl.ds(4 * i + 1, 3)] = o48.reshape(3, 16, D).astype(BF16)
        return acc[0:8]

    def body(it, _):
        @pl.when(it == NLOOP - 1)
        def _():
            c_out[0].start()
            c_out[1].start()

        mem = mem_scr[...]
        for u in range(UNROLL):
            mem = pair(it * UNROLL + u, mem, u == UNROLL - 1)
        mem_scr[...] = mem
        return 0

    mem_scr[...] = mem0[...].astype(F32)
    lax.fori_loop(0, NLOOP, body, 0)

    c_out[2].start()
    acc = _nn(ox_scr[1].astype(BF16), wo_rows(0, H * DH))
    outb[4 * NIT:4 * NIT + 2] = acc.reshape(2, 16, D).astype(BF16)
    c_out[3].start()


def _kernel(*refs):
    refs, osem = refs[:-1], refs[-1]
    pl.run_scoped(lambda sems: _body(sems, osem, *refs), pltpu.SemaphoreType.DMA((NSEM,)))
    out_hbm = refs[11]
    pltpu.make_async_copy(out_hbm, out_hbm, osem).wait()


@jax.jit
def pallas_concat_heads__spectral_gfnet__memory_aug_recurrent_mem_tr__prompt_kernel(
    A_x, A_w_r, A_w_i, B_x, B_mem0, B_Wq, B_Wk, B_Wv, B_Wo, B_seg_len,
):
    del B_seg_len
    assert A_x.shape == (1, S, D) and B_x.shape == (1, S, D) and B_mem0.shape == (1, M, D)
    cm, tw = _fft_consts()
    hbm = pl.BlockSpec(memory_space=pltpu.HBM)
    out = pl.pallas_call(
        _kernel,
        out_shape=jax.ShapeDtypeStruct((S // 16, 16, 2 * D), BF16),
        in_specs=[hbm] * 11,
        out_specs=hbm,
        scratch_shapes=[
            pltpu.VMEM((129, 16, D), BF16),
            pltpu.VMEM((4, 16 * HP + 128, 128), F32),
            pltpu.VMEM((256, S), BF16),
            pltpu.VMEM((256, S), BF16),
            pltpu.VMEM((12 * 64, 128), U32),
            pltpu.VMEM((32, 128), F32),
            pltpu.VMEM((16, 2, U_ROWS, 128), F32),
            pltpu.VMEM((128, 16, D), BF16),
            pltpu.VMEM((NIT, 2 * SEG, D), BF16),
            pltpu.VMEM((NIT, 16, D), BF16),
            pltpu.VMEM((NIT * 8, D), U32),
            pltpu.VMEM((6 * D, 16, 128), BF16),
            pltpu.VMEM((XS0 + 64 * HP + 160, 128), U32),
            pltpu.VMEM((H * DH, D), BF16),
            pltpu.VMEM((NPRE, NIT * 16, 256), F32),
            pltpu.VMEM((M, D), F32),
            pltpu.VMEM((8, H * DH), F32),
            pltpu.VMEM((M, H * DH), F32),
            pltpu.VMEM((2, SEG, H * DH), F32),
            pltpu.VMEM((4 * NIT + 2, 16, D), BF16),
            pltpu.VMEM((2, 1, S), BF16),
            pltpu.VMEM((16, 128), F32),
            pltpu.VMEM((M, D), BF16),
            pltpu.VMEM((3 * NP - NPRE, 8, 256), F32),
            pltpu.VMEM((80, 80), F32),
            pltpu.SMEM((1,), jnp.int32),
            pltpu.SemaphoreType.DMA(()),
        ],
        compiler_params=pltpu.CompilerParams(vmem_limit_bytes=110 * 1024 * 1024),
    )(
        A_x.reshape(S // 16, 16, D), A_w_r.T, A_w_i.T,
        B_x.reshape(NIT, 2 * SEG, D), B_mem0.reshape(M, D),
        B_Wq, B_Wk, B_Wv, B_Wo.reshape(H * DH, D),
        jnp.asarray(cm), jnp.asarray(tw),
    )
    return out.reshape(1, S, 2 * D)
```

```python
import functools

import numpy as np
import jax
import jax.numpy as jnp
from jax import lax
import jax.experimental.pallas as pl
import jax.experimental.pallas.tpu as pltpu

F32 = jnp.float32
BF16 = jnp.bfloat16
U32 = jnp.uint32

S, D = 2048, 512
H, DH = 32, 128
M, SEG = 8, 32
L = M + SEG
NP = H // 2
NIT = S // (2 * SEG)
SCALE = DH ** -0.5
LOG2E = 1.4426950408889634
NEG = -1000000000.0
R2 = float(np.sqrt(0.5))


def _nt(a, b):
    return lax.dot_general(a, b, (((1,), (1,)), ((), ())), preferred_element_type=F32)


def _nn(a, b):
    return jnp.dot(a, b, preferred_element_type=F32)


def _tobf(u):
    return pltpu.bitcast(u, BF16)


def _tou(b):
    return pltpu.bitcast(b, U32)


def _swap(a):
    return pltpu.roll(a, 64, a.ndim - 1)


def _cs(num, den):
    ang = 2.0 * np.pi * np.mod(num, den) / den
    c, s = np.cos(ang), np.sin(ang)
    c[np.abs(c) < 1e-12] = 0.0
    s[np.abs(s) < 1e-12] = 0.0
    return c, s


def _pack_rows(a):
    b = np.asarray(a, np.float32).astype(jnp.bfloat16).view(np.uint16).astype(np.uint32)
    return b[0::2] | (b[1::2] << 16)


def _fft_consts():
    d1, e64, j32 = np.arange(128), np.arange(64), np.arange(32)
    f0 = np.concatenate([8 * j32, 8 * j32 + 4])
    f2 = np.concatenate([8 * j32 + 2, 8 * j32 + 6])
    fa = np.concatenate([8 * j32 + 1, 8 * j32 + 7])
    fb = np.concatenate([8 * j32 + 5, 8 * j32 + 3])
    c, s = _cs(np.outer(f0, d1), D)
    l0 = np.concatenate([c, -s], 0)
    l0[64] = 1.0 - 2.0 * (d1 % 2)
    c, s = _cs(np.outer(f2, d1), D)
    l2 = np.concatenate([c, -s], 0)

    def odd(f, imsign):
        c, s = _cs(np.outer(f, e64), D)
        sg = np.where(f % 4 == 1, imsign, -imsign)[:, None]
        return np.block([[c, sg * s], [-s, sg * c]])

    la, lb = odd(fa, -1.0), odd(fb, 1.0)
    g, hm = [], []
    for par in range(2):
        c, s = _cs(np.outer(2 * e64 + par, e64), 128)
        sg = 1.0 - 2.0 * par
        g.append(np.block([[c, -s], [s, c]]))
        hm.append(np.block([[c, -sg * s], [s, sg * c]]))
    sc = 2.0 / (S * D)
    i0 = sc * l0
    i0[0] *= 0.5
    i0[64] *= 0.5
    il = lambda a: a.reshape(2, 4, 16, 128).transpose(1, 0, 2, 3).reshape(128, 128)
    mats = [il(l0), il(l2), il(la), il(lb), g[0], g[1], il(hm[0]), il(hm[1]), i0, sc * l2, sc * la, sc * lb]
    tc, ts = _cs(np.outer(np.arange(16), d1), S)
    return _pack_rows(np.concatenate(mats, 0)), np.concatenate([tc, ts], 0).astype(np.float32)


def _cmul_const(z, k, n, sign):
    re, im = z
    k = k % n
    if k == 0:
        return z
    if 4 * k == n:
        return (-im, re) if sign > 0 else (im, -re)
    c = float(np.cos(2 * np.pi * k / n))
    s = float(sign * np.sin(2 * np.pi * k / n))
    if (8 * k) % n == 0:
        a, b = re * c, im * c
        return (a - b, b + a) if s / c > 0 else (a + b, b - a)
    return (re * c - im * s, re * s + im * c)


def _dft4(a, b, c, d, sign):
    s0 = (a[0] + c[0], a[1] + c[1])
    s1 = (a[0] - c[0], a[1] - c[1])
    s2 = (b[0] + d[0], b[1] + d[1])
    s3 = (b[0] - d[0], b[1] - d[1])
    y0 = (s0[0] + s2[0], s0[1] + s2[1])
    y2 = (s0[0] - s2[0], s0[1] - s2[1])
    ya = (s1[0] + s3[1], s1[1] - s3[0])
    yb = (s1[0] - s3[1], s1[1] + s3[0])
    return [y0, ya, y2, yb] if sign < 0 else [y0, yb, y2, ya]


UNROLL = 4
NLOOP = NIT // UNROLL
NU0 = 2
NA, NB = 3, 8
BA, BB = 4, 3
N5 = 3
NTAIL = 4
B0 = 3
NOPRE = (35, 39, 43, 47)
FSPLIT = (4, 8, 12, 16, 20, 24, 28, 32, 36, 40, 44, 48, 48)
LAG = 2
D3 = (3, 6, 9, 11, 14, 15)
UP = 9
HP = 132
UQ = 96
U_LAST = 4 * UQ
U_PIN, U_ROWS = 392, 408
WO0 = 12 * 16 * HP
WO_ROWS = H * DH // NB
XS0 = WO0 + 4 * 2048

SEM_U0 = 0
SEM_XE = SEM_U0 + NU0
SEM_U0B = SEM_XE + 1
SEM_A = SEM_U0B + 1
SEM_XA = SEM_A + NA
SEM_C = SEM_XA + 2
SEM_W = SEM_C + 1
SEM_U = SEM_W + NB
SEM_F = SEM_U + NB - 1
NSEM = SEM_F + 1


def _body(sems, osem, xa_hbm, wr_hbm, wi_hbm, xb_hbm, mem0_hbm, wq_hbm, wk_hbm, wv_hbm, wo_hbm,
          cm_hbm, tw_hbm, out_hbm,
          xa, ys, wr, wi, cm, tw, u_scr, yb, xb, xe, xeu,
          raw, w, wo_raw, pre, mem_scr, tail8, om_scr, ox_scr, outb,
          wlast, t256, mem0, carry8, fill_scr, opq):
    cp = pltpu.make_async_copy

    wsrc = (wq_hbm, wk_hbm, wv_hbm)

    def w_copies(p0, p1, sem):
        out = []
        while p0 < p1:
            u, c = divmod(p0, 16)
            n = min(p1 - p0, 16 - c)
            for half in range(2):
                d0 = 256 * half + 16 * c
                out.append(cp(wsrc[u // 4].at[d0:d0 + 16 * n, 8 * (u % 4):8 * (u % 4) + 8, :],
                              raw.at[16 * p0:16 * (p0 + n), 8 * half:8 * half + 8, :], sem))
            p0 += n
        return out

    pu = 8 // NU0
    xe_cp = lambda j, sem: cp(xb_hbm.at[:, 24:40, 128 * j:128 * j + 128], xe.at[:, :, 128 * j:128 * j + 128], sem)
    c_xe = [xe_cp(0, sems.at[SEM_XE]), xe_cp(2, sems.at[SEM_XE])]
    c_in = list(c_xe)
    for k in range(NU0):
        c_in += w_copies(k * pu, (k + 1) * pu, sems.at[SEM_U0 + k])
    c_u0b = [xe_cp(1, sems.at[SEM_U0B]), xe_cp(3, sems.at[SEM_U0B])] + w_copies(8, 16, sems.at[SEM_U0B])
    c_in += c_u0b
    for g in range(NA):
        c_in += w_copies(16 * (g + 1), 16 * (g + 2), sems.at[SEM_A + g])
        if g:
            c_in.append(cp(xa_hbm.at[64 * (g - 1):64 * g], xa.at[64 * (g - 1):64 * g], sems.at[SEM_XA + g - 1]))
    c_c = [cp(cm_hbm, cm, sems.at[SEM_C]), cp(tw_hbm, tw, sems.at[SEM_C])]
    c_c += w_copies(16 * (NA + 1), 16 * (NA + 2), sems.at[SEM_C])
    c_in += c_c
    for g in range(NB):
        sem = sems.at[SEM_W + g]
        if g < NB - 1:
            c_in += w_copies(16 * (NA + 2 + g), 16 * (NA + 3 + g), sems.at[SEM_U + g])
        rows = slice(g * WO_ROWS, (g + 1) * WO_ROWS)
        c_in.append(cp(wo_hbm.at[rows], wo_raw.at[rows], sem))
        rows = slice(32 * g, 32 * g + 32)
        c_in += [cp(wr_hbm.at[rows], wr.at[rows], sem), cp(wi_hbm.at[rows], wi.at[rows], sem)]
    c_f = [cp(mem0_hbm, mem0, sems.at[SEM_F]),
           cp(wr_hbm.at[256:257], wlast.at[0], sems.at[SEM_F]),
           cp(wi_hbm.at[256:257], wlast.at[1], sems.at[SEM_F]),
           cp(xb_hbm, xb, sems.at[SEM_F])]
    for c in c_in + c_f:
        c.start()

    opq[0] = U_PIN
    ox_scr[1] = jnp.zeros((SEG, H * DH), F32)
    u_scr[:, :, U_LAST:U_LAST + 8, :] = jnp.zeros((16, 2, 8, 128), F32)
    u_scr[0, 0, U_PIN + 8:U_PIN + 16, :] = jnp.zeros((8, 128), F32)
    ys[0, 16 * HP + 8:16 * HP + 16, :] = jnp.zeros((8, 128), F32)
    xa[128] = jnp.zeros((16, D), BF16)

    row = lax.broadcasted_iota(jnp.int32, (80, 80), 0)
    col = lax.broadcasted_iota(jnp.int32, (80, 80), 1)
    rhead = jnp.where(row < 16, row // 8, (row - 16) // SEG)
    same_head = rhead == col // L
    fill_scr[...] = jnp.where(same_head, NEG / SCALE, -jnp.inf).astype(F32)

    def wait_raw(p0, n, sem):
        blk = raw.at[pl.ds(p0 * 16, n * 16)]
        cp(blk, blk, sem).wait()

    def relayout(u, c, zero=None):
        eo = _tou(raw[pl.ds(u * 256 + c * 16, 16)])
        if zero is not None:
            eo = eo | zero
        eo = eo.reshape(8, 2, 8, 128)
        e, o = eo[:, 0], eo[:, 1]
        h0 = (e & jnp.uint32(0xFFFF)) | (o << 16)
        h1 = (e >> 16) | (o & jnp.uint32(0xFFFF0000))
        base = u * (16 * HP) + c * 8
        for par, hh in enumerate((h0, h1)):
            for t in range(8):
                w[pl.ds(base + par * 8 * HP + t, 8, stride=HP), :] = hh[t]

    def wplane(u, j, par):
        r0 = u * (16 * HP) + (par * 8 + j) * HP
        return _tobf(jnp.concatenate([w[pl.ds(r0, 128), :], w[pl.ds(r0 + 4 * HP, 128), :]], axis=0))

    def retile_wo(r16):
        v = _tou(wo_raw[pl.ds(pl.multiple_of(r16 * 16, 16), 16), :])
        for j in range(4):
            w[pl.ds(WO0 + j * 2048 + r16 * 8, 8), :] = v[:, j * 128:(j + 1) * 128]

    def wo_rows(r0, n):
        return _tobf(jnp.concatenate(
            [w[WO0 + j * 2048 + r0 // 2:WO0 + j * 2048 + (r0 + n) // 2, :] for j in range(4)], axis=1))

    def stage_x(n1):
        v = _tou(xa[n1].astype(F32))
        for j in range(4):
            for half in range(2):
                w[pl.ds(XS0 + (j * 16 + half * 8) * HP + n1, 8, stride=HP), :] = (
                    v[8 * half:8 * half + 8, j * 128:(j + 1) * 128])

    def precompute(un, j, h, m0, nm, zero=None):
        u = xeu[m0 * 8:(m0 + nm) * 8, :]
        if zero is not None:
            top = jnp.concatenate([u[0:8, 0:128] | zero, u[0:8, 128:D]], axis=1)
            u = jnp.concatenate([top, u[8:]], axis=0)
        r = _nn(_tobf(u), wplane(un, j, h))
        pre[un * 4 + j, m0:m0 + nm, :, h * 128:(h + 1) * 128] = r.reshape(nm, 16, 128)
        return r

    def half_dot(blocks, t, zero=None):
        un, j = blocks[t // 4]
        return precompute(un, j, (t // 2) % 2, (t % 2) * 16, 16, zero)

    def mat(k):
        return _tobf(cm[64 * k:64 * k + 64, :])

    def lo_half(rows):
        return lax.broadcasted_iota(jnp.int32, (rows, 128), 1) < 64

    first = lax.broadcasted_iota(jnp.int32, (8, 128), 0) == 0
    classes = tuple(tuple((UQ * a + r, 8, UP) for r in cl for a in range(4))
                    for cl in ((0, 4), (2, 6), (1, 7), (5, 3)))

    def part(u, h, rows=16):
        return jnp.concatenate([u[(2 * g + h) * rows:(2 * g + h + 1) * rows] for g in range(4)], axis=0)

    def f1_s(n2, x12, kk):
        h, k = kk % 2, kk // 2
        u = _nn(x12[h][k], mat(4 + h))
        r = 0
        for cl in classes[2 * k:2 * k + 2]:
            for (st, n, sd) in cl:
                u_scr[n2, h, pl.ds(st, n, stride=sd), :] = u[r:r + n]
                r += n

    def f1_d(n2, prev):
        def ldx(j):
            r0 = XS0 + (j * 16 + n2) * HP
            u = jnp.concatenate([w[pl.ds(r0 + par, 64, stride=2), :] for par in range(2)], axis=0)
            return pltpu.bitcast(u, F32)

        x0, x1, x2, x3 = [ldx(j) for j in range(4)]
        lo = lo_half(128)
        p, q, b, c = x0 + x2, x1 + x3, x0 - x2, x1 - x3
        r = _swap(jnp.where(lo, c, (b - c) * R2))
        y = jnp.where(lo, b, (b + c) * R2)
        t = []
        for k, a in enumerate((p + q, p - q, y + r, y - r)):
            t.append(_nt(mat(k), a.astype(BF16)))
            if prev is not None:
                f1_s(n2 - LAG, prev, k)
        t256[n2:n2 + 1, :] = t[0][16:17]
        t[0] = jnp.concatenate([t[0][0:16], jnp.where(first, 0.0, t[0][16:24]), t[0][24:128]], axis=0)
        tr = jnp.concatenate([part(u, 0) for u in t], axis=0)
        ti = jnp.concatenate([part(u, 1) for u in t], axis=0)
        lo = lo_half(256)
        rb = _swap(jnp.where(lo, ti, tr))
        x12 = (jnp.where(lo, tr, rb), jnp.where(lo, rb, ti))
        return [[x[128 * k:128 * k + 128].astype(BF16) for k in range(2)] for x in x12]

    def f1_all():
        zvec = _tou(ys[0, 16 * HP + 8:16 * HP + 16, :])
        xq = [None] * LAG
        dots = (0, 2, 4, 7, 9, 11, 14, 17)
        for n2 in range(16 + LAG):
            if n2 in dots:
                k = dots.index(n2)
                r = half_dot(((NA, 3), (NA + 1, 3)), k)
                for j in range(4 if k < 4 else 0):
                    relayout(NA + 1, 4 * k + j, _tou(r[64 * j:64 * j + 8]) & zvec)
            if n2 < 16:
                xq.append(f1_d(n2, xq.pop(0)))
            else:
                xp = xq.pop(0)
                for kk in range(4):
                    f1_s(n2 - LAG, xp, kk)
        t = t256[...]
        lo = lo_half(16)
        for h, v in enumerate((t, _swap(t))):
            u = _nn(jnp.where(lo, v, 0.0).astype(BF16), mat(4 + h))
            for n2 in range(16):
                u_scr[n2, h, U_LAST:U_LAST + 1, :] = u[n2:n2 + 1]

    tok = [None]

    def f2_pieces(ru, filt):
        def ld(n):
            z = [u_scr[n, h, pl.ds(ru, 8), :] for h in range(2)]
            if tok[0] is not None:
                z = [pltpu.bitcast(_tou(v) | tok[0], F32) for v in z]
            return tuple(z)

        lo = lo_half(8)

        def st(n, z):
            u_scr[n, 0, pl.ds(ru, 8), :] = z[0]
            u_scr[n, 1, pl.ds(ru, 8), :] = z[1]

        def ld_in(n):
            e, o = ld(n)
            p, q = e + o, e - o
            r = _swap(jnp.where(lo, q, p))
            re, im = jnp.where(lo, p, r), jnp.where(lo, r, q)
            if n == 0:
                return re, im
            c, s = tw[n:n + 1, :], tw[16 + n:17 + n, :]
            return re * c + im * s, im * c - re * s

        def st_out(n, z):
            re, im = z
            if n:
                c, s = tw[n:n + 1, :], tw[16 + n:17 + n, :]
                re, im = re * c - im * s, im * c + re * s
            a = jnp.where(lo, re, im)
            r = _swap(jnp.where(lo, im, re))
            st(n, (a + r, a - r))

        def outer(b, sign):
            y = _dft4(*[(ld_in if sign < 0 else ld)(4 * a + b) for a in range(4)], sign)
            for a in range(4):
                (st if sign < 0 else st_out)(4 * a + b, y[a])

        def inner(p):
            x = _dft4(*[_cmul_const(ld(4 * p + b), b * p, 16, -1) for b in range(4)], -1)
            y = []
            for q in range(4):
                lanes = slice((p + 4 * q) * 128, (p + 4 * q + 1) * 128)
                a, b = filt(lanes)
                y.append((x[q][0] * a - x[q][1] * b, x[q][0] * b + x[q][1] * a))
            v = _dft4(*y, +1)
            for b in range(4):
                st(4 * p + b, _cmul_const(v[b], b * p, 16, +1))

        return ([functools.partial(outer, b, -1) for b in range(4)],
                [functools.partial(inner, p) for p in range(4)],
                [functools.partial(outer, b, +1) for b in range(4)])

    def f3_s(n2, zero=None):
        lo = lo_half(128)
        zs = []
        for par in range(2):
            cls = [jnp.concatenate([u_scr[n2, par, pl.ds(st, n, stride=sd), :] for (st, n, sd) in cl], axis=0)
                   for cl in classes]
            hmu = cm[64 * (6 + par):64 * (7 + par), :]
            sign = jnp.where(lo_half(8), 2.0 * par - 1.0, 1.0 - 2.0 * par)
            last = _swap(u_scr[n2, par, U_LAST:U_LAST + 8, :]) * sign
            if zero is not None and par == 1:
                last = last + zero
            rhs_a = jnp.concatenate([cls[0], cls[1]], axis=0).astype(BF16)
            rhs_b = jnp.concatenate([jnp.where(first, last, cls[0][0:8]), cls[0][8:64], cls[1]],
                                    axis=0).astype(BF16)
            zo = _nt(_tobf(hmu), jnp.concatenate([cls[2], cls[3]], axis=0).astype(BF16))
            zs.append((_nt(_tobf(part(hmu, 0, 8)), rhs_a), _nt(_tobf(part(hmu, 1, 8)), rhs_b),
                       part(zo, 0), part(zo, 1)))
        out = []
        for k in range(2):
            re = jnp.concatenate([zs[0][2 * k], zs[1][2 * k]], axis=0)
            im = jnp.concatenate([zs[0][2 * k + 1], zs[1][2 * k + 1]], axis=0)
            r = _swap(jnp.where(lo, im, re))
            out += [jnp.where(lo, re, r).astype(BF16), jnp.where(lo, r, im).astype(BF16)]
        return out

    def f3_d(n2, z):
        b0, b2, g1, g5 = [_nn(z[k], mat(8 + k)) for k in range(4)]
        lo = lo_half(128)
        y = g1 + g5
        r = _swap(g1 - g5)
        b = jnp.where(lo, y, (y + r) * R2)
        c = jnp.where(lo, r, (y - r) * R2)
        p, q = b0 + b2, b0 - b2
        for j, v in enumerate((p + b, q + c, p - b, q - c)):
            for par in range(2):
                ys[j, pl.ds(n2 * HP + par, 64, stride=2), :] = v[64 * par:64 * par + 64]

    def gather_y(n1, half):
        v = [ys[j, pl.ds(half * 8 * HP + n1, 8, stride=HP), :] for j in range(4)]
        yb[n1, half * 8:half * 8 + 8, :] = jnp.concatenate(v, axis=1).astype(BF16)

    def f3_all():
        prow = pl.multiple_of(opq[0] + (16 * HP - U_PIN), 8)
        b0 = [(NA + 2 + k, 3) for k in range(N5)]
        nin = len(D3)
        assert nin == 4 * N5 - NTAIL - 2
        wl = [wlast[k].astype(F32) for k in range(2)]
        stages = f2_pieces(U_LAST, lambda lanes: [jnp.broadcast_to(v[:, lanes], (8, 128)) for v in wl])
        zvec = _tou(ys[0, 16 * HP + 8:16 * HP + 16, :])
        r = half_dot(b0, 0)
        for k, pc in enumerate(stages[0] + stages[1] + stages[2]):
            tok[0] = (_tou(r[(k - 4) * 24:(k - 4) * 24 + 8]) & zvec) if k >= 4 else None
            pc()
        tok[0] = None
        half_dot(b0, 1)
        zq = [f3_s(0), f3_s(1)]
        zero = None
        for n2 in range(16):
            if n2 in D3:
                half_dot(b0, 2 + D3.index(n2), _tou(zero) if n2 >= 14 else None)
            if n2 + 2 < 16:
                zq.append(f3_s(n2 + 2, zero))
            zero = ys[0, pl.ds(prow + 8, 8), :]
            f3_d(n2, zq.pop(0))
            if n2 >= 8:
                ys[0, pl.ds(prow, 8), :] = zero
                for n1 in range((n2 - 8) * 16, (n2 - 7) * 16):
                    gather_y(n1, 0)
        npin = 8 * (NTAIL - 1) - 3
        for k in range(NTAIL):
            r = half_dot(b0, 2 + nin + k, _tou(zero) if k == 0 else None)
            for j in range(min(8, npin - 8 * (k - 1)) if k else 0):
                ys[0, pl.ds(prow, 8), :] = r[32 * j:32 * j + 8]
                for n1 in range((8 * k - 8 + j) * 128 // npin, (8 * k - 7 + j) * 128 // npin):
                    gather_y(n1, 1)

    def unit0(k, _):
        wait_raw(k * pu, pu, sems.at[SEM_U0 + k])
        for t in range(pu):
            relayout(0, k * pu + t)
        return 0

    def retile_xe(j):
        xeu[:, 128 * j:128 * j + 128] = _tou(xe[:, :, 128 * j:128 * j + 128].reshape(NIT * 16, 128))

    def partial(b, kh):
        lhs = jnp.concatenate([xeu[:, 128 * j:128 * j + 128] for j in (kh, kh + 2)], axis=1)
        rhs = jnp.concatenate(
            [jnp.concatenate([w[pl.ds((par * 8 + b + 4 * half) * HP + 64 * kh, 64), :] for half in range(2)], axis=0)
             for par in range(2)], axis=1)
        r = _nn(_tobf(lhs), _tobf(rhs))
        r = r.reshape(NIT, 16, 256)
        pre[b] = r + pre[b] if kh else r

    for c in c_xe:
        c.wait()
    retile_xe(0)
    retile_xe(2)
    lax.fori_loop(0, NU0, unit0, 0)
    partial(0, 0)
    partial(1, 0)
    for c in c_u0b:
        c.wait()
    partial(2, 0)
    retile_xe(1)
    retile_xe(3)
    for pc in range(8, 16):
        relayout(0, pc)
    for b in range(B0):
        partial(b, 1)

    def body_a(g, _):
        p0 = 16 * (g + 1)
        wait_raw(p0, 16, sems.at[SEM_A + g])

        @pl.when(g > 0)
        def _():
            gm = jnp.maximum(g - 1, 0)
            blk = xa.at[pl.ds(64 * gm, 64)]
            cp(blk, blk, sems.at[SEM_XA + gm]).wait()

        un = jnp.minimum(g + 1, NA)
        for t in range(8):
            precompute(g, 3, t // 4, (t % 4) * 8, 8)
            relayout(un, 2 * t)
            relayout(un, 2 * t + 1)
        for t in range(12):
            half_dot([(g + 1, j) for j in range(3)], t)
            for k in range(64 * t // 12, 64 * (t + 1) // 12):
                stage_x(jnp.where(g > 0, 64 * (g - 1) + k, 128))
        return 0

    lax.fori_loop(0, NA, body_a, 0)
    for c in c_c:
        c.wait()
    f1_all()

    def body_b(g, _):
        gu = jnp.minimum(g, NB - 2)

        @pl.when(g < NB - 1)
        def _():
            wait_raw(16 * (NA + 2 + gu), 16, sems.at[SEM_U + gu])

        sem = sems.at[SEM_W + g]
        r32 = pl.multiple_of(g * 32, 32)
        for blk in (wo_raw.at[pl.ds(pl.multiple_of(g * WO_ROWS, WO_ROWS), WO_ROWS)],
                    wr.at[pl.ds(r32, 32)], wi.at[pl.ds(r32, 32)]):
            cp(blk, blk, sem).wait()
        pin_row = pl.multiple_of(opq[0], 8)
        filt = lambda k, lanes: [v[pl.ds(r32 + 8 * k, 8), lanes].astype(F32) for v in (wr, wi)]
        ru = (g >> 1) * UQ + (g & 1) * (4 * UP)
        groups = [f2_pieces(ru + UP * k, functools.partial(filt, k)) for k in range(4)]
        pieces = [pc for st in range(3) for k in range(4) for pc in groups[k][st]]
        nd = 4 * BB
        zeros = [None, None]
        zvec = _tou(ys[0, 16 * HP + 8:16 * HP + 16, :])
        for pc in pieces[:FSPLIT[0]]:
            pc()
        for t in range(nd):
            v = half_dot([(NA + 1 + g, j) for j in range(BB)], t, zeros.pop(0))
            for k in range(16 * t // nd, 16 * (t + 1) // nd):
                relayout(NA + 2 + gu, k)
            for k in range(32 * t // nd, 32 * (t + 1) // nd):
                retile_wo(g * (WO_ROWS // 16) + k)
            todo = pieces[FSPLIT[t]:FSPLIT[t + 1]]
            for k, pc in enumerate(todo):
                r0 = 8 * ((32 * k) // len(todo))
                tok[0] = _tou(v[r0:r0 + 8]) & zvec
                pc()
            tok[0] = None
            zeros.append(_tou(u_scr[0, 0, pl.ds(pin_row + 8, 8), :]) if todo else None)
        return 0

    lax.fori_loop(0, NB, body_b, 0)
    for c in c_f:
        c.wait()
    f3_all()

    rpos = jnp.where(row < 16, L, (row - 16) % SEG + M)
    mask = same_head & (rpos >= col % L)

    def qkv(st, i, lhs, lhs_v, p, even):
        def proj(blk):
            wb = jnp.concatenate([wplane(blk // 4, blk % 4, par) for par in range(2)], axis=1)
            if blk not in NOPRE:
                r = _nn(lhs, wb)
                if even:
                    return r[0:8], jnp.concatenate([r[8:32], pre[blk, i, 0:8, :]], axis=0)
                return r[0:8], jnp.concatenate([pre[blk, i, 8:16, :], r[8:32]], axis=0)
            r = _nn(lhs_v, wb)
            if even:
                carry8[NOPRE.index(blk)] = r[40:48]
                return r[0:8], r[8:40]
            return r[0:8], jnp.concatenate([carry8[NOPRE.index(blk)], r[8:32]], axis=0)

        mq, xq = proj(p)
        mk, xk = proj(NP + p)
        mv, xv = proj(2 * NP + p)
        h0 = lambda a: a[:, 0:128]
        h1 = lambda a: a[:, 128:256]
        st["q"][p] = jnp.concatenate([h0(mq), h1(mq), h0(xq), h1(xq)], axis=0).astype(BF16)
        st["k"][p] = jnp.concatenate([h0(mk), h0(xk), h1(mk), h1(xk)], axis=0).astype(BF16)
        st["v"][p] = jnp.concatenate([h0(mv), h0(xv), h1(mv), h1(xv)], axis=0).astype(BF16)

    def qk_group(st, g):
        for p in range(4 * g, 4 * g + 4):
            s = _nt(st["q"][p], st["k"][p])
            s = jnp.where(mask, s, fill_scr[...])
            m = jnp.max(s, axis=-1, keepdims=True)
            e = jnp.exp2((s - m) * (SCALE * LOG2E))
            l = jnp.sum(e, axis=-1, keepdims=True)
            st["p"][p] = e * pl.reciprocal(l, approx=True)

    def put_om(p, o):
        om_scr[:, (2 * p) * 128:(2 * p + 1) * 128] = o[0:8]
        om_scr[:, (2 * p + 1) * 128:(2 * p + 2) * 128] = o[8:16]

    def put_ox(b, p, o):
        ox_scr[b, :, (2 * p) * 128:(2 * p + 1) * 128] = o[0:32]
        ox_scr[b, :, (2 * p + 1) * 128:(2 * p + 2) * 128] = o[32:64]

    def pvm_group(st, g, b):
        for p in range(4 * g, 4 * g + 4):
            put_om(p, _nn(st["p"][p][0:16].astype(BF16), st["v"][p]))

    def pvx_group(st, g, b):
        for p in range(4 * g, 4 * g + 4):
            put_ox(b, p, _nn(st["p"][p][16:80].astype(BF16), st["v"][p]))

    def pv_group(st, g, b):
        for p in range(4 * g, 4 * g + 4):
            o = _nn(st["p"][p].astype(BF16), st["v"][p])
            put_om(p, o[0:16])
            put_ox(b, p, o[16:80])

    def oproj(c, even, acc):
        cs = slice(c * 512, (c + 1) * 512)
        if even:
            lhs = jnp.concatenate([om_scr[:, cs], ox_scr[1, 0:24, cs]], axis=0)
            tail8[:, cs] = ox_scr[1, 24:32, cs]
        else:
            lhs = jnp.concatenate([om_scr[:, cs], tail8[:, cs], ox_scr[0, :, cs]], axis=0)
        r = _nn(lhs.astype(BF16), wo_rows(c * 512, 512))
        return r if acc is None else r + acc

    def step(i, lhs_v, even, late):
        b = 0 if even else 1
        st = dict(q={}, k={}, v={}, p={})
        lhs = lhs_v[0:32]
        for p in range(4):
            qkv(st, i, lhs, lhs_v, p, even)
        for g in range(3):
            qkv(st, i, lhs, lhs_v, 4 * g + 4, even)
            qk_group(st, g)
            for p in range(4 * g + 5, 4 * g + 8):
                qkv(st, i, lhs, lhs_v, p, even)
                if not late and g and p == 4 * g + 5:
                    pvx_group(st, g - 1, b)
            pvm_group(st, g, b)
        acc = oproj(0, even, None)
        qk_group(st, 3)
        for c in range(1, 4):
            acc = oproj(c, even, acc)
            if not late and c == 1:
                pvx_group(st, 2, b)
        (pvm_group if late else pv_group)(st, 3, b)
        for c in range(4, 8):
            acc = oproj(c, even, acc)
        if late:
            for g in range(4):
                pvx_group(st, g, b)
        return acc

    nb = 4 * (NIT - UNROLL)
    ob = lambda g0, g1: cp(outb.at[g0:g1], out_hbm.at[g0 - 2:g1 - 2, :, D:2 * D], osem)
    c_out = [cp(yb, out_hbm.at[:, :, 0:D], osem), ob(2, nb), ob(nb, 4 * NIT), ob(4 * NIT, 4 * NIT + 2)]

    def even_lhs(i, mem):
        return jnp.concatenate([mem, xb[i, 0:40, :].astype(F32)], axis=0).astype(BF16)

    def pair(i, mem, last):
        acc = step(i, even_lhs(i, mem), True, True)
        outb[4 * i] = acc[8:24].astype(BF16)
        stash = acc[24:32]
        xf = xb[i, 40:64, :].astype(F32)
        acc = step(i, jnp.concatenate([acc[0:8], xf], axis=0).astype(BF16), False, not last)
        o48 = jnp.concatenate([stash, acc[8:48]], axis=0)
        outb[pl.ds(4 * i + 1, 3)] = o48.reshape(3, 16, D).astype(BF16)
        return acc[0:8]

    def body(it, _):
        @pl.when(it == NLOOP - 1)
        def _():
            c_out[0].start()
            c_out[1].start()

        mem = mem_scr[...]
        for u in range(UNROLL):
            mem = pair(it * UNROLL + u, mem, u == UNROLL - 1)
        mem_scr[...] = mem
        return 0

    mem_scr[...] = mem0[...].astype(F32)
    lax.fori_loop(0, NLOOP, body, 0)

    c_out[2].start()
    acc = _nn(ox_scr[1].astype(BF16), wo_rows(0, H * DH))
    outb[4 * NIT:4 * NIT + 2] = acc.reshape(2, 16, D).astype(BF16)
    c_out[3].start()


def _kernel(*refs):
    refs, osem = refs[:-1], refs[-1]
    pl.run_scoped(lambda sems: _body(sems, osem, *refs), pltpu.SemaphoreType.DMA((NSEM,)))
    out_hbm = refs[11]
    pltpu.make_async_copy(out_hbm, out_hbm, osem).wait()


@jax.jit
def pallas_concat_heads__spectral_gfnet__memory_aug_recurrent_mem_tr__prompt_kernel(
    A_x, A_w_r, A_w_i, B_x, B_mem0, B_Wq, B_Wk, B_Wv, B_Wo, B_seg_len,
):
    del B_seg_len
    assert A_x.shape == (1, S, D) and B_x.shape == (1, S, D) and B_mem0.shape == (1, M, D)
    cm, tw = _fft_consts()
    hbm = pl.BlockSpec(memory_space=pltpu.HBM)
    out = pl.pallas_call(
        _kernel,
        out_shape=jax.ShapeDtypeStruct((S // 16, 16, 2 * D), BF16),
        in_specs=[hbm] * 11,
        out_specs=hbm,
        scratch_shapes=[
            pltpu.VMEM((129, 16, D), BF16),
            pltpu.VMEM((4, 16 * HP + 128, 128), F32),
            pltpu.VMEM((256, S), BF16),
            pltpu.VMEM((256, S), BF16),
            pltpu.VMEM((12 * 64, 128), U32),
            pltpu.VMEM((32, 128), F32),
            pltpu.VMEM((16, 2, U_ROWS, 128), F32),
            pltpu.VMEM((128, 16, D), BF16),
            pltpu.VMEM((NIT, 2 * SEG, D), BF16),
            pltpu.VMEM((NIT, 16, D), BF16),
            pltpu.VMEM((NIT * 8, D), U32),
            pltpu.VMEM((6 * D, 16, 128), BF16),
            pltpu.VMEM((XS0 + 64 * HP + 160, 128), U32),
            pltpu.VMEM((H * DH, D), BF16),
            pltpu.VMEM((3 * NP, NIT, 16, 256), F32),
            pltpu.VMEM((M, D), F32),
            pltpu.VMEM((8, H * DH), F32),
            pltpu.VMEM((M, H * DH), F32),
            pltpu.VMEM((2, SEG, H * DH), F32),
            pltpu.VMEM((4 * NIT + 2, 16, D), BF16),
            pltpu.VMEM((2, 1, S), BF16),
            pltpu.VMEM((16, 128), F32),
            pltpu.VMEM((M, D), BF16),
            pltpu.VMEM((len(NOPRE), 8, 256), F32),
            pltpu.VMEM((80, 80), F32),
            pltpu.SMEM((1,), jnp.int32),
            pltpu.SemaphoreType.DMA(()),
        ],
        compiler_params=pltpu.CompilerParams(vmem_limit_bytes=110 * 1024 * 1024),
    )(
        A_x.reshape(S // 16, 16, D), A_w_r.T, A_w_i.T,
        B_x.reshape(NIT, 2 * SEG, D), B_mem0.reshape(M, D),
        B_Wq, B_Wk, B_Wv, B_Wo.reshape(H * DH, D),
        jnp.asarray(cm), jnp.asarray(tw),
    )
    return out.reshape(1, S, 2 * D)
```

```python
import functools

import numpy as np
import jax
import jax.numpy as jnp
from jax import lax
import jax.experimental.pallas as pl
import jax.experimental.pallas.tpu as pltpu

F32 = jnp.float32
BF16 = jnp.bfloat16
U32 = jnp.uint32

S, D = 2048, 512
H, DH = 32, 128
M, SEG = 8, 32
L = M + SEG
NP = H // 2
NIT = S // (2 * SEG)
SCALE = DH ** -0.5
LOG2E = 1.4426950408889634
NEG = -1000000000.0
R2 = float(np.sqrt(0.5))


def _nt(a, b):
    return lax.dot_general(a, b, (((1,), (1,)), ((), ())), preferred_element_type=F32)


def _nn(a, b):
    return jnp.dot(a, b, preferred_element_type=F32)


def _tobf(u):
    return pltpu.bitcast(u, BF16)


def _tou(b):
    return pltpu.bitcast(b, U32)


def _swap(a):
    return pltpu.roll(a, 64, a.ndim - 1)


def _cs(num, den):
    ang = 2.0 * np.pi * np.mod(num, den) / den
    c, s = np.cos(ang), np.sin(ang)
    c[np.abs(c) < 1e-12] = 0.0
    s[np.abs(s) < 1e-12] = 0.0
    return c, s


def _pack_rows(a):
    b = np.asarray(a, np.float32).astype(jnp.bfloat16).view(np.uint16).astype(np.uint32)
    return b[0::2] | (b[1::2] << 16)


def _fft_consts():
    d1, e64, j32 = np.arange(128), np.arange(64), np.arange(32)
    f0 = np.concatenate([8 * j32, 8 * j32 + 4])
    f2 = np.concatenate([8 * j32 + 2, 8 * j32 + 6])
    fa = np.concatenate([8 * j32 + 1, 8 * j32 + 7])
    fb = np.concatenate([8 * j32 + 5, 8 * j32 + 3])
    c, s = _cs(np.outer(f0, d1), D)
    l0 = np.concatenate([c, -s], 0)
    l0[64] = 1.0 - 2.0 * (d1 % 2)
    c, s = _cs(np.outer(f2, d1), D)
    l2 = np.concatenate([c, -s], 0)

    def odd(f, imsign):
        c, s = _cs(np.outer(f, e64), D)
        sg = np.where(f % 4 == 1, imsign, -imsign)[:, None]
        return np.block([[c, sg * s], [-s, sg * c]])

    la, lb = odd(fa, -1.0), odd(fb, 1.0)
    g, hm = [], []
    for par in range(2):
        c, s = _cs(np.outer(2 * e64 + par, e64), 128)
        sg = 1.0 - 2.0 * par
        g.append(np.block([[c, -s], [s, c]]))
        hm.append(np.block([[c, -sg * s], [s, sg * c]]))
    sc = 2.0 / (S * D)
    i0 = sc * l0
    i0[0] *= 0.5
    i0[64] *= 0.5
    il = lambda a: a.reshape(2, 4, 16, 128).transpose(1, 0, 2, 3).reshape(128, 128)
    mats = [il(l0), il(l2), il(la), il(lb), g[0], g[1], il(hm[0]), il(hm[1]), i0, sc * l2, sc * la, sc * lb]
    tc, ts = _cs(np.outer(np.arange(16), d1), S)
    return _pack_rows(np.concatenate(mats, 0)), np.concatenate([tc, ts], 0).astype(np.float32)


def _cmul_const(z, k, n, sign):
    re, im = z
    k = k % n
    if k == 0:
        return z
    if 4 * k == n:
        return (-im, re) if sign > 0 else (im, -re)
    c = float(np.cos(2 * np.pi * k / n))
    s = float(sign * np.sin(2 * np.pi * k / n))
    if (8 * k) % n == 0:
        a, b = re * c, im * c
        return (a - b, b + a) if s / c > 0 else (a + b, b - a)
    return (re * c - im * s, re * s + im * c)


def _dft4(a, b, c, d, sign):
    s0 = (a[0] + c[0], a[1] + c[1])
    s1 = (a[0] - c[0], a[1] - c[1])
    s2 = (b[0] + d[0], b[1] + d[1])
    s3 = (b[0] - d[0], b[1] - d[1])
    y0 = (s0[0] + s2[0], s0[1] + s2[1])
    y2 = (s0[0] - s2[0], s0[1] - s2[1])
    ya = (s1[0] + s3[1], s1[1] - s3[0])
    yb = (s1[0] - s3[1], s1[1] + s3[0])
    return [y0, ya, y2, yb] if sign < 0 else [y0, yb, y2, ya]


UNROLL = 4
NLOOP = NIT // UNROLL
NU0 = 2
NA, NB = 3, 8
BB = 3
N5 = 3
NTAIL = 4
B0 = 3
NOPRE = (35, 39, 43, 47)
FSPLIT = (4, 8, 12, 16, 20, 24, 28, 32, 36, 40, 44, 48, 48)
LAG = 2
D3 = (3, 6, 9, 11, 14, 15)
UP = 9
HP = 132
UQ = 96
U_LAST = 4 * UQ
U_PIN, U_ROWS = 392, 408
WO0 = 12 * 16 * HP
WO_ROWS = H * DH // NB
XS0 = WO0 + 4 * 2048

SEM_U0 = 0
SEM_XE = SEM_U0 + NU0
SEM_U0B = SEM_XE + 1
SEM_A = SEM_U0B + 1
SEM_XA = SEM_A + NA
SEM_C = SEM_XA + 2
SEM_W = SEM_C + 1
SEM_U = SEM_W + NB
SEM_F = SEM_U + NB - 1
NSEM = SEM_F + 1


def _body(sems, osem, xa_hbm, wr_hbm, wi_hbm, xb_hbm, mem0_hbm, wq_hbm, wk_hbm, wv_hbm, wo_hbm,
          cm_hbm, tw_hbm, out_hbm,
          xa, ys, wr, wi, cm, tw, u_scr, yb, xb, xe, xeu,
          raw, w, wo_raw, pre, mem_scr, tail8, om_scr, ox_scr, outb,
          wlast, t256, mem0, carry8, fill_scr, opq):
    cp = pltpu.make_async_copy

    wsrc = (wq_hbm, wk_hbm, wv_hbm)

    def w_copies(p0, p1, sem):
        out = []
        while p0 < p1:
            u, c = divmod(p0, 16)
            n = min(p1 - p0, 16 - c)
            for half in range(2):
                d0 = 256 * half + 16 * c
                out.append(cp(wsrc[u // 4].at[d0:d0 + 16 * n, 8 * (u % 4):8 * (u % 4) + 8, :],
                              raw.at[16 * p0:16 * (p0 + n), 8 * half:8 * half + 8, :], sem))
            p0 += n
        return out

    pu = 8 // NU0
    xe_cp = lambda j, sem: cp(xb_hbm.at[:, 24:40, 128 * j:128 * j + 128],
                              xe.at[:, :, 128 * j:128 * j + 128], sem)
    c_xe = [xe_cp(0, sems.at[SEM_XE]), xe_cp(2, sems.at[SEM_XE])]
    c_in = list(c_xe)
    for k in range(NU0):
        c_in += w_copies(k * pu, (k + 1) * pu, sems.at[SEM_U0 + k])
    c_u0b = [xe_cp(1, sems.at[SEM_U0B]), xe_cp(3, sems.at[SEM_U0B])] + w_copies(8, 16, sems.at[SEM_U0B])
    c_in += c_u0b
    for g in range(NA):
        c_in += w_copies(16 * (g + 1), 16 * (g + 2), sems.at[SEM_A + g])
        if g:
            c_in.append(cp(xa_hbm.at[64 * (g - 1):64 * g], xa.at[64 * (g - 1):64 * g], sems.at[SEM_XA + g - 1]))
    c_c = [cp(cm_hbm, cm, sems.at[SEM_C]), cp(tw_hbm, tw, sems.at[SEM_C])]
    c_c += w_copies(16 * (NA + 1), 16 * (NA + 2), sems.at[SEM_C])
    c_in += c_c
    for g in range(NB):
        sem = sems.at[SEM_W + g]
        if g < NB - 1:
            c_in += w_copies(16 * (NA + 2 + g), 16 * (NA + 3 + g), sems.at[SEM_U + g])
        rows = slice(g * WO_ROWS, (g + 1) * WO_ROWS)
        c_in.append(cp(wo_hbm.at[rows], wo_raw.at[rows], sem))
        rows = slice(32 * g, 32 * g + 32)
        c_in += [cp(wr_hbm.at[rows], wr.at[rows], sem), cp(wi_hbm.at[rows], wi.at[rows], sem)]
    c_f = [cp(mem0_hbm, mem0, sems.at[SEM_F]),
           cp(wr_hbm.at[256:257], wlast.at[0], sems.at[SEM_F]),
           cp(wi_hbm.at[256:257], wlast.at[1], sems.at[SEM_F]),
           cp(xb_hbm, xb, sems.at[SEM_F])]
    for c in c_in + c_f:
        c.start()

    opq[0] = U_PIN
    ox_scr[1] = jnp.zeros((SEG, H * DH), F32)
    u_scr[:, :, U_LAST:U_LAST + 8, :] = jnp.zeros((16, 2, 8, 128), F32)
    u_scr[0, 0, U_PIN + 8:U_PIN + 16, :] = jnp.zeros((8, 128), F32)
    ys[0, 16 * HP + 8:16 * HP + 16, :] = jnp.zeros((8, 128), F32)
    xa[128] = jnp.zeros((16, D), BF16)

    row = lax.broadcasted_iota(jnp.int32, (80, 80), 0)
    col = lax.broadcasted_iota(jnp.int32, (80, 80), 1)
    rhead = jnp.where(row < 16, row // 8, (row - 16) // SEG)
    same_head = rhead == col // L
    fill_scr[...] = jnp.where(same_head, NEG / SCALE, -jnp.inf).astype(F32)

    def wait_raw(p0, n, sem):
        blk = raw.at[pl.ds(p0 * 16, n * 16)]
        cp(blk, blk, sem).wait()

    def relayout(u, c, zero=None):
        eo = _tou(raw[pl.ds(u * 256 + c * 16, 16)])
        if zero is not None:
            eo = eo | zero
        eo = eo.reshape(8, 2, 8, 128)
        e, o = eo[:, 0], eo[:, 1]
        h0 = (e & jnp.uint32(0xFFFF)) | (o << 16)
        h1 = (e >> 16) | (o & jnp.uint32(0xFFFF0000))
        base = u * (16 * HP) + c * 8
        for par, hh in enumerate((h0, h1)):
            for t in range(8):
                w[pl.ds(base + par * 8 * HP + t, 8, stride=HP), :] = hh[t]

    def wplane(u, j, par):
        r0 = u * (16 * HP) + (par * 8 + j) * HP
        return _tobf(jnp.concatenate([w[pl.ds(r0, 128), :], w[pl.ds(r0 + 4 * HP, 128), :]], axis=0))

    def retile_wo(r16):
        v = _tou(wo_raw[pl.ds(pl.multiple_of(r16 * 16, 16), 16), :])
        for j in range(4):
            w[pl.ds(WO0 + j * 2048 + r16 * 8, 8), :] = v[:, j * 128:(j + 1) * 128]

    def wo_rows(r0, n):
        return _tobf(jnp.concatenate(
            [w[WO0 + j * 2048 + r0 // 2:WO0 + j * 2048 + (r0 + n) // 2, :] for j in range(4)], axis=1))

    def stage_x(n1):
        v = _tou(xa[n1].astype(F32))
        for j in range(4):
            for half in range(2):
                w[pl.ds(XS0 + (j * 16 + half * 8) * HP + n1, 8, stride=HP), :] = (
                    v[8 * half:8 * half + 8, j * 128:(j + 1) * 128])

    def precompute(un, j, h, m0, nm, zero=None):
        u = xeu[m0 * 8:(m0 + nm) * 8, :]
        if zero is not None:
            top = jnp.concatenate([u[0:8, 0:128] | zero, u[0:8, 128:D]], axis=1)
            u = jnp.concatenate([top, u[8:]], axis=0)
        r = _nn(_tobf(u), wplane(un, j, h))
        pre[un * 4 + j, m0:m0 + nm, :, h * 128:(h + 1) * 128] = r.reshape(nm, 16, 128)
        return r

    def half_dot(blocks, t, zero=None):
        un, j = blocks[t // 4]
        return precompute(un, j, (t // 2) % 2, (t % 2) * 16, 16, zero)

    def mat(k):
        return _tobf(cm[64 * k:64 * k + 64, :])

    def lo_half(rows):
        return lax.broadcasted_iota(jnp.int32, (rows, 128), 1) < 64

    first = lax.broadcasted_iota(jnp.int32, (8, 128), 0) == 0
    classes = tuple(tuple((UQ * a + r, 8, UP) for r in cl for a in range(4))
                    for cl in ((0, 4), (2, 6), (1, 7), (5, 3)))

    def part(u, h, rows=16):
        return jnp.concatenate([u[(2 * g + h) * rows:(2 * g + h + 1) * rows] for g in range(4)], axis=0)

    def f1_s(n2, x12, kk):
        h, k = kk % 2, kk // 2
        u = _nn(x12[h][k], mat(4 + h))
        r = 0
        for cl in classes[2 * k:2 * k + 2]:
            for (st, n, sd) in cl:
                u_scr[n2, h, pl.ds(st, n, stride=sd), :] = u[r:r + n]
                r += n

    def f1_d(n2, prev):
        def ldx(j):
            r0 = XS0 + (j * 16 + n2) * HP
            u = jnp.concatenate([w[pl.ds(r0 + par, 64, stride=2), :] for par in range(2)], axis=0)
            return pltpu.bitcast(u, F32)

        x0, x1, x2, x3 = [ldx(j) for j in range(4)]
        lo = lo_half(128)
        p, q, b, c = x0 + x2, x1 + x3, x0 - x2, x1 - x3
        r = _swap(jnp.where(lo, c, (b - c) * R2))
        y = jnp.where(lo, b, (b + c) * R2)
        t = []
        for k, a in enumerate((p + q, p - q, y + r, y - r)):
            t.append(_nt(mat(k), a.astype(BF16)))
            if prev is not None:
                f1_s(n2 - LAG, prev, k)
        t256[n2:n2 + 1, :] = t[0][16:17]
        t[0] = jnp.concatenate([t[0][0:16], jnp.where(first, 0.0, t[0][16:24]), t[0][24:128]], axis=0)
        tr = jnp.concatenate([part(u, 0) for u in t], axis=0)
        ti = jnp.concatenate([part(u, 1) for u in t], axis=0)
        lo = lo_half(256)
        rb = _swap(jnp.where(lo, ti, tr))
        x12 = (jnp.where(lo, tr, rb), jnp.where(lo, rb, ti))
        return [[x[128 * k:128 * k + 128].astype(BF16) for k in range(2)] for x in x12]

    def f1_all():
        zvec = _tou(ys[0, 16 * HP + 8:16 * HP + 16, :])
        xq = [None] * LAG
        dots = (0, 2, 4, 7, 9, 11, 14, 17)
        for n2 in range(16 + LAG):
            if n2 in dots:
                k = dots.index(n2)
                r = half_dot(((NA, 3), (NA + 1, 3)), k)
                for j in range(4 if k < 4 else 0):
                    relayout(NA + 1, 4 * k + j, _tou(r[64 * j:64 * j + 8]) & zvec)
            if n2 < 16:
                xq.append(f1_d(n2, xq.pop(0)))
            else:
                xp = xq.pop(0)
                for kk in range(4):
                    f1_s(n2 - LAG, xp, kk)
        t = t256[...]
        lo = lo_half(16)
        for h, v in enumerate((t, _swap(t))):
            u = _nn(jnp.where(lo, v, 0.0).astype(BF16), mat(4 + h))
            for n2 in range(16):
                u_scr[n2, h, U_LAST:U_LAST + 1, :] = u[n2:n2 + 1]

    tok = [None]

    def f2_pieces(ru, filt):
        def ld(n):
            z = [u_scr[n, h, pl.ds(ru, 8), :] for h in range(2)]
            if tok[0] is not None:
                z = [pltpu.bitcast(_tou(v) | tok[0], F32) for v in z]
            return tuple(z)

        lo = lo_half(8)

        def st(n, z):
            u_scr[n, 0, pl.ds(ru, 8), :] = z[0]
            u_scr[n, 1, pl.ds(ru, 8), :] = z[1]

        def ld_in(n):
            e, o = ld(n)
            p, q = e + o, e - o
            r = _swap(jnp.where(lo, q, p))
            re, im = jnp.where(lo, p, r), jnp.where(lo, r, q)
            if n == 0:
                return re, im
            c, s = tw[n:n + 1, :], tw[16 + n:17 + n, :]
            return re * c + im * s, im * c - re * s

        def st_out(n, z):
            re, im = z
            if n:
                c, s = tw[n:n + 1, :], tw[16 + n:17 + n, :]
                re, im = re * c - im * s, im * c + re * s
            a = jnp.where(lo, re, im)
            r = _swap(jnp.where(lo, im, re))
            st(n, (a + r, a - r))

        def outer(b, sign):
            y = _dft4(*[(ld_in if sign < 0 else ld)(4 * a + b) for a in range(4)], sign)
            for a in range(4):
                (st if sign < 0 else st_out)(4 * a + b, y[a])

        def inner(p):
            x = _dft4(*[_cmul_const(ld(4 * p + b), b * p, 16, -1) for b in range(4)], -1)
            y = []
            for q in range(4):
                lanes = slice((p + 4 * q) * 128, (p + 4 * q + 1) * 128)
                a, b = filt(lanes)
                y.append((x[q][0] * a - x[q][1] * b, x[q][0] * b + x[q][1] * a))
            v = _dft4(*y, +1)
            for b in range(4):
                st(4 * p + b, _cmul_const(v[b], b * p, 16, +1))

        return ([functools.partial(outer, b, -1) for b in range(4)],
                [functools.partial(inner, p) for p in range(4)],
                [functools.partial(outer, b, +1) for b in range(4)])

    def f3_s(n2, zero=None):
        lo = lo_half(128)
        zs = []
        for par in range(2):
            cls = [jnp.concatenate([u_scr[n2, par, pl.ds(st, n, stride=sd), :] for (st, n, sd) in cl], axis=0)
                   for cl in classes]
            hmu = cm[64 * (6 + par):64 * (7 + par), :]
            sign = jnp.where(lo_half(8), 2.0 * par - 1.0, 1.0 - 2.0 * par)
            last = _swap(u_scr[n2, par, U_LAST:U_LAST + 8, :]) * sign
            if zero is not None and par == 1:
                last = last + zero
            rhs_a = jnp.concatenate([cls[0], cls[1]], axis=0).astype(BF16)
            rhs_b = jnp.concatenate([jnp.where(first, last, cls[0][0:8]), cls[0][8:64], cls[1]],
                                    axis=0).astype(BF16)
            zo = _nt(_tobf(hmu), jnp.concatenate([cls[2], cls[3]], axis=0).astype(BF16))
            zs.append((_nt(_tobf(part(hmu, 0, 8)), rhs_a), _nt(_tobf(part(hmu, 1, 8)), rhs_b),
                       part(zo, 0), part(zo, 1)))
        out = []
        for k in range(2):
            re = jnp.concatenate([zs[0][2 * k], zs[1][2 * k]], axis=0)
            im = jnp.concatenate([zs[0][2 * k + 1], zs[1][2 * k + 1]], axis=0)
            r = _swap(jnp.where(lo, im, re))
            out += [jnp.where(lo, re, r).astype(BF16), jnp.where(lo, r, im).astype(BF16)]
        return out

    def f3_d(n2, z):
        b0, b2, g1, g5 = [_nn(z[k], mat(8 + k)) for k in range(4)]
        lo = lo_half(128)
        y = g1 + g5
        r = _swap(g1 - g5)
        b = jnp.where(lo, y, (y + r) * R2)
        c = jnp.where(lo, r, (y - r) * R2)
        p, q = b0 + b2, b0 - b2
        for j, v in enumerate((p + b, q + c, p - b, q - c)):
            for par in range(2):
                ys[j, pl.ds(n2 * HP + par, 64, stride=2), :] = v[64 * par:64 * par + 64]

    def gather_y(n1, half):
        v = [ys[j, pl.ds(half * 8 * HP + n1, 8, stride=HP), :] for j in range(4)]
        yb[n1, half * 8:half * 8 + 8, :] = jnp.concatenate(v, axis=1).astype(BF16)

    def f3_all():
        prow = pl.multiple_of(opq[0] + (16 * HP - U_PIN), 8)
        b0 = [(NA + 2 + k, 3) for k in range(N5)]
        nin = len(D3)
        assert nin == 4 * N5 - NTAIL - 2
        wl = [wlast[k].astype(F32) for k in range(2)]
        stages = f2_pieces(U_LAST, lambda lanes: [jnp.broadcast_to(v[:, lanes], (8, 128)) for v in wl])
        zvec = _tou(ys[0, 16 * HP + 8:16 * HP + 16, :])
        r = half_dot(b0, 0)
        for k, pc in enumerate(stages[0] + stages[1] + stages[2]):
            tok[0] = (_tou(r[(k - 4) * 24:(k - 4) * 24 + 8]) & zvec) if k >= 4 else None
            pc()
        tok[0] = None
        half_dot(b0, 1)
        zq = [f3_s(0), f3_s(1)]
        zero = None
        for n2 in range(16):
            if n2 in D3:
                half_dot(b0, 2 + D3.index(n2), _tou(zero) if n2 >= 14 else None)
            if n2 + 2 < 16:
                zq.append(f3_s(n2 + 2, zero))
            zero = ys[0, pl.ds(prow + 8, 8), :]
            f3_d(n2, zq.pop(0))
            if n2 >= 8:
                ys[0, pl.ds(prow, 8), :] = zero
                for n1 in range((n2 - 8) * 16, (n2 - 7) * 16):
                    gather_y(n1, 0)
        npin = 8 * (NTAIL - 1) - 3
        for k in range(NTAIL):
            r = half_dot(b0, 2 + nin + k, _tou(zero) if k == 0 else None)
            for j in range(min(8, npin - 8 * (k - 1)) if k else 0):
                ys[0, pl.ds(prow, 8), :] = r[32 * j:32 * j + 8]
                for n1 in range((8 * k - 8 + j) * 128 // npin, (8 * k - 7 + j) * 128 // npin):
                    gather_y(n1, 1)

    def unit0(k, _):
        wait_raw(k * pu, pu, sems.at[SEM_U0 + k])
        for t in range(pu):
            relayout(0, k * pu + t)
        return 0

    def retile_xe(j):
        xeu[:, 128 * j:128 * j + 128] = _tou(xe[:, :, 128 * j:128 * j + 128].reshape(NIT * 16, 128))

    def partial(b, kh):
        lhs = jnp.concatenate([xeu[:, 128 * j:128 * j + 128] for j in (kh, kh + 2)], axis=1)
        rhs = jnp.concatenate(
            [jnp.concatenate([w[pl.ds((par * 8 + b + 4 * half) * HP + 64 * kh, 64), :]
                              for half in range(2)], axis=0) for par in range(2)], axis=1)
        r = _nn(_tobf(lhs), _tobf(rhs))
        r = r.reshape(NIT, 16, 256)
        pre[b] = r + pre[b] if kh else r

    for c in c_xe:
        c.wait()
    retile_xe(0)
    retile_xe(2)
    lax.fori_loop(0, NU0, unit0, 0)
    partial(0, 0)
    partial(1, 0)
    for c in c_u0b:
        c.wait()
    partial(2, 0)
    retile_xe(1)
    retile_xe(3)
    for pc in range(8, 16):
        relayout(0, pc)
    for b in range(B0):
        partial(b, 1)

    def body_a(g, _):
        p0 = 16 * (g + 1)
        wait_raw(p0, 16, sems.at[SEM_A + g])

        @pl.when(g > 0)
        def _():
            gm = jnp.maximum(g - 1, 0)
            blk = xa.at[pl.ds(64 * gm, 64)]
            cp(blk, blk, sems.at[SEM_XA + gm]).wait()

        un = jnp.minimum(g + 1, NA)
        for t in range(8):
            precompute(g, 3, t // 4, (t % 4) * 8, 8)
            relayout(un, 2 * t)
            relayout(un, 2 * t + 1)
        for t in range(12):
            half_dot([(g + 1, j) for j in range(3)], t)
            for k in range(64 * t // 12, 64 * (t + 1) // 12):
                stage_x(jnp.where(g > 0, 64 * (g - 1) + k, 128))
        return 0

    lax.fori_loop(0, NA, body_a, 0)
    for c in c_c:
        c.wait()
    f1_all()

    def body_b(g, _):
        gu = jnp.minimum(g, NB - 2)

        @pl.when(g < NB - 1)
        def _():
            wait_raw(16 * (NA + 2 + gu), 16, sems.at[SEM_U + gu])

        sem = sems.at[SEM_W + g]
        r32 = pl.multiple_of(g * 32, 32)
        for blk in (wo_raw.at[pl.ds(pl.multiple_of(g * WO_ROWS, WO_ROWS), WO_ROWS)],
                    wr.at[pl.ds(r32, 32)], wi.at[pl.ds(r32, 32)]):
            cp(blk, blk, sem).wait()
        pin_row = pl.multiple_of(opq[0], 8)
        filt = lambda k, lanes: [v[pl.ds(r32 + 8 * k, 8), lanes].astype(F32) for v in (wr, wi)]
        ru = (g >> 1) * UQ + (g & 1) * (4 * UP)
        groups = [f2_pieces(ru + UP * k, functools.partial(filt, k)) for k in range(4)]
        pieces = [pc for st in range(3) for k in range(4) for pc in groups[k][st]]
        nd = 4 * BB
        zeros = [None, None]
        zvec = _tou(ys[0, 16 * HP + 8:16 * HP + 16, :])
        for pc in pieces[:FSPLIT[0]]:
            pc()
        for t in range(nd):
            v = half_dot([(NA + 1 + g, j) for j in range(BB)], t, zeros.pop(0))
            for k in range(16 * t // nd, 16 * (t + 1) // nd):
                relayout(NA + 2 + gu, k)
            for k in range(32 * t // nd, 32 * (t + 1) // nd):
                retile_wo(g * (WO_ROWS // 16) + k)
            todo = pieces[FSPLIT[t]:FSPLIT[t + 1]]
            for k, pc in enumerate(todo):
                r0 = 8 * ((32 * k) // len(todo))
                tok[0] = _tou(v[r0:r0 + 8]) & zvec
                pc()
            tok[0] = None
            zeros.append(_tou(u_scr[0, 0, pl.ds(pin_row + 8, 8), :]) if todo else None)
        return 0

    lax.fori_loop(0, NB, body_b, 0)
    for c in c_f:
        c.wait()
    f3_all()

    rpos = jnp.where(row < 16, L, (row - 16) % SEG + M)
    mask = same_head & (rpos >= col % L)

    def qkv(st, i, lhs, lhs_v, p, even):
        def proj(blk):
            wb = jnp.concatenate([wplane(blk // 4, blk % 4, par) for par in range(2)], axis=1)
            if blk not in NOPRE:
                r = _nn(lhs, wb)
                if even:
                    return r[0:8], jnp.concatenate([r[8:32], pre[blk, i, 0:8, :]], axis=0)
                return r[0:8], jnp.concatenate([pre[blk, i, 8:16, :], r[8:32]], axis=0)
            r = _nn(lhs_v, wb)
            if even:
                carry8[NOPRE.index(blk)] = r[40:48]
                return r[0:8], r[8:40]
            return r[0:8], jnp.concatenate([carry8[NOPRE.index(blk)], r[8:32]], axis=0)

        mq, xq = proj(p)
        mk, xk = proj(NP + p)
        mv, xv = proj(2 * NP + p)
        h0 = lambda a: a[:, 0:128]
        h1 = lambda a: a[:, 128:256]
        st["q"][p] = jnp.concatenate([h0(mq), h1(mq), h0(xq), h1(xq)], axis=0).astype(BF16)
        st["k"][p] = jnp.concatenate([h0(mk), h0(xk), h1(mk), h1(xk)], axis=0).astype(BF16)
        st["v"][p] = jnp.concatenate([h0(mv), h0(xv), h1(mv), h1(xv)], axis=0).astype(BF16)

    def qk_group(st, g):
        for p in range(4 * g, 4 * g + 4):
            s = _nt(st["q"][p], st["k"][p])
            s = jnp.where(mask, s, fill_scr[...])
            m = jnp.max(s, axis=-1, keepdims=True)
            e = jnp.exp2((s - m) * (SCALE * LOG2E))
            l = jnp.sum(e, axis=-1, keepdims=True)
            st["p"][p] = e * pl.reciprocal(l, approx=True)

    def put_om(p, o):
        om_scr[:, (2 * p) * 128:(2 * p + 1) * 128] = o[0:8]
        om_scr[:, (2 * p + 1) * 128:(2 * p + 2) * 128] = o[8:16]

    def put_ox(b, p, o):
        ox_scr[b, :, (2 * p) * 128:(2 * p + 1) * 128] = o[0:32]
        ox_scr[b, :, (2 * p + 1) * 128:(2 * p + 2) * 128] = o[32:64]

    def pvm_group(st, g, b):
        for p in range(4 * g, 4 * g + 4):
            put_om(p, _nn(st["p"][p][0:16].astype(BF16), st["v"][p]))

    def pvx_group(st, g, b):
        for p in range(4 * g, 4 * g + 4):
            put_ox(b, p, _nn(st["p"][p][16:80].astype(BF16), st["v"][p]))

    def pv_group(st, g, b):
        for p in range(4 * g, 4 * g + 4):
            o = _nn(st["p"][p].astype(BF16), st["v"][p])
            put_om(p, o[0:16])
            put_ox(b, p, o[16:80])

    def oproj(c, even, acc):
        cs = slice(c * 512, (c + 1) * 512)
        if even:
            lhs = jnp.concatenate([om_scr[:, cs], ox_scr[1, 0:24, cs]], axis=0)
            tail8[:, cs] = ox_scr[1, 24:32, cs]
        else:
            lhs = jnp.concatenate([om_scr[:, cs], tail8[:, cs], ox_scr[0, :, cs]], axis=0)
        r = _nn(lhs.astype(BF16), wo_rows(c * 512, 512))
        return r if acc is None else r + acc

    def step(i, lhs_v, even, late):
        b = 0 if even else 1
        st = dict(q={}, k={}, v={}, p={})
        lhs = lhs_v[0:32]
        for p in range(4):
            qkv(st, i, lhs, lhs_v, p, even)
        for g in range(3):
            qkv(st, i, lhs, lhs_v, 4 * g + 4, even)
            qk_group(st, g)
            for p in range(4 * g + 5, 4 * g + 8):
                qkv(st, i, lhs, lhs_v, p, even)
                if not late and g and p == 4 * g + 5:
                    pvx_group(st, g - 1, b)
            pvm_group(st, g, b)
        acc = oproj(0, even, None)
        qk_group(st, 3)
        for c in range(1, 4):
            acc = oproj(c, even, acc)
            if not late and c == 1:
                pvx_group(st, 2, b)
        (pvm_group if late else pv_group)(st, 3, b)
        for c in range(4, 8):
            acc = oproj(c, even, acc)
        if late:
            for g in range(4):
                pvx_group(st, g, b)
        return acc

    nb = 4 * (NIT - UNROLL)
    ob = lambda g0, g1: cp(outb.at[g0:g1], out_hbm.at[g0 - 2:g1 - 2, :, D:2 * D], osem)
    c_out = [cp(yb, out_hbm.at[:, :, 0:D], osem), ob(2, nb), ob(nb, 4 * NIT), ob(4 * NIT, 4 * NIT + 2)]

    def even_lhs(i, mem):
        return jnp.concatenate([mem, xb[i, 0:40, :].astype(F32)], axis=0).astype(BF16)

    def pair(i, mem, last):
        acc = step(i, even_lhs(i, mem), True, True)
        outb[4 * i] = acc[8:24].astype(BF16)
        stash = acc[24:32]
        xf = xb[i, 40:64, :].astype(F32)
        acc = step(i, jnp.concatenate([acc[0:8], xf], axis=0).astype(BF16), False, not last)
        o48 = jnp.concatenate([stash, acc[8:48]], axis=0)
        outb[pl.ds(4 * i + 1, 3)] = o48.reshape(3, 16, D).astype(BF16)
        return acc[0:8]

    def body(it, _):
        @pl.when(it == NLOOP - 1)
        def _():
            c_out[0].start()
            c_out[1].start()

        mem = mem_scr[...]
        for u in range(UNROLL):
            mem = pair(it * UNROLL + u, mem, u == UNROLL - 1)
        mem_scr[...] = mem
        return 0

    mem_scr[...] = mem0[...].astype(F32)
    lax.fori_loop(0, NLOOP, body, 0)

    c_out[2].start()
    acc = _nn(ox_scr[1].astype(BF16), wo_rows(0, H * DH))
    outb[4 * NIT:4 * NIT + 2] = acc.reshape(2, 16, D).astype(BF16)
    c_out[3].start()


def _kernel(*refs):
    refs, osem = refs[:-1], refs[-1]
    pl.run_scoped(lambda sems: _body(sems, osem, *refs), pltpu.SemaphoreType.DMA((NSEM,)))
    out_hbm = refs[11]
    pltpu.make_async_copy(out_hbm, out_hbm, osem).wait()


@jax.jit
def pallas_concat_heads__spectral_gfnet__memory_aug_recurrent_mem_tr__prompt_kernel(
    A_x, A_w_r, A_w_i, B_x, B_mem0, B_Wq, B_Wk, B_Wv, B_Wo, B_seg_len,
):
    del B_seg_len
    assert A_x.shape == (1, S, D) and B_x.shape == (1, S, D) and B_mem0.shape == (1, M, D)
    cm, tw = _fft_consts()
    hbm = pl.BlockSpec(memory_space=pltpu.HBM)
    out = pl.pallas_call(
        _kernel,
        out_shape=jax.ShapeDtypeStruct((S // 16, 16, 2 * D), BF16),
        in_specs=[hbm] * 11,
        out_specs=hbm,
        scratch_shapes=[
            pltpu.VMEM((129, 16, D), BF16),
            pltpu.VMEM((4, 16 * HP + 128, 128), F32),
            pltpu.VMEM((256, S), BF16),
            pltpu.VMEM((256, S), BF16),
            pltpu.VMEM((12 * 64, 128), U32),
            pltpu.VMEM((32, 128), F32),
            pltpu.VMEM((16, 2, U_ROWS, 128), F32),
            pltpu.VMEM((128, 16, D), BF16),
            pltpu.VMEM((NIT, 2 * SEG, D), BF16),
            pltpu.VMEM((NIT, 16, D), BF16),
            pltpu.VMEM((NIT * 8, D), U32),
            pltpu.VMEM((6 * D, 16, 128), BF16),
            pltpu.VMEM((XS0 + 64 * HP + 160, 128), U32),
            pltpu.VMEM((H * DH, D), BF16),
            pltpu.VMEM((3 * NP, NIT, 16, 256), F32),
            pltpu.VMEM((M, D), F32),
            pltpu.VMEM((8, H * DH), F32),
            pltpu.VMEM((M, H * DH), F32),
            pltpu.VMEM((2, SEG, H * DH), F32),
            pltpu.VMEM((4 * NIT + 2, 16, D), BF16),
            pltpu.VMEM((2, 1, S), BF16),
            pltpu.VMEM((16, 128), F32),
            pltpu.VMEM((M, D), BF16),
            pltpu.VMEM((len(NOPRE), 8, 256), F32),
            pltpu.VMEM((80, 80), F32),
            pltpu.SMEM((1,), jnp.int32),
            pltpu.SemaphoreType.DMA(()),
        ],
        compiler_params=pltpu.CompilerParams(vmem_limit_bytes=110 * 1024 * 1024),
    )(
        A_x.reshape(S // 16, 16, D), A_w_r.T, A_w_i.T,
        B_x.reshape(NIT, 2 * SEG, D), B_mem0.reshape(M, D),
        B_Wq, B_Wk, B_Wv, B_Wo.reshape(H * DH, D),
        jnp.asarray(cm), jnp.asarray(tw),
    )
    return out.reshape(1, S, 2 * D)
```
